```python
import jax
import jax.numpy as jnp

def _softmax(x, axis=-1):
    return jax.nn.softmax(x, axis=axis)
def _gelu(x):
    return jax.nn.gelu(x, approximate=True)
def _silu(x):
    return jax.nn.silu(x)
def _sigmoid(x):
    return jax.nn.sigmoid(x)
def _layernorm(x, axis=-1, eps=1e-5):
    m = jnp.mean(x, axis=axis, keepdims=True)
    v = jnp.var(x, axis=axis, keepdims=True)
    return (x - m) / jnp.sqrt(v + eps)
def _scatter_add(tgt, idx, src, axis=0):
    return tgt.at[idx].add(src)
def _segment_sum(src, seg, n):
    return jax.ops.segment_sum(src, seg, n)
class _Rng:
    def __init__(self, key):
        self._k = key
    def _next(self):
        self._k, sub = jax.random.split(self._k)
        return sub
    def normal(self, shape):
        return jax.random.normal(self._next(), shape, dtype=jnp.bfloat16)
    def randint(self, lo, hi, shape):
        return jax.random.randint(self._next(), shape, lo, hi, dtype=jnp.int32)
    def uniform(self, shape, lo=0.0, hi=1.0):
        return jax.random.uniform(self._next(), shape, jnp.bfloat16, lo, hi)
    def permutation(self, n):
        return jax.random.permutation(self._next(), n)


kernel_name = 'parallel_sum__ssm_conv_h3__dense_activation_gelu__prompt'

def setup_inputs():
    _rng = _Rng(jax.random.key(int.from_bytes(__import__("os").urandom(4), "little")))
    _w = (lambda a: (lambda t: t.astype(jnp.bfloat16) if jnp.issubdtype(t.dtype, jnp.floating) else t)(jnp.asarray(a)))
    def _A_setup():
        B, S, D = 1, 2048, 640
        ks = 4
        return {
            "q": _w((lambda *s: _rng.normal(s) * 0.05)(B, S, D)),
            "k": _w((lambda *s: _rng.normal(s) * 0.05)(B, S, D)),
            "v": _w((lambda *s: _rng.normal(s) * 0.05)(B, S, D)),
            "shift_k": _w((lambda *s: _rng.normal(s) * 0.05)(D, ks) * 0.5),
            "ssm_k": _w((lambda *s: _rng.normal(s) * 0.05)(D, S) * (1.0 / S ** 0.5)),
            "ssm_D": _w((lambda *s: _rng.normal(s) * 0.05)(D)),
        }
    _A_in = _A_setup()

    def _B_setup():
        B, S, D, F = 1, 2048, 640, 1728
        return {
            "x": _w((lambda *s: _rng.normal(s) * 0.05)(B, S, D)),
            "w1": _w((lambda *s: _rng.normal(s) * 0.05)(D, F) * (D ** -0.5)),
            "b1": _w((lambda *s: _rng.normal(s) * 0.05)(F) * 0.01),
            "w2": _w((lambda *s: _rng.normal(s) * 0.05)(F, D) * (F ** -0.5)),
            "b2": _w((lambda *s: _rng.normal(s) * 0.05)(D) * 0.01),
        }
    _B_in = _B_setup()

    return {
        "A_q": _A_in["q"],
        "A_k": _A_in["k"],
        "A_v": _A_in["v"],
        "A_shift_k": _A_in["shift_k"],
        "A_ssm_k": _A_in["ssm_k"],
        "A_ssm_D": _A_in["ssm_D"],
        "B_x": _B_in["x"],
        "B_w1": _B_in["w1"],
        "B_b1": _B_in["b1"],
        "B_w2": _B_in["w2"],
        "B_b2": _B_in["b2"],
    }

def reference(A_q, A_k, A_v, A_shift_k, A_ssm_k, A_ssm_D, B_x, B_w1, B_b1, B_w2, B_b2):
    def _A_ref(q, k, v, shift_k, ssm_k, ssm_D):
        B, S, D = q.shape
        ks = shift_k.shape[-1]
        k_pad = jnp.pad(k, ((0, 0), (ks - 1, 0), (0, 0)))
        k_shift = jnp.zeros_like(k)
        for t in range(ks):
            k_shift = k_shift + k_pad[:, t:t + S, :] * shift_k[:, ks - 1 - t][None, None, :]
        kv = k_shift * v
        L = 2 * S
        kv_pad = jnp.pad(kv, ((0, 0), (0, S), (0, 0)))
        kf_pad = jnp.pad(ssm_k, ((0, 0), (0, S)))
        kv_f = (lambda x, axes=(-2,-1): jnp.fft.rfft2(x.astype(jnp.float32), axes=axes))(kv_pad[:, None, :, :], axes=(1, 2))
        kf_f = (lambda x, axes=(-2,-1): jnp.fft.rfft2(x.astype(jnp.float32), axes=axes))(kf_pad[:, None, :], axes=(1, 2))
        kf_f = (lambda x, *d: x.transpose(*d))(kf_f, 1, 2, 0)
        y_f = kv_f * kf_f[None, :, :, :]
        y = (lambda x, s, axes=(-2,-1): jnp.fft.irfft2(x, s=s, axes=axes).astype(jnp.bfloat16))(y_f, (1, L), axes=(1, 2))[:, 0, :S, :]
        y = y + kv * ssm_D[None, None, :]
        return q * y

    def _B_ref(x, w1, b1, w2, b2):
        h = jnp.einsum("bsd,df->bsf", x, w1) + b1
        h = _gelu(h)
        return jnp.einsum("bsf,fd->bsd", h, w2) + b2

    x = A_q
    xn = _layernorm(x, axis=-1)
    return x + _A_ref(xn, A_k, A_v, A_shift_k, A_ssm_k, A_ssm_D) + _B_ref(xn, B_w1, B_b1, B_w2, B_b2)
```

```python
import functools

import numpy as np
import jax
import jax.numpy as jnp
import jax.experimental.pallas as pl
import jax.experimental.pallas.tpu as pltpu

R = 4
P = 128
H = P // 2
TB = R * P
NFFT = 2 * TB
LANES = 128
RG = 8
import os
_E = lambda k, d: int(os.environ.get(k, d))
LAG = int(os.environ.get('LAG', 2))
C_LN, C_PREP, C_FIN = _E('CLN', 135), _E('CP', 100), _E('CF', 135)
PR, LR = _E('PR', 32), _E('LR', 32)
C_M = (125, 130, _E('CM2', 140), _E('CM3', 150))
NT = int(os.environ.get('NT', 0))
PT = _E('PT', 4)
MB = [int(x) for x in os.environ.get('MB', '1').split(',')]
NCUT = _E('NCUT', 3)
FC = 256


def _pack_rows(m):
    u = np.ascontiguousarray(m, np.float32).view(np.uint32).astype(np.uint64)
    h = ((u + 0x7FFF + ((u >> 16) & 1)) >> 16).astype(np.uint32)
    return h[..., 0::2, :] | (h[..., 1::2, :] << np.uint32(16))


def _dft_tables():
    g = np.concatenate([np.arange(0, P, 2), np.arange(1, P, 2)]).astype(np.float64)
    s = np.arange(P, dtype=np.float64)
    fwd, inv = [], []
    for r in range(R):
        th = 2.0 * np.pi * (g[:, None] + 0.5) * (R * s[None, :] + r) / NFFT
        fwd.append(np.concatenate([np.cos(th), -np.sin(th)], 0))
        inv.append(np.stack([np.cos(th).T, -np.sin(th).T], 2).reshape(P, 2 * P) * (2.0 / NFFT))
    return _pack_rows(np.stack(fwd)), _pack_rows(np.stack(inv))


_FWD, _INV = _dft_tables()
_GC = float(np.sqrt(2.0 / np.pi))
f32, bf16, u32 = jnp.float32, jnp.bfloat16, jnp.uint32


def _layout(nb, nc, F):
    spec = dict(q=(nb * nc, TB // 2), k=(nc, 8 + nb * TB // 2), v=(nb * nc, TB // 2), kt=(nb * nc, TB // 2),
                o=(nb * nc, TB // 2), w1=(nc, F // 2), w2=(nc, F // 2),
                xn=(nb * R * nc, H), xu=(nb * R * nc, H), xk=(nb * R * nc, H),
                u=((nb - 1) * R * nc, 2 * P), kf=((nb - 1) * R * nc, 2 * P), kp=((nb - 1) * R * nc, 2 * P),
                z=(nb * R * nc, P), tick=(1, 8))
    off, out = 0, {}
    for name, (n, rows) in spec.items():
        out[name] = (off, rows)
        off += n * rows
    return out, off


def _lo(w):
    return pltpu.bitcast(w << 16, f32)


def _hi(w):
    return pltpu.bitcast(w & np.uint32(0xFFFF0000), f32)


def _packed(x):
    return pltpu.bitcast(x.astype(bf16), u32)


def _pair(a, b):
    return pltpu.bitcast(pltpu.pack_elementwise([a, b], packed_dtype=bf16), u32)


def _kernel(zero_ref, q_hbm, k_hbm, v_hbm, sk_hbm, w1_hbm, w2_hbm,
            shift_ref, sd_ref, b1_ref, b2_ref, fwd_ref, inv_ref,
            o_hbm,
            arena16, ebuf, fbuf, sbuf, prm, b1s, hbuf, in_sem, w_sem, out_sem, cut_buf, cut_sem, *, nc, nb, D, F):
    lanes = [slice(c * LANES, (c + 1) * LANES) for c in range(nc)]
    lay, total = _layout(nb, nc, F)
    arena = arena16.bitcast(u32)
    zero = pl.multiple_of(zero_ref[0], 8)

    i0 = jnp.zeros((), jnp.int32)

    def rows(start, n):
        return pl.ds(pl.multiple_of(i0 + start, 8), n)

    def late(ref):
        return ref.at[pl.ds(zero, ref.shape[0]), :]

    ordered = late(arena)
    e_ord, f_ord = [late(r) for r in ebuf], [late(r) for r in fbuf]
    E_ROWS, F_ROWS = 2 * R * 2 * P, 2 * R * P

    def at(name, *idx):
        n = 0
        for i in idx[:-1]:
            n = n * R + i
        return lay[name][0] + (n * nc + idx[-1]) * lay[name][1]

    def ld(row, n):
        return pltpu.bitcast(ordered[rows(row, n), :], f32)

    def st(row, val):
        arena[rows(row, val.shape[0]), :] = pltpu.bitcast(val, u32)

    def slab16(row, n):
        return arena16.at[2 * row:2 * (row + n), :]

    def wide(name, *idx):
        return jnp.concatenate([arena[rows(at(name, *idx, c), lay[name][1]), :] for c in range(nc)], axis=1)

    def cols_in(src, b, offs, sem):
        return [pltpu.make_async_copy(src.at[pl.ds(b * TB, TB), lanes[c]], slab16(offs[c], TB // 2), sem)
                for c in range(nc)]

    def conv_in(b):
        return (cols_in(k_hbm, b, [at("k", c) + 8 + b * TB // 2 for c in range(nc)], in_sem.at[0, b])
                + cols_in(v_hbm, b, [at("v", b, c) for c in range(nc)], in_sem.at[1, b])
                + [pltpu.make_async_copy(sk_hbm.at[:, pl.ds(b * TB, TB)], sbuf[b], in_sem.at[2, b])])

    def q_in(b):
        return cols_in(q_hbm, b, [at("q", b, c) for c in range(nc)], in_sem.at[3, b])

    def out_copy(b, c):
        return pltpu.make_async_copy(slab16(at("o", b, c), TB // 2),
                                     o_hbm.at[pl.ds(b * TB, TB), lanes[c]], out_sem.at[b])

    w1_in = [pltpu.make_async_copy(w1_hbm.at[:, lanes[c]], slab16(at("w1", c), F // 2), w_sem.at[0])
             for c in range(nc)]
    w2_in = [pltpu.make_async_copy(w2_hbm.at[:, lanes[c]], slab16(at("w2", c), F // 2), w_sem.at[1])
             for c in range(nc)]

    def start(cs):
        for c in cs:
            c.start()

    def wait(cs):
        for c in cs:
            c.wait()

    def t_unit(b, c):
        slab16(at("kt", b, c), TB // 2)[...] = sbuf[b][lanes[c], :].T

    def prep_unit(b, j, c, s0):
        base = at("k", c) + 8 + b * TB // 2 + j + 2 * s0
        t = ordered[rows(at("k", c), 8), :]
        if PT == 0:
            t = pltpu.roll(t, 1, 1)
        else:
            t = pltpu.bitcast(t, f32)
            for _ in range(PT):
                t = jnp.tanh(t)

        wa = ordered[pl.ds(base - 2, PR, stride=2), :]
        wb = ordered[pl.ds(base - 1, PR, stride=2), :]
        wc = ordered[pl.ds(base, PR, stride=2), :]
        ks = [_hi(wa), _lo(wb), _hi(wb), _lo(wc), _hi(wc)]
        vw = ordered[pl.ds(at("v", b, c) + j + 2 * s0, PR, stride=2), :]
        vs = [_lo(vw), _hi(vw)]
        tw = ordered[pl.ds(at("kt", b, c) + j + 2 * s0, PR, stride=2), :]
        ts = [_lo(tw), _hi(tw)]
        for e in range(2):
            acc = ks[3 + e] * prm[0:1, lanes[c]]
            for i in range(1, 4):
                acc = acc + ks[3 + e - i] * prm[i:i + 1, lanes[c]]
            st(at("xu", b, 2 * j + e, c) + s0 // 2, _packed(acc * vs[e]))
            st(at("xk", b, 2 * j + e, c) + s0 // 2, _packed(ts[e]))
        st(at("tick", 0), t)

    def m_unit(b, g0, c):
        def cld(name, slot, m):
            row = at(name, slot, m, c) + g0
            return ld(row, RG), ld(row + P, RG)

        def cst(name, m, vr, vi):
            row = at(name, b, m, c) + g0
            st(row, vr)
            st(row + P, vi)

        def bfly(which):
            offs = [(which * R + r) * 2 * P + g0 for r in range(R)]
            er = [e_ord[b][rows(o, RG), lanes[c]] for o in offs]
            ei = [e_ord[b][rows(o + P, RG), lanes[c]] for o in offs]
            ar, ai = er[0] + er[2], ei[0] + ei[2]
            br, bi = er[0] - er[2], ei[0] - ei[2]
            cr, ci = er[1] + er[3], ei[1] + ei[3]
            dr, di = er[1] - er[3], ei[1] - ei[3]
            return ([ar + cr, br + di, ar - cr, br - di],
                    [ai + ci, bi - dr, ai - ci, bi + dr])

        tick = pltpu.roll(e_ord[b][rows(g0, RG), lanes[c]], 1, 1)
        ur, ui = bfly(0)
        kr, ki = bfly(1)
        if b == 0:
            kr = [x + prm[4:5, lanes[c]] for x in kr]
        keep = []
        for m in range(R):
            if b == 0:
                keep.append((kr[m], ki[m]))
            else:
                pr, pi = cld("kp", b - 1, m)
                keep.append((kr[m] - pi, ki[m] + pr) if g0 < P // 2 else (kr[m] + pi, ki[m] - pr))
        if b < nb - 1:
            for m in range(R):
                cst("kp", m, kr[m], ki[m])
                cst("u", m, ur[m], ui[m])
                cst("kf", m, *keep[m])
        else:
            st(at("tick", 0), keep[R - 1][1])
        yr, yi = [], []
        for m in range(R):
            accr = acci = None
            for jj in range(b + 1):
                a_r, a_i = (ur[m], ui[m]) if jj == b else cld("u", jj, m)
                b_r, b_i = keep[m] if jj == 0 else cld("kf", b - jj, m)
                pr_ = a_r * b_r - a_i * b_i
                pi_ = a_r * b_i + a_i * b_r
                accr = pr_ if accr is None else accr + pr_
                acci = pi_ if acci is None else acci + pi_
            yr.append(accr)
            yi.append(acci)
            if b >= 2 and m in MB:
                st(at("tick", 0), acci)
        ar, ai = yr[0] + yr[2], yi[0] + yi[2]
        br, bi = yr[0] - yr[2], yi[0] - yi[2]
        cr, ci = yr[1] + yr[3], yi[1] + yi[3]
        dr, di = yr[1] - yr[3], yi[1] - yi[3]
        zr = [ar + cr, br - di, ar - cr, br + di]
        zi = [ai + ci, bi + dr, ai - ci, bi - dr]
        for r in range(R):
            st(at("z", b, r, c) + g0, _pair(zr[r], zi[r]))
        ebuf[b][E_ROWS:E_ROWS + RG, 0:LANES] = tick
        st(at("tick", 0), tick)

    def q_words(src, b, j, c):
        return src[pl.ds(at("q", b, c) + j, P, stride=2), :]

    def ln_rows(src, b, r, s0):
        return jnp.concatenate([(_lo, _hi)[r % 2](src[pl.ds(at("q", b, c) + r // 2 + 2 * s0, LR, stride=2), :])
                                for c in range(nc)], axis=1)

    mean, rstd = {}, {}

    def ln_mean(src, key):
        mean[key] = jnp.mean(ln_rows(src, *key), axis=-1, keepdims=True)

    def ln_rstd(src, key):
        xc = ln_rows(src, *key) - mean[key]
        rstd[key] = jax.lax.rsqrt(jnp.mean(xc * xc, axis=-1, keepdims=True) + 1e-5)

    def ln_store(src, key):
        b, r, s0 = key
        xn = _packed((ln_rows(src, *key) - mean.pop(key)) * rstd.pop(key))
        for c in range(nc):
            st(at("xn", b, r, c) + s0 // 2, xn[:, lanes[c]])

    def ln_unit(src, keys, n):
        for stage, fn in enumerate((ln_mean, ln_rstd, ln_store)):
            if 0 <= n - stage < len(keys):
                fn(src, keys[n - stage])

    def emit_out(src, fsrc, b, j, c, o, tick=None):
        outs = []
        for e in range(2):
            r = 2 * j + e
            xn = pltpu.bitcast(src[rows(at("xn", b, r, c), H), :], bf16).astype(f32)
            outs.append(o[e] + xn * fsrc[(R + r) * P:(R + r + 1) * P, lanes[c]])
        arena[pl.ds(at("o", b, c) + j, P, stride=2), :] = _pair(*outs)
        if tick is not None:
            fbuf[b][F_ROWS:F_ROWS + 8, 0:LANES] = tick
            st(at("tick", 0), tick)
        if j == 1:
            out_copy(b, c).start()

    def fin_unit(b, j, c):
        o = [f_ord[b][(2 * j + e) * P:(2 * j + e + 1) * P, lanes[c]] for e in range(2)]
        tick = pltpu.roll(f_ord[b][0:8, lanes[c]], 1, 1)
        emit_out(ordered, f_ord[b], b, j, c, o, tick)

    queue = []
    credit = [0]

    def fill(cycles):
        credit[0] += cycles
        while queue and credit[0] >= queue[0][2]:
            _, fn, cost = queue.pop(0)
            credit[0] -= cost
            fn()
        if not queue:
            credit[0] = min(credit[0], 128)

    def need(tag):
        while any(t == tag for t, _, _ in queue):
            queue.pop(0)[1]()

    marks = {}
    pieces = []
    cursor = [0]

    def weights(row, n):
        i = cursor[0]
        assert pieces[i][0] == row
        cursor[0] += 1
        for p in range(len(marks), min(i + 1 + LAG, len(pieces))):
            need(pieces[p][1])
            marks[p] = ordered[rows(pieces[p][0], 8), :]
            fill(pieces[p][2])
        return pltpu.bitcast(jnp.concatenate([marks[i], arena[rows(row + 8, n - 8), :]], axis=0), bf16)

    def mm1_op(b, j, s0, s1):
        need(("ln", b, j))
        w = jnp.concatenate([weights(at("w1", c) + s0 // 2, (s1 - s0) // 2) for c in range(nc)], axis=1)
        x = pltpu.bitcast(jnp.concatenate([wide("xn", b, 2 * j), wide("xn", b, 2 * j + 1)], axis=0), bf16)
        h = jax.lax.dot_general(x, w, (((1,), (1,)), ((), ())), preferred_element_type=f32) + b1s[0:1, s0:s1]
        u = h * (h * h * (_GC * 0.044715) + _GC)
        hh = 0.5 * h
        hbuf[b][j][:, s0:s1] = _packed(hh * jnp.tanh(u) + hh)

    def mm2_op(b, j, c, fused):
        w = jnp.concatenate([weights(at("w2", c) + s0 // 2, (min(s0 + FC, F) - s0) // 2)
                             for s0 in range(0, F, FC)], axis=0)
        mlp = jnp.dot(pltpu.bitcast(hbuf[b][j][...], bf16), w, preferred_element_type=f32) + prm[5:6, lanes[c]]
        qw = q_words(arena, b, j, c)
        o = [mlp[0:P] + _lo(qw), mlp[P:2 * P] + _hi(qw)]
        if fused:
            emit_out(arena, fbuf[b], b, j, c, o)
        else:
            for e in range(2):
                fbuf[b][(2 * j + e) * P:(2 * j + e + 1) * P, lanes[c]] = o[e]

    def fwd_op(b, r, src, dst):
        e = jnp.dot(pltpu.bitcast(fwd_ref[r], bf16), jnp.concatenate([weights(at(src, b, r, c), H) for c in range(nc)], axis=1),
                    preferred_element_type=f32)
        ebuf[b][(dst * R + r) * 2 * P:(dst * R + r + 1) * 2 * P, :] = e

    def inv_op(b, r):
        y = jnp.dot(pltpu.bitcast(inv_ref[r], bf16), jnp.concatenate([weights(at("z", b, r, c), P) for c in range(nc)], axis=1),
                    preferred_element_type=f32)
        fbuf[b][(R + r) * P:(R + r + 1) * P, :] = y

    part = functools.partial

    prog = []

    def push(units):
        prog.append(part(queue.extend, units))

    def ln(src, blocks):
        keys = [(b, r, s0) for b in blocks for r in range(R) for s0 in range(0, P, LR)]
        tag = lambda n: ("ln", keys[n][0], keys[n][1] // 2)
        return [(tag(max(n - 2, 0)), part(ln_unit, src, keys, n), C_LN) for n in range(len(keys) + 2)]

    def prep(b):
        units = [(("prep", b, 0), part(t_unit, b, 0), 0)]
        for j in range(2):
            for c in range(nc):
                if j == 0 and c + 1 < nc:
                    units.append((("prep", b, 0), part(t_unit, b, c + 1), 200 if c == 0 else 0))
                units += [(("prep", b, j), part(prep_unit, b, j, c, s0), C_PREP) for s0 in range(0, P, PR)]
        return units

    def spectral(b):
        return [(("m", b), part(m_unit, b, g0, c), C_M[b]) for g0 in range(0, P, RG) for c in range(nc)]

    def fin(b):
        return [(("fin", b), part(fin_unit, b, j, c), C_FIN) for c in range(nc) for j in range(2)]

    def mix(main, extra):
        out = []
        for i, u in enumerate(main):
            out += extra[i * len(extra) // len(main):(i + 1) * len(extra) // len(main)] + [u]
        return out

    def mm1(b, lo=0, hi=None):
        for j, s0 in [(j, s0) for j in range(2) for s0 in range(0, F, FC)][lo:hi]:
            s1 = min(s0 + FC, F)
            pieces.extend((at("w1", c) + s0 // 2, None, 64 * pl.cdiv(s1 - s0, LANES)) for c in range(nc))
            prog.append(part(mm1_op, b, j, s0, s1))

    def mm2(b, lo=0, hi=None, fused=False):
        for c, j in [(c, j) for c in range(nc) for j in range(2)][lo:hi]:
            pieces.extend((at("w2", c) + s0 // 2, None, 128) for s0 in range(0, F, FC))
            prog.append(part(mm2_op, b, j, c, fused))

    def fwd(b):
        for r in range(R):
            for dst, src in enumerate(("xu", "xk")):
                pieces.extend((at(src, b, r, c), ("prep", b, r // 2), 64) for c in range(nc))
                prog.append(part(fwd_op, b, r, src, dst))

    def inv(b):
        for r in range(R):
            pieces.extend((at("z", b, r, c), ("m", b), 64) for c in range(nc))
            prog.append(part(inv_op, b, r))

    def run(then_wait=()):
        for step in prog:
            step()
        prog.clear(), pieces.clear(), marks.clear()
        cursor[0] = 0
        credit[0] = -256
        wait(then_wait)

    first = q_in(0) + w1_in
    second = q_in(1) + q_in(2) + q_in(3)
    third = conv_in(0) + w2_in
    fourth = conv_in(1) + conv_in(2) + conv_in(3)

    cuts = [pltpu.make_async_copy(q_hbm.at[0:16, 0:LANES], cut_buf.at[i], cut_sem.at[i]) for i in range(NCUT)]
    start(first)
    start(cuts)
    for c in range(nc):
        st(at("k", c), jnp.zeros((8, LANES), u32))
    prm[0:4, :] = shift_ref[...].astype(f32)
    prm[4:5, :] = sd_ref[...].astype(f32).reshape(1, D)
    prm[5:6, :] = b2_ref[...].astype(f32).reshape(1, D)
    b1s[...] = b1_ref[...].astype(f32).reshape(1, F)
    wait(first)
    start(second)
    push([(t, f, 0) for t, f, _ in ln(arena, [0])])
    mm1(0, 0, 5)
    run(second)
    start(third)
    push(ln(ordered, [1, 2, 3]))
    mm1(0, 5)
    run(third)
    start(fourth)
    push(prep(0))
    mm1(1, 0, 8)
    fwd(0)
    push(spectral(0))
    mm1(1, 8)
    mm1(2, 0, 9)
    run(fourth)
    push(prep(1) + prep(2) + prep(3))
    mm1(2, 9)
    mm1(3, 0, 2)
    fwd(1)
    mm1(3, 2, 5)
    fwd(2)
    run(cuts[0:1])
    push(spectral(1))
    mm1(3, 5)
    fwd(3)
    push(spectral(2) + spectral(3))
    mm2(0, 0, 4)
    run(cuts[1:2])
    mm2(0, 4)
    inv(0)
    mm2(1, 0, 5)
    run(cuts[2:3])
    mm2(1, 5)
    inv(1)
    push(fin(0) + fin(1))
    mm2(2)
    inv(2)
    push(fin(2))
    inv(3)
    mm2(3, fused=True)
    prog.append(part(need, ("fin", 2)))
    run()
    for b in range(nb):
        wait([out_copy(b, c) for c in range(nc)])


@jax.jit
def pallas_parallel_sum__ssm_conv_h3__dense_activation_gelu__prompt_kernel(
    A_q: jax.Array,
    A_k: jax.Array,
    A_v: jax.Array,
    A_shift_k: jax.Array,
    A_ssm_k: jax.Array,
    A_ssm_D: jax.Array,
    B_x: jax.Array,
    B_w1: jax.Array,
    B_b1: jax.Array,
    B_w2: jax.Array,
    B_b2: jax.Array,
):
    B, S, D = A_q.shape
    F = B_w1.shape[1]
    nc, nb = D // LANES, S // TB
    q, k, v = (a.reshape(S, D) for a in (A_q, A_k, A_v))
    hbm = pl.BlockSpec(memory_space=pltpu.HBM)
    vmem = pl.BlockSpec(memory_space=pltpu.VMEM)
    out = pl.pallas_call(
        functools.partial(_kernel, nc=nc, nb=nb, D=D, F=F),
        in_specs=[pl.BlockSpec(memory_space=pltpu.SMEM)] + [hbm] * 6 + [vmem] * 6,
        out_specs=hbm,
        out_shape=jax.ShapeDtypeStruct((S, D), A_q.dtype),
        scratch_shapes=[
            pltpu.VMEM((2 * _layout(nb, nc, F)[1], LANES), bf16),
            [pltpu.VMEM((2 * R * 2 * P + 8, D), f32) for _ in range(nb)],
            [pltpu.VMEM((2 * R * P + 8, D), f32) for _ in range(nb)],
            [pltpu.VMEM((D, TB), bf16) for _ in range(nb)],
            pltpu.VMEM((8, D), f32),
            pltpu.VMEM((1, F), f32),
            [[pltpu.VMEM((P, F), u32) for _ in range(2)] for _ in range(nb)],
            pltpu.SemaphoreType.DMA((4, nb)),
            pltpu.SemaphoreType.DMA((2,)),
            pltpu.SemaphoreType.DMA((nb,)),
            pltpu.VMEM((NCUT, 16, LANES), bf16),
            pltpu.SemaphoreType.DMA((NCUT,)),
        ],
        compiler_params=pltpu.CompilerParams(vmem_limit_bytes=120 * 1024 * 1024),
    )(jnp.asarray(np.zeros((1,), np.int32)), q, k, v, A_ssm_k, B_w1.T, B_w2, A_shift_k.T, A_ssm_D, B_b1, B_b2,
      jnp.asarray(_FWD), jnp.asarray(_INV))
    return out.reshape(B, S, D)
```

```python
import functools

import numpy as np
import jax
import jax.numpy as jnp
import jax.experimental.pallas as pl
import jax.experimental.pallas.tpu as pltpu

R = 4
P = 128
H = P // 2
TB = R * P
NFFT = 2 * TB
LANES = 128
RG = 8
import os
_E = lambda k, d: int(os.environ.get(k, d))
LAG = int(os.environ.get('LAG', 2))
C_LN, C_PREP, C_FIN = _E('CLN', 135), _E('CP', 100), _E('CF', 135)
PR, LR = _E('PR', 32), _E('LR', 32)
C_M = (125, 130, _E('CM2', 140), _E('CM3', 150))
NT = int(os.environ.get('NT', 0))
PT = _E('PT', 4)
MB = [int(x) for x in os.environ.get('MB', '1').split(',')]
NCUT = _E('NCUT', 3)
FC = 256


def _pack_rows(m):
    u = np.ascontiguousarray(m, np.float32).view(np.uint32).astype(np.uint64)
    h = ((u + 0x7FFF + ((u >> 16) & 1)) >> 16).astype(np.uint32)
    return h[..., 0::2, :] | (h[..., 1::2, :] << np.uint32(16))


def _dft_tables():
    g = np.concatenate([np.arange(0, P, 2), np.arange(1, P, 2)]).astype(np.float64)
    s = np.arange(P, dtype=np.float64)
    fwd, inv = [], []
    for r in range(R):
        th = 2.0 * np.pi * (g[:, None] + 0.5) * (R * s[None, :] + r) / NFFT
        fwd.append(np.concatenate([np.cos(th), -np.sin(th)], 0))
        inv.append(np.stack([np.cos(th).T, -np.sin(th).T], 2).reshape(P, 2 * P) * (2.0 / NFFT))
    return _pack_rows(np.stack(fwd)), _pack_rows(np.stack(inv))


_FWD, _INV = _dft_tables()
_GC = float(np.sqrt(2.0 / np.pi))
f32, bf16, u32 = jnp.float32, jnp.bfloat16, jnp.uint32


def _layout(nb, nc, F):
    spec = dict(q=(nb * nc, TB // 2), k=(nc, 8 + nb * TB // 2), v=(nb * nc, TB // 2), kt=(nb * nc, TB // 2),
                o=(nb * nc, TB // 2), w1=(nc, F // 2), w2=(nc, F // 2),
                xn=(nb * R * nc, H), xu=(nb * R * nc, H), xk=(nb * R * nc, H),
                u=((nb - 1) * R * nc, 2 * P), kf=((nb - 1) * R * nc, 2 * P), kp=((nb - 1) * R * nc, 2 * P),
                z=(nb * R * nc, P), tick=(1, 8))
    off, out = 0, {}
    for name, (n, rows) in spec.items():
        out[name] = (off, rows)
        off += n * rows
    return out, off


def _lo(w):
    return pltpu.bitcast(w << 16, f32)


def _hi(w):
    return pltpu.bitcast(w & np.uint32(0xFFFF0000), f32)


def _packed(x):
    return pltpu.bitcast(x.astype(bf16), u32)


def _pair(a, b):
    return pltpu.bitcast(pltpu.pack_elementwise([a, b], packed_dtype=bf16), u32)


def _kernel(zero_ref, q_hbm, k_hbm, v_hbm, sk_hbm, w1_hbm, w2_hbm,
            shift_hbm, sd_hbm, b1_hbm, b2_hbm, fwd_hbm, inv_hbm,
            o_hbm,
            shift_ref, sd_ref, b1_ref, b2_ref, fwd_ref, inv_ref,
            arena16, ebuf, fbuf, sbuf, prm, b1s, hbuf, in_sem, w_sem, out_sem, cut_buf, cut_sem, *, nc, nb, D, F):
    lanes = [slice(c * LANES, (c + 1) * LANES) for c in range(nc)]
    lay, total = _layout(nb, nc, F)
    arena = arena16.bitcast(u32)
    zero = pl.multiple_of(zero_ref[0], 8)

    i0 = jnp.zeros((), jnp.int32)

    def rows(start, n):
        return pl.ds(pl.multiple_of(i0 + start, 8), n)

    def late(ref):
        return ref.at[pl.ds(zero, ref.shape[0]), :]

    ordered = late(arena)
    e_ord, f_ord = [late(r) for r in ebuf], [late(r) for r in fbuf]
    E_ROWS, F_ROWS = 2 * R * 2 * P, 2 * R * P

    def at(name, *idx):
        n = 0
        for i in idx[:-1]:
            n = n * R + i
        return lay[name][0] + (n * nc + idx[-1]) * lay[name][1]

    def ld(row, n):
        return pltpu.bitcast(ordered[rows(row, n), :], f32)

    def st(row, val):
        arena[rows(row, val.shape[0]), :] = pltpu.bitcast(val, u32)

    def slab16(row, n):
        return arena16.at[2 * row:2 * (row + n), :]

    def wide(name, *idx):
        return jnp.concatenate([arena[rows(at(name, *idx, c), lay[name][1]), :] for c in range(nc)], axis=1)

    def cols_in(src, b, offs, sem):
        return [pltpu.make_async_copy(src.at[pl.ds(b * TB, TB), lanes[c]], slab16(offs[c], TB // 2), sem)
                for c in range(nc)]

    def conv_in(b):
        return (cols_in(k_hbm, b, [at("k", c) + 8 + b * TB // 2 for c in range(nc)], in_sem.at[0, b])
                + cols_in(v_hbm, b, [at("v", b, c) for c in range(nc)], in_sem.at[1, b])
                + [pltpu.make_async_copy(sk_hbm.at[:, pl.ds(b * TB, TB)], sbuf[b], in_sem.at[2, b])])

    def q_in(b):
        return cols_in(q_hbm, b, [at("q", b, c) for c in range(nc)], in_sem.at[3, b])

    def out_copy(b, c):
        return pltpu.make_async_copy(slab16(at("o", b, c), TB // 2),
                                     o_hbm.at[pl.ds(b * TB, TB), lanes[c]], out_sem.at[b])

    def w1_in(lo, hi, n):
        return [pltpu.make_async_copy(w1_hbm.at[lo:hi, lanes[c]], slab16(at("w1", c) + lo // 2, (hi - lo) // 2),
                                      w_sem.at[n]) for c in range(nc)]

    small_in = [pltpu.make_async_copy(src, dst, w_sem.at[3]) for src, dst in (
        (shift_hbm, shift_ref), (sd_hbm, sd_ref), (b1_hbm, b1_ref), (b2_hbm, b2_ref))]
    tables_in = [pltpu.make_async_copy(src, dst, w_sem.at[4]) for src, dst in (
        (fwd_hbm, fwd_ref), (inv_hbm, inv_ref))]
    w2_in = [pltpu.make_async_copy(w2_hbm.at[:, lanes[c]], slab16(at("w2", c), F // 2), w_sem.at[1])
             for c in range(nc)]

    def start(cs):
        for c in cs:
            c.start()

    def wait(cs):
        for c in cs:
            c.wait()

    def t_unit(b, c):
        slab16(at("kt", b, c), TB // 2)[...] = sbuf[b][lanes[c], :].T

    def prep_unit(b, j, c, s0):
        base = at("k", c) + 8 + b * TB // 2 + j + 2 * s0
        t = ordered[rows(at("k", c), 8), :]
        if PT == 0:
            t = pltpu.roll(t, 1, 1)
        else:
            t = pltpu.bitcast(t, f32)
            for _ in range(PT):
                t = jnp.tanh(t)

        wa = ordered[pl.ds(base - 2, PR, stride=2), :]
        wb = ordered[pl.ds(base - 1, PR, stride=2), :]
        wc = ordered[pl.ds(base, PR, stride=2), :]
        ks = [_hi(wa), _lo(wb), _hi(wb), _lo(wc), _hi(wc)]
        vw = ordered[pl.ds(at("v", b, c) + j + 2 * s0, PR, stride=2), :]
        vs = [_lo(vw), _hi(vw)]
        tw = ordered[pl.ds(at("kt", b, c) + j + 2 * s0, PR, stride=2), :]
        ts = [_lo(tw), _hi(tw)]
        for e in range(2):
            acc = ks[3 + e] * prm[0:1, lanes[c]]
            for i in range(1, 4):
                acc = acc + ks[3 + e - i] * prm[i:i + 1, lanes[c]]
            st(at("xu", b, 2 * j + e, c) + s0 // 2, _packed(acc * vs[e]))
            st(at("xk", b, 2 * j + e, c) + s0 // 2, _packed(ts[e]))
        st(at("tick", 0), t)

    def m_unit(b, g0, c):
        def cld(name, slot, m):
            row = at(name, slot, m, c) + g0
            return ld(row, RG), ld(row + P, RG)

        def cst(name, m, vr, vi):
            row = at(name, b, m, c) + g0
            st(row, vr)
            st(row + P, vi)

        def bfly(which):
            offs = [(which * R + r) * 2 * P + g0 for r in range(R)]
            er = [e_ord[b][rows(o, RG), lanes[c]] for o in offs]
            ei = [e_ord[b][rows(o + P, RG), lanes[c]] for o in offs]
            ar, ai = er[0] + er[2], ei[0] + ei[2]
            br, bi = er[0] - er[2], ei[0] - ei[2]
            cr, ci = er[1] + er[3], ei[1] + ei[3]
            dr, di = er[1] - er[3], ei[1] - ei[3]
            return ([ar + cr, br + di, ar - cr, br - di],
                    [ai + ci, bi - dr, ai - ci, bi + dr])

        tick = pltpu.roll(e_ord[b][rows(g0, RG), lanes[c]], 1, 1)
        ur, ui = bfly(0)
        kr, ki = bfly(1)
        if b == 0:
            kr = [x + prm[4:5, lanes[c]] for x in kr]
        keep = []
        for m in range(R):
            if b == 0:
                keep.append((kr[m], ki[m]))
            else:
                pr, pi = cld("kp", b - 1, m)
                keep.append((kr[m] - pi, ki[m] + pr) if g0 < P // 2 else (kr[m] + pi, ki[m] - pr))
        if b < nb - 1:
            for m in range(R):
                cst("kp", m, kr[m], ki[m])
                cst("u", m, ur[m], ui[m])
                cst("kf", m, *keep[m])
        else:
            st(at("tick", 0), keep[R - 1][1])
        yr, yi = [], []
        for m in range(R):
            accr = acci = None
            for jj in range(b + 1):
                a_r, a_i = (ur[m], ui[m]) if jj == b else cld("u", jj, m)
                b_r, b_i = keep[m] if jj == 0 else cld("kf", b - jj, m)
                pr_ = a_r * b_r - a_i * b_i
                pi_ = a_r * b_i + a_i * b_r
                accr = pr_ if accr is None else accr + pr_
                acci = pi_ if acci is None else acci + pi_
            yr.append(accr)
            yi.append(acci)
            if b >= 2 and m in MB:
                st(at("tick", 0), acci)
        ar, ai = yr[0] + yr[2], yi[0] + yi[2]
        br, bi = yr[0] - yr[2], yi[0] - yi[2]
        cr, ci = yr[1] + yr[3], yi[1] + yi[3]
        dr, di = yr[1] - yr[3], yi[1] - yi[3]
        zr = [ar + cr, br - di, ar - cr, br + di]
        zi = [ai + ci, bi + dr, ai - ci, bi - dr]
        for r in range(R):
            st(at("z", b, r, c) + g0, _pair(zr[r], zi[r]))
        ebuf[b][E_ROWS:E_ROWS + RG, 0:LANES] = tick
        st(at("tick", 0), tick)

    def q_words(src, b, j, c):
        return src[pl.ds(at("q", b, c) + j, P, stride=2), :]

    def ln_rows(src, b, r, s0):
        return jnp.concatenate([(_lo, _hi)[r % 2](src[pl.ds(at("q", b, c) + r // 2 + 2 * s0, LR, stride=2), :])
                                for c in range(nc)], axis=1)

    mean, rstd = {}, {}

    def ln_mean(src, key):
        mean[key] = jnp.mean(ln_rows(src, *key), axis=-1, keepdims=True)

    def ln_rstd(src, key):
        xc = ln_rows(src, *key) - mean[key]
        rstd[key] = jax.lax.rsqrt(jnp.mean(xc * xc, axis=-1, keepdims=True) + 1e-5)

    def ln_store(src, key):
        b, r, s0 = key
        xn = _packed((ln_rows(src, *key) - mean.pop(key)) * rstd.pop(key))
        for c in range(nc):
            st(at("xn", b, r, c) + s0 // 2, xn[:, lanes[c]])

    def ln_unit(src, keys, n):
        for stage, fn in enumerate((ln_mean, ln_rstd, ln_store)):
            if 0 <= n - stage < len(keys):
                fn(src, keys[n - stage])

    def emit_out(src, fsrc, b, j, c, o, tick=None):
        outs = []
        for e in range(2):
            r = 2 * j + e
            xn = pltpu.bitcast(src[rows(at("xn", b, r, c), H), :], bf16).astype(f32)
            outs.append(o[e] + xn * fsrc[(R + r) * P:(R + r + 1) * P, lanes[c]])
        arena[pl.ds(at("o", b, c) + j, P, stride=2), :] = _pair(*outs)
        if tick is not None:
            fbuf[b][F_ROWS:F_ROWS + 8, 0:LANES] = tick
            st(at("tick", 0), tick)
        if j == 1:
            out_copy(b, c).start()

    def fin_unit(b, j, c):
        o = [f_ord[b][(2 * j + e) * P:(2 * j + e + 1) * P, lanes[c]] for e in range(2)]
        tick = pltpu.roll(f_ord[b][0:8, lanes[c]], 1, 1)
        emit_out(ordered, f_ord[b], b, j, c, o, tick)

    queue = []
    credit = [0]

    def fill(cycles):
        credit[0] += cycles
        while queue and credit[0] >= queue[0][2]:
            _, fn, cost = queue.pop(0)
            credit[0] -= cost
            fn()
        if not queue:
            credit[0] = min(credit[0], 128)

    def need(tag):
        while any(t == tag for t, _, _ in queue):
            queue.pop(0)[1]()

    marks = {}
    pieces = []
    cursor = [0]

    def weights(row, n):
        i = cursor[0]
        assert pieces[i][0] == row
        cursor[0] += 1
        for p in range(len(marks), min(i + 1 + LAG, len(pieces))):
            need(pieces[p][1])
            marks[p] = ordered[rows(pieces[p][0], 8), :]
            fill(pieces[p][2])
        return pltpu.bitcast(jnp.concatenate([marks[i], arena[rows(row + 8, n - 8), :]], axis=0), bf16)

    def mm1_op(b, j, s0, s1):
        need(("ln", b, j))
        w = jnp.concatenate([weights(at("w1", c) + s0 // 2, (s1 - s0) // 2) for c in range(nc)], axis=1)
        x = pltpu.bitcast(jnp.concatenate([wide("xn", b, 2 * j), wide("xn", b, 2 * j + 1)], axis=0), bf16)
        h = jax.lax.dot_general(x, w, (((1,), (1,)), ((), ())), preferred_element_type=f32) + b1s[0:1, s0:s1]
        u = h * (h * h * (_GC * 0.044715) + _GC)
        hh = 0.5 * h
        hbuf[b][j][:, s0:s1] = _packed(hh * jnp.tanh(u) + hh)

    def mm2_op(b, j, c, fused):
        w = jnp.concatenate([weights(at("w2", c) + s0 // 2, (min(s0 + FC, F) - s0) // 2)
                             for s0 in range(0, F, FC)], axis=0)
        mlp = jnp.dot(pltpu.bitcast(hbuf[b][j][...], bf16), w, preferred_element_type=f32) + prm[5:6, lanes[c]]
        qw = q_words(arena, b, j, c)
        o = [mlp[0:P] + _lo(qw), mlp[P:2 * P] + _hi(qw)]
        if fused:
            emit_out(arena, fbuf[b], b, j, c, o)
        else:
            for e in range(2):
                fbuf[b][(2 * j + e) * P:(2 * j + e + 1) * P, lanes[c]] = o[e]

    def fwd_op(b, r, src, dst):
        e = jnp.dot(pltpu.bitcast(fwd_ref[r], bf16), jnp.concatenate([weights(at(src, b, r, c), H) for c in range(nc)], axis=1),
                    preferred_element_type=f32)
        ebuf[b][(dst * R + r) * 2 * P:(dst * R + r + 1) * 2 * P, :] = e

    def inv_op(b, r):
        y = jnp.dot(pltpu.bitcast(inv_ref[r], bf16), jnp.concatenate([weights(at("z", b, r, c), P) for c in range(nc)], axis=1),
                    preferred_element_type=f32)
        fbuf[b][(R + r) * P:(R + r + 1) * P, :] = y

    part = functools.partial

    prog = []

    def push(units):
        prog.append(part(queue.extend, units))

    def ln(src, blocks):
        keys = [(b, r, s0) for b in blocks for r in range(R) for s0 in range(0, P, LR)]
        tag = lambda n: ("ln", keys[n][0], keys[n][1] // 2)
        return [(tag(max(n - 2, 0)), part(ln_unit, src, keys, n), C_LN) for n in range(len(keys) + 2)]

    def prep(b):
        units = [(("prep", b, 0), part(t_unit, b, 0), 0)]
        for j in range(2):
            for c in range(nc):
                if j == 0 and c + 1 < nc:
                    units.append((("prep", b, 0), part(t_unit, b, c + 1), 200 if c == 0 else 0))
                units += [(("prep", b, j), part(prep_unit, b, j, c, s0), C_PREP) for s0 in range(0, P, PR)]
        return units

    def spectral(b):
        return [(("m", b), part(m_unit, b, g0, c), C_M[b]) for g0 in range(0, P, RG) for c in range(nc)]

    def fin(b):
        return [(("fin", b), part(fin_unit, b, j, c), C_FIN) for c in range(nc) for j in range(2)]

    def mix(main, extra):
        out = []
        for i, u in enumerate(main):
            out += extra[i * len(extra) // len(main):(i + 1) * len(extra) // len(main)] + [u]
        return out

    def mm1(b, lo=0, hi=None):
        for s0, j in [(s0, j) for s0 in range(0, F, FC) for j in range(2)][lo:hi]:
            s1 = min(s0 + FC, F)
            pieces.extend((at("w1", c) + s0 // 2, None, 64 * pl.cdiv(s1 - s0, LANES)) for c in range(nc))
            prog.append(part(mm1_op, b, j, s0, s1))

    def mm2(b, lo=0, hi=None, fused=False):
        for c, j in [(c, j) for c in range(nc) for j in range(2)][lo:hi]:
            pieces.extend((at("w2", c) + s0 // 2, None, 128) for s0 in range(0, F, FC))
            prog.append(part(mm2_op, b, j, c, fused))

    def fwd(b):
        for r in range(R):
            for dst, src in enumerate(("xu", "xk")):
                pieces.extend((at(src, b, r, c), ("prep", b, r // 2), 64) for c in range(nc))
                prog.append(part(fwd_op, b, r, src, dst))

    def inv(b):
        for r in range(R):
            pieces.extend((at("z", b, r, c), ("m", b), 64) for c in range(nc))
            prog.append(part(inv_op, b, r))

    def run(then_wait=()):
        for step in prog:
            step()
        prog.clear(), pieces.clear(), marks.clear()
        cursor[0] = 0
        credit[0] = -256
        wait(then_wait)

    WA = 3 * FC
    feed = [q_in(0), w1_in(0, WA, 0) + small_in, w1_in(WA, F, 2) + q_in(1), q_in(2) + q_in(3),
            conv_in(0) + tables_in, conv_in(1) + conv_in(2) + conv_in(3) + w2_in]
    cuts = [pltpu.make_async_copy(q_hbm.at[0:16, 0:LANES], cut_buf.at[i], cut_sem.at[i]) for i in range(NCUT)]

    def params():
        prm[0:4, :] = shift_ref[...].astype(f32)
        prm[4:5, :] = sd_ref[...].astype(f32).reshape(1, D)
        prm[5:6, :] = b2_ref[...].astype(f32).reshape(1, D)
        b1s[...] = b1_ref[...].astype(f32).reshape(1, F)

    start(feed[0] + feed[1])
    for c in range(nc): st(at("k", c), jnp.zeros((8, LANES), u32))
    wait(feed[0])
    start(feed[2])
    push(ln(arena, [0]))
    prog.append(part(need, ("ln", 0, 1)))
    run(feed[1])
    start(feed[3])
    params()
    mm1(0, 0, 6)
    run(feed[2])
    start(feed[4] + cuts)
    push(ln(ordered, [1]))
    mm1(0, 6, 10)
    run(feed[3])
    start(feed[5])
    push(ln(ordered, [2, 3]))
    mm1(0, 10)
    mm1(1, 0, 4)
    run(feed[4])
    push(prep(0))
    mm1(1, 4, 12)
    fwd(0)
    push(spectral(0))
    mm1(1, 12)
    mm1(2)
    run(feed[5])
    push(prep(1) + prep(2) + prep(3))
    mm1(3, 0, 7)
    fwd(1)
    mm1(3, 7)
    run(cuts[0:1])
    push(spectral(1) + spectral(2) + spectral(3))
    fwd(2)
    fwd(3)
    mm2(0, 0, 7)
    run(cuts[1:2])
    mm2(0, 7)
    inv(0)
    mm2(1, 0, 8)
    run(cuts[2:3])
    push(fin(0) + fin(1))
    mm2(1, 8)
    inv(1)
    mm2(2)
    inv(2)
    push(fin(2))
    inv(3)
    mm2(3, fused=True)
    prog.append(part(need, ("fin", 2)))
    run()
    for b in range(nb):
        wait([out_copy(b, c) for c in range(nc)])


@jax.jit
def pallas_parallel_sum__ssm_conv_h3__dense_activation_gelu__prompt_kernel(
    A_q: jax.Array,
    A_k: jax.Array,
    A_v: jax.Array,
    A_shift_k: jax.Array,
    A_ssm_k: jax.Array,
    A_ssm_D: jax.Array,
    B_x: jax.Array,
    B_w1: jax.Array,
    B_b1: jax.Array,
    B_w2: jax.Array,
    B_b2: jax.Array,
):
    B, S, D = A_q.shape
    F = B_w1.shape[1]
    nc, nb = D // LANES, S // TB
    q, k, v = (a.reshape(S, D) for a in (A_q, A_k, A_v))
    hbm = pl.BlockSpec(memory_space=pltpu.HBM)
    out = pl.pallas_call(
        functools.partial(_kernel, nc=nc, nb=nb, D=D, F=F),
        in_specs=[pl.BlockSpec(memory_space=pltpu.SMEM)] + [hbm] * 12,
        out_specs=hbm,
        out_shape=jax.ShapeDtypeStruct((S, D), A_q.dtype),
        scratch_shapes=[
            pltpu.VMEM((4, D), bf16), pltpu.VMEM((D,), bf16), pltpu.VMEM((F,), bf16), pltpu.VMEM((D,), bf16),
            pltpu.VMEM(_FWD.shape, u32), pltpu.VMEM(_INV.shape, u32),
            pltpu.VMEM((2 * _layout(nb, nc, F)[1], LANES), bf16),
            [pltpu.VMEM((2 * R * 2 * P + 8, D), f32) for _ in range(nb)],
            [pltpu.VMEM((2 * R * P + 8, D), f32) for _ in range(nb)],
            [pltpu.VMEM((D, TB), bf16) for _ in range(nb)],
            pltpu.VMEM((8, D), f32),
            pltpu.VMEM((1, F), f32),
            [[pltpu.VMEM((P, F), u32) for _ in range(2)] for _ in range(nb)],
            pltpu.SemaphoreType.DMA((4, nb)),
            pltpu.SemaphoreType.DMA((5,)),
            pltpu.SemaphoreType.DMA((nb,)),
            pltpu.VMEM((NCUT, 16, LANES), bf16),
            pltpu.SemaphoreType.DMA((NCUT,)),
        ],
        compiler_params=pltpu.CompilerParams(vmem_limit_bytes=120 * 1024 * 1024),
    )(jnp.asarray(np.zeros((1,), np.int32)), q, k, v, A_ssm_k, B_w1.T, B_w2, A_shift_k.T, A_ssm_D, B_b1, B_b2,
      jnp.asarray(_FWD), jnp.asarray(_INV))
    return out.reshape(B, S, D)
```

```python
import functools

import numpy as np
import jax
import jax.numpy as jnp
import jax.experimental.pallas as pl
import jax.experimental.pallas.tpu as pltpu

R = 4
P = 128
H = P // 2
TB = R * P
NFFT = 2 * TB
LANES = 128
RG = 8
import os
_E = lambda k, d: int(os.environ.get(k, d))
LAG = int(os.environ.get('LAG', 2))
C_LN, C_PREP, C_FIN = _E('CLN', 135), _E('CP', 115), _E('CF', 135)
PR, LR = _E('PR', 32), _E('LR', 32)
C_M = (_E('CM0', 120), _E('CM1', 125), _E('CM2', 125), _E('CM3', 130))
NT = int(os.environ.get('NT', 0))
PT = _E('PT', 7)
MB = [int(x) for x in os.environ.get('MB', '1').split(',')]
NCUT = _E('NCUT', 2)
M128, KP = _E('M128', 0), _E('KP', 256)
TL = _E('TL', 2)
FC = 256


def _pack_rows(m):
    u = np.ascontiguousarray(m, np.float32).view(np.uint32).astype(np.uint64)
    h = ((u + 0x7FFF + ((u >> 16) & 1)) >> 16).astype(np.uint32)
    return h[..., 0::2, :] | (h[..., 1::2, :] << np.uint32(16))


def _dft_tables():
    g = np.concatenate([np.arange(0, P, 2), np.arange(1, P, 2)]).astype(np.float64)
    s = np.arange(P, dtype=np.float64)
    fwd, inv = [], []
    for r in range(R):
        th = 2.0 * np.pi * (g[:, None] + 0.5) * (R * s[None, :] + r) / NFFT
        fwd.append(np.concatenate([np.cos(th), -np.sin(th)], 0))
        inv.append(np.stack([np.cos(th).T, -np.sin(th).T], 2).reshape(P, 2 * P) * (2.0 / NFFT))
    return _pack_rows(np.stack(fwd)), _pack_rows(np.stack(inv))


_FWD, _INV = _dft_tables()
_GC = float(np.sqrt(2.0 / np.pi))
f32, bf16, u32 = jnp.float32, jnp.bfloat16, jnp.uint32


def _layout(nb, nc, F):
    spec = dict(q=(nb * nc, TB // 2), k=(nc, 8 + nb * TB // 2), v=(nb * nc, TB // 2), kt=(nb * nc, TB // 2),
                sk=(nb * R * nc, H),
                o=(nb * nc, TB // 2), w1=(nc, F // 2), w2=(nc, F // 2),
                xn=(nb * R * nc, H), xu=(nb * R * nc, H), xk=(nb * R * nc, H),
                u=((nb - 1) * R * nc, 2 * P), kf=((nb - 1) * R * nc, 2 * P), kp=((nb - 1) * R * nc, 2 * P),
                z=(nb * R * nc, P), tick=(1, 8))
    off, out = 0, {}
    for name, (n, rows) in spec.items():
        out[name] = (off, rows)
        off += n * rows
    return out, off


def _lo(w):
    return pltpu.bitcast(w << 16, f32)


def _hi(w):
    return pltpu.bitcast(w & np.uint32(0xFFFF0000), f32)


def _packed(x):
    return pltpu.bitcast(x.astype(bf16), u32)


def _pair(a, b):
    return pltpu.bitcast(pltpu.pack_elementwise([a, b], packed_dtype=bf16), u32)


def _kernel(zero_ref, q_hbm, k_hbm, v_hbm, sk_hbm, w1_hbm, w2_hbm,
            shift_hbm, sd_hbm, b1_hbm, b2_hbm, fwd_hbm, inv_hbm,
            o_hbm,
            shift_ref, sd_ref, b1_ref, b2_ref, fwd_ref, inv_ref,
            arena16, ebuf, fbuf, prm, b1s, hbuf, in_sem, w_sem, out_sem, cut_buf, cut_sem, *, nc, nb, D, F):
    lanes = [slice(c * LANES, (c + 1) * LANES) for c in range(nc)]
    lay, total = _layout(nb, nc, F)
    arena = arena16.bitcast(u32)
    zero = pl.multiple_of(zero_ref[0], 8)

    i0 = jnp.zeros((), jnp.int32)

    def rows(start, n):
        return pl.ds(pl.multiple_of(i0 + start, 8), n)

    def late(ref):
        return ref.at[pl.ds(zero, ref.shape[0]), :]

    ordered = late(arena)
    e_ord, f_ord = [late(r) for r in ebuf], [late(r) for r in fbuf]
    E_ROWS, F_ROWS = 2 * R * 2 * P, 2 * R * P

    def at(name, *idx):
        n = 0
        for i in idx[:-1]:
            n = n * R + i
        return lay[name][0] + (n * nc + idx[-1]) * lay[name][1]

    def ld(row, n):
        return pltpu.bitcast(ordered[rows(row, n), :], f32)

    def st(row, val):
        arena[rows(row, val.shape[0]), :] = pltpu.bitcast(val, u32)

    def slab16(row, n):
        return arena16.at[2 * row:2 * (row + n), :]

    def wide(name, *idx):
        return jnp.concatenate([arena[rows(at(name, *idx, c), lay[name][1]), :] for c in range(nc)], axis=1)

    def cols_in(src, b, offs, sem):
        return [pltpu.make_async_copy(src.at[pl.ds(b * TB, TB), lanes[c]], slab16(offs[c], TB // 2), sem)
                for c in range(nc)]

    def conv_in(b):
        return (cols_in(k_hbm, b, [at("k", c) + 8 + b * TB // 2 for c in range(nc)], in_sem.at[0, b])
                + cols_in(v_hbm, b, [at("v", b, c) for c in range(nc)], in_sem.at[1, b])
                + [pltpu.make_async_copy(sk_hbm.at[lanes[c], pl.ds(b * TB + n * P, P)],
                                         slab16(at("sk", b, n, c), H), in_sem.at[2, b])
                   for c in range(nc) for n in range(R)])

    def q_in(b):
        return cols_in(q_hbm, b, [at("q", b, c) for c in range(nc)], in_sem.at[3, b])

    def out_copy(b, c):
        return pltpu.make_async_copy(slab16(at("o", b, c), TB // 2),
                                     o_hbm.at[pl.ds(b * TB, TB), lanes[c]], out_sem.at[b])

    def w1_in(lo, hi, n):
        return [pltpu.make_async_copy(w1_hbm.at[lo:hi, lanes[c]], slab16(at("w1", c) + lo // 2, (hi - lo) // 2),
                                      w_sem.at[n]) for c in range(nc)]

    small_in = [pltpu.make_async_copy(src, dst, w_sem.at[3]) for src, dst in (
        (shift_hbm, shift_ref), (sd_hbm, sd_ref), (b1_hbm, b1_ref), (b2_hbm, b2_ref))]
    tables_in = [pltpu.make_async_copy(fwd_hbm, fwd_ref, w_sem.at[4]),
                 pltpu.make_async_copy(inv_hbm, inv_ref, w_sem.at[5])]
    w2_in = [pltpu.make_async_copy(w2_hbm.at[:, lanes[c]], slab16(at("w2", c), F // 2), w_sem.at[1])
             for c in range(nc)]

    def start(cs):
        for c in cs:
            c.start()

    def wait(cs):
        for c in cs:
            c.wait()

    tiles = {}

    def t_load(b, c, n):
        w = pltpu.bitcast(ordered[rows(at("sk", b, n, c), H), :], bf16)
        tiles[b, c, n] = pltpu.bitcast(w.T, u32)

    def t_store(b, c, n):
        st(at("kt", b, c) + n * H, tiles.pop((b, c, n)))

    def prep_unit(b, j, c, s0):
        base = at("k", c) + 8 + b * TB // 2 + j + 2 * s0
        t = ordered[rows(at("k", c), 8), :]
        if PT == 0:
            t = pltpu.roll(t, 1, 1)
        else:
            t = pltpu.bitcast(t, f32)
            for _ in range(PT):
                t = jnp.tanh(t)

        wa = ordered[pl.ds(base - 2, PR, stride=2), :]
        wb = ordered[pl.ds(base - 1, PR, stride=2), :]
        wc = ordered[pl.ds(base, PR, stride=2), :]
        ks = [_hi(wa), _lo(wb), _hi(wb), _lo(wc), _hi(wc)]
        vw = ordered[pl.ds(at("v", b, c) + j + 2 * s0, PR, stride=2), :]
        vs = [_lo(vw), _hi(vw)]
        tw = ordered[pl.ds(at("kt", b, c) + j + 2 * s0, PR, stride=2), :]
        ts = [_lo(tw), _hi(tw)]
        for e in range(2):
            acc = ks[3 + e] * prm[0:1, lanes[c]]
            for i in range(1, 4):
                acc = acc + ks[3 + e - i] * prm[i:i + 1, lanes[c]]
            st(at("xu", b, 2 * j + e, c) + s0 // 2, _packed(acc * vs[e]))
            st(at("xk", b, 2 * j + e, c) + s0 // 2, _packed(ts[e]))
        st(at("tick", 0), t)

    def m_unit(b, g0, c):
        def cld(name, slot, m):
            row = at(name, slot, m, c) + g0
            return ld(row, RG), ld(row + P, RG)

        def cst(name, m, vr, vi):
            row = at(name, b, m, c) + g0
            st(row, vr)
            st(row + P, vi)

        def bfly(which):
            offs = [(which * R + r) * 2 * P + g0 for r in range(R)]
            er = [e_ord[b][rows(o, RG), lanes[c]] for o in offs]
            ei = [e_ord[b][rows(o + P, RG), lanes[c]] for o in offs]
            ar, ai = er[0] + er[2], ei[0] + ei[2]
            br, bi = er[0] - er[2], ei[0] - ei[2]
            cr, ci = er[1] + er[3], ei[1] + ei[3]
            dr, di = er[1] - er[3], ei[1] - ei[3]
            return ([ar + cr, br + di, ar - cr, br - di],
                    [ai + ci, bi - dr, ai - ci, bi + dr])

        tick = pltpu.roll(e_ord[b][rows(g0, RG), lanes[c]], 1, 1)
        ur, ui = bfly(0)
        kr, ki = bfly(1)
        if b == 0:
            kr = [x + prm[4:5, lanes[c]] for x in kr]
        keep = []
        for m in range(R):
            if b == 0:
                keep.append((kr[m], ki[m]))
            else:
                pr, pi = cld("kp", b - 1, m)
                keep.append((kr[m] - pi, ki[m] + pr) if g0 < P // 2 else (kr[m] + pi, ki[m] - pr))
        if b < nb - 1:
            for m in range(R):
                cst("kp", m, kr[m], ki[m])
                cst("u", m, ur[m], ui[m])
                cst("kf", m, *keep[m])
        else:
            st(at("tick", 0), keep[R - 1][1])
        yr, yi = [], []
        for m in range(R):
            accr = acci = None
            for jj in range(b + 1):
                a_r, a_i = (ur[m], ui[m]) if jj == b else cld("u", jj, m)
                b_r, b_i = keep[m] if jj == 0 else cld("kf", b - jj, m)
                pr_ = a_r * b_r - a_i * b_i
                pi_ = a_r * b_i + a_i * b_r
                accr = pr_ if accr is None else accr + pr_
                acci = pi_ if acci is None else acci + pi_
            yr.append(accr)
            yi.append(acci)
            if b >= 2 and m in MB:
                st(at("tick", 0), acci)
        ar, ai = yr[0] + yr[2], yi[0] + yi[2]
        br, bi = yr[0] - yr[2], yi[0] - yi[2]
        cr, ci = yr[1] + yr[3], yi[1] + yi[3]
        dr, di = yr[1] - yr[3], yi[1] - yi[3]
        zr = [ar + cr, br - di, ar - cr, br + di]
        zi = [ai + ci, bi + dr, ai - ci, bi - dr]
        for r in range(R):
            st(at("z", b, r, c) + g0, _pair(zr[r], zi[r]))
        ebuf[b][E_ROWS:E_ROWS + RG, 0:LANES] = tick
        st(at("tick", 0), tick)

    def q_words(src, b, j, c):
        return src[pl.ds(at("q", b, c) + j, P, stride=2), :]

    def ln_rows(src, b, r, s0):
        return jnp.concatenate([(_lo, _hi)[r % 2](src[pl.ds(at("q", b, c) + r // 2 + 2 * s0, LR, stride=2), :])
                                for c in range(nc)], axis=1)

    mean, rstd = {}, {}

    def ln_mean(src, key):
        mean[key] = jnp.mean(ln_rows(src, *key), axis=-1, keepdims=True)

    def ln_rstd(src, key):
        xc = ln_rows(src, *key) - mean[key]
        rstd[key] = jax.lax.rsqrt(jnp.mean(xc * xc, axis=-1, keepdims=True) + 1e-5)

    def ln_store(src, key):
        b, r, s0 = key
        xn = _packed((ln_rows(src, *key) - mean.pop(key)) * rstd.pop(key))
        for c in range(nc):
            st(at("xn", b, r, c) + s0 // 2, xn[:, lanes[c]])

    def ln_unit(src, keys, n):
        for stage, fn in enumerate((ln_mean, ln_rstd, ln_store)):
            if 0 <= n - stage < len(keys):
                fn(src, keys[n - stage])

    def emit_out(src, fsrc, b, j, c, o, tick=None):
        outs = []
        for e in range(2):
            r = 2 * j + e
            xn = pltpu.bitcast(src[rows(at("xn", b, r, c), H), :], bf16).astype(f32)
            outs.append(o[e] + xn * fsrc[(R + r) * P:(R + r + 1) * P, lanes[c]])
        arena[pl.ds(at("o", b, c) + j, P, stride=2), :] = _pair(*outs)
        if tick is not None:
            fbuf[b][F_ROWS:F_ROWS + 8, 0:LANES] = tick
            st(at("tick", 0), tick)
        if j == 1:
            out_copy(b, c).start()

    def fin_gate(b):
        fbuf[b][F_ROWS:F_ROWS + 8, 0:LANES] = ld(at("k", 0), 8)

    def fin_unit(b, j, c):
        o = [f_ord[b][(2 * j + e) * P:(2 * j + e + 1) * P, lanes[c]] for e in range(2)]
        tick = pltpu.roll(f_ord[b][0:8, lanes[c]], 1, 1)
        emit_out(ordered, f_ord[b], b, j, c, o, tick)

    queue = []
    credit = [0]

    def fill(cycles):
        credit[0] += cycles
        while queue and credit[0] >= queue[0][2]:
            _, fn, cost = queue.pop(0)
            credit[0] -= cost
            fn()
        if not queue:
            credit[0] = min(credit[0], 128)

    def need(tag):
        while any(t == tag for t, _, _ in queue):
            queue.pop(0)[1]()

    marks = {}
    pieces = []
    cursor = [0]

    def weights(row, n):
        i = cursor[0]
        assert pieces[i][0] == row
        cursor[0] += 1
        for p in range(len(marks), min(i + 1 + LAG, len(pieces))):
            need(pieces[p][1])
            marks[p] = ordered[rows(pieces[p][0], 8), :]
            fill(pieces[p][2])
        return pltpu.bitcast(jnp.concatenate([marks[i], arena[rows(row + 8, n - 8), :]], axis=0), bf16)

    def mm1_op(b, j, s0, s1):
        need(("ln", b, j))
        w = jnp.concatenate([weights(at("w1", c) + s0 // 2, (s1 - s0) // 2) for c in range(nc)], axis=1)
        x = pltpu.bitcast(jnp.concatenate([wide("xn", b, 2 * j), wide("xn", b, 2 * j + 1)], axis=0), bf16)
        h = jax.lax.dot_general(x, w, (((1,), (1,)), ((), ())), preferred_element_type=f32) + b1s[0:1, s0:s1]
        u = h * (h * h * (_GC * 0.044715) + _GC)
        hh = 0.5 * h
        hbuf[b][j][:, s0:s1] = _packed(hh * jnp.tanh(u) + hh)

    def mm2_op(b, j, c, fused):
        def w():
            return jnp.concatenate([weights(at("w2", c) + s0 // 2, (min(s0 + KP, F) - s0) // 2)
                                    for s0 in range(0, F, KP)], axis=0)
        if M128:
            mlp = [jnp.dot(pltpu.bitcast(hbuf[b][j][e * H:(e + 1) * H, :], bf16), w(), preferred_element_type=f32)
                   for e in range(2)]
        else:
            mlp = jnp.dot(pltpu.bitcast(hbuf[b][j][...], bf16), w(), preferred_element_type=f32)
            mlp = [mlp[0:P], mlp[P:2 * P]]
        qw = q_words(arena, b, j, c)
        o = [mlp[0] + prm[5:6, lanes[c]] + _lo(qw), mlp[1] + prm[5:6, lanes[c]] + _hi(qw)]
        if fused:
            emit_out(arena, fbuf[b], b, j, c, o)
        else:
            for e in range(2):
                fbuf[b][(2 * j + e) * P:(2 * j + e + 1) * P, lanes[c]] = o[e]

    def fwd_op(b, r, src, dst):
        e = jnp.dot(pltpu.bitcast(fwd_ref[r], bf16), jnp.concatenate([weights(at(src, b, r, c), H) for c in range(nc)], axis=1),
                    preferred_element_type=f32)
        ebuf[b][(dst * R + r) * 2 * P:(dst * R + r + 1) * 2 * P, :] = e

    def inv_op(b, r):
        y = jnp.dot(pltpu.bitcast(inv_ref[r], bf16), jnp.concatenate([weights(at("z", b, r, c), P) for c in range(nc)], axis=1),
                    preferred_element_type=f32)
        fbuf[b][(R + r) * P:(R + r + 1) * P, :] = y

    part = functools.partial

    prog = []

    def push(units):
        prog.append(part(queue.extend, units))

    def ln(src, blocks, cost=C_LN):
        keys = [(b, r, s0) for b in blocks for r in range(R) for s0 in range(0, P, LR)]
        tag = lambda n: ("ln", keys[n][0], keys[n][1] // 2)
        return [(tag(max(n - 2, 0)), part(ln_unit, src, keys, n), cost) for n in range(len(keys) + 2)]

    def prep(blocks):
        ts = [(b, c, n) for b in blocks for c in range(nc) for n in range(R)]
        out = []
        for i in range(-TL - 1, len(ts)):
            tag = ("prep", ts[max(i, 0)][0])
            if i + TL + 1 < len(ts):
                out.append((tag, part(t_load, *ts[i + TL + 1]), 0))
            for j in range(2):
                if j == 1 and -1 <= i < len(ts) - 1:
                    out.append((tag, part(t_store, *ts[i + 1]), 0))
                if i >= 0:
                    out.append((tag, part(prep_unit, ts[i][0], j, ts[i][1], ts[i][2] * PR), C_PREP))
                else:
                    out.append((tag, lambda: None, C_PREP))
        return out

    def spectral(b):
        return [(("m", b), part(m_unit, b, g0, c), C_M[b]) for g0 in range(0, P, RG) for c in range(nc)]

    def fin(b, n=nc):
        return [(("fin", b), part(fin_gate, b), 0)] + [
            (("fin", b), part(fin_unit, b, j, c), C_FIN) for c in range(n) for j in range(2)]

    def mix(main, extra):
        out = []
        for i, u in enumerate(main):
            out += extra[i * len(extra) // len(main):(i + 1) * len(extra) // len(main)] + [u]
        return out

    def mm1(b, lo=0, hi=None):
        for s0, j in [(s0, j) for s0 in range(0, F, FC) for j in range(2)][lo:hi]:
            s1 = min(s0 + FC, F)
            pieces.extend((at("w1", c) + s0 // 2, None, 64 * pl.cdiv(s1 - s0, LANES)) for c in range(nc))
            prog.append(part(mm1_op, b, j, s0, s1))

    def mm2(b, lo=0, hi=None, fused=False):
        for c, j in [(c, j) for c in range(nc) for j in range(2)][lo:hi]:
            pieces.extend((at("w2", c) + s0 // 2, None, pl.cdiv(min(KP, F - s0), LANES) * (32 if M128 else 64))
                          for _ in range(1 + M128) for s0 in range(0, F, KP))
            prog.append(part(mm2_op, b, j, c, fused))

    def fwd(b):
        for r in range(R):
            for dst, src in enumerate(("xu", "xk")):
                pieces.extend((at(src, b, r, c), ("prep", b), 64) for c in range(nc))
                prog.append(part(fwd_op, b, r, src, dst))

    def inv(b):
        for r in range(R):
            pieces.extend((at("z", b, r, c), ("m", b), 64) for c in range(nc))
            prog.append(part(inv_op, b, r))

    def run(then_wait=()):
        for step in prog:
            step()
        prog.clear(), pieces.clear(), marks.clear()
        cursor[0] = 0
        credit[0] = -256
        wait(then_wait)

    feed = [q_in(0), w1_in(0, 4 * FC, 0) + small_in, w1_in(4 * FC, F, 2) + q_in(1),
            q_in(2) + conv_in(0) + tables_in[:1], w2_in + conv_in(1) + q_in(3) + tables_in[1:],
            conv_in(2) + conv_in(3)]
    cuts = [pltpu.make_async_copy(q_hbm.at[0:16, 0:LANES], cut_buf.at[i], cut_sem.at[i]) for i in range(NCUT)]

    def params():
        prm[0:4, :] = shift_ref[...].astype(f32)
        prm[4:5, :] = sd_ref[...].astype(f32).reshape(1, D)
        prm[5:6, :] = b2_ref[...].astype(f32).reshape(1, D)
        b1s[...] = b1_ref[...].astype(f32).reshape(1, F)

    start(feed[0] + feed[1])
    for c in range(nc): st(at("k", c), jnp.zeros((8, LANES), u32))
    wait(feed[0])
    push(ln(arena, [0]))
    prog.append(part(need, ("ln", 0, 1)))
    run(feed[1])
    start(feed[2] + cuts)
    params()
    mm1(0, 0, 8)
    run(feed[2])
    start(feed[3])
    push(ln(ordered, [1], 160))
    mm1(0, 8)
    mm1(1, 0, 4)
    run(feed[3])
    start(feed[4])
    push(prep([0]))
    mm1(1, 4)
    push(ln(ordered, [2]))
    fwd(0)
    push(spectral(0))
    mm1(2)
    run(feed[4])
    start(feed[5])
    push(prep([1]))
    mm2(0, 0, 6)
    push(ln(ordered, [3]))
    fwd(1)
    push(spectral(1))
    mm1(3)
    mm2(0, 6, 8)
    run(feed[5])
    push(prep([2, 3]))
    mm2(0, 8)
    inv(0)
    mm2(1, 0, 3)
    fwd(2)
    mm2(1, 3, 5)
    run(cuts[0:1])
    push(spectral(2))
    fwd(3)
    mm2(1, 5)
    inv(1)
    mm2(2, 0, 2)
    run(cuts[1:2])
    push(spectral(3))
    mm2(2, 2)
    inv(2)
    mm2(3, 0, 2)
    inv(3)
    push(fin(0) + fin(1) + fin(2) + fin(3, 1))
    mm2(3, 2, fused=True)
    prog.append(part(need, ("fin", 3)))
    run()
    for b in range(nb):
        wait([out_copy(b, c) for c in range(nc)])


@jax.jit
def pallas_parallel_sum__ssm_conv_h3__dense_activation_gelu__prompt_kernel(
    A_q: jax.Array,
    A_k: jax.Array,
    A_v: jax.Array,
    A_shift_k: jax.Array,
    A_ssm_k: jax.Array,
    A_ssm_D: jax.Array,
    B_x: jax.Array,
    B_w1: jax.Array,
    B_b1: jax.Array,
    B_w2: jax.Array,
    B_b2: jax.Array,
):
    B, S, D = A_q.shape
    F = B_w1.shape[1]
    nc, nb = D // LANES, S // TB
    q, k, v = (a.reshape(S, D) for a in (A_q, A_k, A_v))
    hbm = pl.BlockSpec(memory_space=pltpu.HBM)
    out = pl.pallas_call(
        functools.partial(_kernel, nc=nc, nb=nb, D=D, F=F),
        in_specs=[pl.BlockSpec(memory_space=pltpu.SMEM)] + [hbm] * 12,
        out_specs=hbm,
        out_shape=jax.ShapeDtypeStruct((S, D), A_q.dtype),
        scratch_shapes=[
            pltpu.VMEM((4, D), bf16), pltpu.VMEM((D,), bf16), pltpu.VMEM((F,), bf16), pltpu.VMEM((D,), bf16),
            pltpu.VMEM(_FWD.shape, u32), pltpu.VMEM(_INV.shape, u32),
            pltpu.VMEM((2 * _layout(nb, nc, F)[1], LANES), bf16),
            [pltpu.VMEM((2 * R * 2 * P + 8, D), f32) for _ in range(nb)],
            [pltpu.VMEM((2 * R * P + 8, D), f32) for _ in range(nb)],
            pltpu.VMEM((8, D), f32),
            pltpu.VMEM((1, F), f32),
            [[pltpu.VMEM((P, F), u32) for _ in range(2)] for _ in range(nb)],
            pltpu.SemaphoreType.DMA((4, nb)),
            pltpu.SemaphoreType.DMA((6,)),
            pltpu.SemaphoreType.DMA((nb,)),
            pltpu.VMEM((NCUT, 16, LANES), bf16),
            pltpu.SemaphoreType.DMA((NCUT,)),
        ],
        compiler_params=pltpu.CompilerParams(vmem_limit_bytes=120 * 1024 * 1024),
    )(jnp.asarray(np.zeros((1,), np.int32)), q, k, v, A_ssm_k, B_w1.T, B_w2, A_shift_k.T, A_ssm_D, B_b1, B_b2,
      jnp.asarray(_FWD), jnp.asarray(_INV))
    return out.reshape(B, S, D)
```

```python
import functools

import numpy as np
import jax
import jax.numpy as jnp
import jax.experimental.pallas as pl
import jax.experimental.pallas.tpu as pltpu

R = 4
P = 128
H = P // 2
TB = R * P
NFFT = 2 * TB
LANES = 128
RG = 8
import os
_E = lambda k, d: int(os.environ.get(k, d))
LAG = int(os.environ.get('LAG', 2))
C_LN, C_PREP, C_FIN = _E('CLN', 135), _E('CP', 115), _E('CF', 105)
PR, LR = _E('PR', 32), _E('LR', 32)
C_M = (_E('CM0', 120), _E('CM1', 125), _E('CM2', 125), _E('CM3', 130))
NT = int(os.environ.get('NT', 0))
PT = _E('PT', 7)
MB = [int(x) for x in os.environ.get('MB', '1').split(',')]
NCUT = _E('NCUT', 2)
M128, KP = _E('M128', 0), _E('KP', 256)
TL = _E('TL', 2)
FR, FT = _E('FR', 64), _E('FT', 7)
FC = 256


def _pack_rows(m):
    u = np.ascontiguousarray(m, np.float32).view(np.uint32).astype(np.uint64)
    h = ((u + 0x7FFF + ((u >> 16) & 1)) >> 16).astype(np.uint32)
    return h[..., 0::2, :] | (h[..., 1::2, :] << np.uint32(16))


def _dft_tables():
    g = np.concatenate([np.arange(0, P, 2), np.arange(1, P, 2)]).astype(np.float64)
    s = np.arange(P, dtype=np.float64)
    fwd, inv = [], []
    for r in range(R):
        th = 2.0 * np.pi * (g[:, None] + 0.5) * (R * s[None, :] + r) / NFFT
        fwd.append(np.concatenate([np.cos(th), -np.sin(th)], 0))
        inv.append(np.stack([np.cos(th).T, -np.sin(th).T], 2).reshape(P, 2 * P) * (2.0 / NFFT))
    return _pack_rows(np.stack(fwd)), _pack_rows(np.stack(inv))


_FWD, _INV = _dft_tables()
_GC = float(np.sqrt(2.0 / np.pi))
f32, bf16, u32 = jnp.float32, jnp.bfloat16, jnp.uint32


def _layout(nb, nc, F):
    spec = dict(q=(nb * nc, TB // 2), k=(nc, 8 + nb * TB // 2), v=(nb * nc, TB // 2), kt=(nb * nc, TB // 2),
                sk=(nb * R * nc, H),
                o=(nb * nc, TB // 2), w1=(nc, F // 2), w2=(nc, F // 2),
                xn=(nb * R * nc, H), xu=(nb * R * nc, H), xk=(nb * R * nc, H),
                u=((nb - 1) * R * nc, 2 * P), kf=((nb - 1) * R * nc, 2 * P), kp=((nb - 1) * R * nc, 2 * P),
                z=(nb * R * nc, P), tick=(1, 8))
    off, out = 0, {}
    for name, (n, rows) in spec.items():
        out[name] = (off, rows)
        off += n * rows
    return out, off


def _lo(w):
    return pltpu.bitcast(w << 16, f32)


def _hi(w):
    return pltpu.bitcast(w & np.uint32(0xFFFF0000), f32)


def _packed(x):
    return pltpu.bitcast(x.astype(bf16), u32)


def _pair(a, b):
    return pltpu.bitcast(pltpu.pack_elementwise([a, b], packed_dtype=bf16), u32)


def _kernel(zero_ref, q_hbm, k_hbm, v_hbm, sk_hbm, w1_hbm, w2_hbm,
            shift_hbm, sd_hbm, b1_hbm, b2_hbm, fwd_hbm, inv_hbm,
            o_hbm,
            shift_ref, sd_ref, b1_ref, b2_ref, fwd_ref, inv_ref,
            arena16, ebuf, fbuf, obuf, prm, b1s, hbuf, in_sem, w_sem, out_sem, cut_buf, cut_sem, *, nc, nb, D, F):
    lanes = [slice(c * LANES, (c + 1) * LANES) for c in range(nc)]
    lay, total = _layout(nb, nc, F)
    arena = arena16.bitcast(u32)
    zero = pl.multiple_of(zero_ref[0], 8)

    i0 = jnp.zeros((), jnp.int32)

    def rows(start, n):
        return pl.ds(pl.multiple_of(i0 + start, 8), n)

    def late(ref):
        return ref.at[pl.ds(zero, ref.shape[0]), :]

    ordered = late(arena)
    e_ord, f_ord = [late(r) for r in ebuf], [late(r) for r in fbuf]
    E_ROWS, F_ROWS = 2 * R * 2 * P, 2 * R * P

    def at(name, *idx):
        n = 0
        for i in idx[:-1]:
            n = n * R + i
        return lay[name][0] + (n * nc + idx[-1]) * lay[name][1]

    def ld(row, n):
        return pltpu.bitcast(ordered[rows(row, n), :], f32)

    def st(row, val):
        arena[rows(row, val.shape[0]), :] = pltpu.bitcast(val, u32)

    def slab16(row, n):
        return arena16.at[2 * row:2 * (row + n), :]

    def wide(name, *idx):
        return jnp.concatenate([arena[rows(at(name, *idx, c), lay[name][1]), :] for c in range(nc)], axis=1)

    def cols_in(src, b, offs, sem):
        return [pltpu.make_async_copy(src.at[pl.ds(b * TB, TB), lanes[c]], slab16(offs[c], TB // 2), sem)
                for c in range(nc)]

    def conv_in(b):
        return (cols_in(k_hbm, b, [at("k", c) + 8 + b * TB // 2 for c in range(nc)], in_sem.at[0, b])
                + cols_in(v_hbm, b, [at("v", b, c) for c in range(nc)], in_sem.at[1, b])
                + [pltpu.make_async_copy(sk_hbm.at[lanes[c], pl.ds(b * TB + n * P, P)],
                                         slab16(at("sk", b, n, c), H), in_sem.at[2, b])
                   for c in range(nc) for n in range(R)])

    def q_in(b):
        return cols_in(q_hbm, b, [at("q", b, c) for c in range(nc)], in_sem.at[3, b])

    def out_copy(b, c, src=ordered):
        return pltpu.make_async_copy(slab16(at("o", b, c), TB // 2) if src is ordered else obuf[b].at[c],
                                     o_hbm.at[pl.ds(b * TB, TB), lanes[c]], out_sem.at[b])

    def w1_in(lo, hi, n):
        return [pltpu.make_async_copy(w1_hbm.at[lo:hi, lanes[c]], slab16(at("w1", c) + lo // 2, (hi - lo) // 2),
                                      w_sem.at[n]) for c in range(nc)]

    small_in = [pltpu.make_async_copy(src, dst, w_sem.at[3]) for src, dst in (
        (shift_hbm, shift_ref), (sd_hbm, sd_ref), (b1_hbm, b1_ref), (b2_hbm, b2_ref))]
    tables_in = [pltpu.make_async_copy(fwd_hbm, fwd_ref, w_sem.at[4]),
                 pltpu.make_async_copy(inv_hbm, inv_ref, w_sem.at[5])]
    w2_in = [pltpu.make_async_copy(w2_hbm.at[:, lanes[c]], slab16(at("w2", c), F // 2), w_sem.at[1])
             for c in range(nc)]

    def start(cs):
        for c in cs:
            c.start()

    def wait(cs):
        for c in cs:
            c.wait()

    tiles = {}

    def t_load(b, c, n):
        w = pltpu.bitcast(ordered[rows(at("sk", b, n, c), H), :], bf16)
        tiles[b, c, n] = pltpu.bitcast(w.T, u32)

    def t_store(b, c, n):
        st(at("kt", b, c) + n * H, tiles.pop((b, c, n)))

    def prep_unit(b, j, c, s0):
        base = at("k", c) + 8 + b * TB // 2 + j + 2 * s0
        t = ordered[rows(at("k", c), 8), :]
        if PT == 0:
            t = pltpu.roll(t, 1, 1)
        else:
            t = pltpu.bitcast(t, f32)
            for _ in range(PT):
                t = jnp.tanh(t)

        wa = ordered[pl.ds(base - 2, PR, stride=2), :]
        wb = ordered[pl.ds(base - 1, PR, stride=2), :]
        wc = ordered[pl.ds(base, PR, stride=2), :]
        ks = [_hi(wa), _lo(wb), _hi(wb), _lo(wc), _hi(wc)]
        vw = ordered[pl.ds(at("v", b, c) + j + 2 * s0, PR, stride=2), :]
        vs = [_lo(vw), _hi(vw)]
        tw = ordered[pl.ds(at("kt", b, c) + j + 2 * s0, PR, stride=2), :]
        ts = [_lo(tw), _hi(tw)]
        for e in range(2):
            acc = ks[3 + e] * prm[0:1, lanes[c]]
            for i in range(1, 4):
                acc = acc + ks[3 + e - i] * prm[i:i + 1, lanes[c]]
            st(at("xu", b, 2 * j + e, c) + s0 // 2, _packed(acc * vs[e]))
            st(at("xk", b, 2 * j + e, c) + s0 // 2, _packed(ts[e]))
        st(at("tick", 0), t)

    def m_unit(b, g0, c):
        def cld(name, slot, m):
            row = at(name, slot, m, c) + g0
            return ld(row, RG), ld(row + P, RG)

        def cst(name, m, vr, vi):
            row = at(name, b, m, c) + g0
            st(row, vr)
            st(row + P, vi)

        def bfly(which):
            offs = [(which * R + r) * 2 * P + g0 for r in range(R)]
            er = [e_ord[b][rows(o, RG), lanes[c]] for o in offs]
            ei = [e_ord[b][rows(o + P, RG), lanes[c]] for o in offs]
            ar, ai = er[0] + er[2], ei[0] + ei[2]
            br, bi = er[0] - er[2], ei[0] - ei[2]
            cr, ci = er[1] + er[3], ei[1] + ei[3]
            dr, di = er[1] - er[3], ei[1] - ei[3]
            return ([ar + cr, br + di, ar - cr, br - di],
                    [ai + ci, bi - dr, ai - ci, bi + dr])

        tick = pltpu.roll(e_ord[b][rows(g0, RG), lanes[c]], 1, 1)
        for _ in range(NT):
            tick = jnp.tanh(tick)
        ur, ui = bfly(0)
        kr, ki = bfly(1)
        if b == 0:
            kr = [x + prm[4:5, lanes[c]] for x in kr]
        keep = []
        for m in range(R):
            if b == 0:
                keep.append((kr[m], ki[m]))
            else:
                pr, pi = cld("kp", b - 1, m)
                keep.append((kr[m] - pi, ki[m] + pr) if g0 < P // 2 else (kr[m] + pi, ki[m] - pr))
        if b < nb - 1:
            for m in range(R):
                cst("kp", m, kr[m], ki[m])
                cst("u", m, ur[m], ui[m])
                cst("kf", m, *keep[m])
        else:
            st(at("tick", 0), keep[R - 1][1])
        yr, yi = [], []
        for m in range(R):
            accr = acci = None
            for jj in range(b + 1):
                a_r, a_i = (ur[m], ui[m]) if jj == b else cld("u", jj, m)
                b_r, b_i = keep[m] if jj == 0 else cld("kf", b - jj, m)
                pr_ = a_r * b_r - a_i * b_i
                pi_ = a_r * b_i + a_i * b_r
                accr = pr_ if accr is None else accr + pr_
                acci = pi_ if acci is None else acci + pi_
            yr.append(accr)
            yi.append(acci)
            if b >= 2 and m in MB:
                st(at("tick", 0), acci)
        ar, ai = yr[0] + yr[2], yi[0] + yi[2]
        br, bi = yr[0] - yr[2], yi[0] - yi[2]
        cr, ci = yr[1] + yr[3], yi[1] + yi[3]
        dr, di = yr[1] - yr[3], yi[1] - yi[3]
        zr = [ar + cr, br - di, ar - cr, br + di]
        zi = [ai + ci, bi + dr, ai - ci, bi - dr]
        for r in range(R):
            st(at("z", b, r, c) + g0, _pair(zr[r], zi[r]))
        ebuf[b][E_ROWS:E_ROWS + RG, 0:LANES] = tick
        st(at("tick", 0), tick)

    def q_words(src, b, j, c):
        return src[pl.ds(at("q", b, c) + j, P, stride=2), :]

    def ln_rows(src, b, r, s0):
        return jnp.concatenate([(_lo, _hi)[r % 2](src[pl.ds(at("q", b, c) + r // 2 + 2 * s0, LR, stride=2), :])
                                for c in range(nc)], axis=1)

    mean, rstd = {}, {}

    def ln_mean(src, key):
        mean[key] = jnp.mean(ln_rows(src, *key), axis=-1, keepdims=True)

    def ln_rstd(src, key):
        xc = ln_rows(src, *key) - mean[key]
        rstd[key] = jax.lax.rsqrt(jnp.mean(xc * xc, axis=-1, keepdims=True) + 1e-5)

    def ln_store(src, key):
        b, r, s0 = key
        xn = _packed((ln_rows(src, *key) - mean.pop(key)) * rstd.pop(key))
        for c in range(nc):
            st(at("xn", b, r, c) + s0 // 2, xn[:, lanes[c]])

    def ln_unit(src, keys, n):
        for stage, fn in enumerate((ln_mean, ln_rstd, ln_store)):
            if 0 <= n - stage < len(keys):
                fn(src, keys[n - stage])

    def emit_out(src, fsrc, b, j, c, o, s0=0):
        n = o[0].shape[0]
        outs = []
        for e in range(2):
            r = 2 * j + e
            xn = pltpu.bitcast(src[rows(at("xn", b, r, c) + s0 // 2, n // 2), :], bf16).astype(f32)
            outs.append(o[e] + xn * fsrc[(R + r) * P + s0:(R + r) * P + s0 + n, lanes[c]])
        if src is ordered:
            arena[pl.ds(at("o", b, c) + j + 2 * s0, n, stride=2), :] = _pair(*outs)
        else:
            obuf[b].at[c].bitcast(u32)[pl.ds(j + 2 * s0, n, stride=2), :] = _pair(*outs)
        if j == 1 and s0 + n == P:
            out_copy(b, c, src).start()

    def fin_gate(b):
        fbuf[b][F_ROWS:F_ROWS + 8, 0:LANES] = ld(at("k", 0), 8)

    def fin_unit(b, j, c, s0):
        o = [f_ord[b][(2 * j + e) * P + s0:(2 * j + e) * P + s0 + FR, lanes[c]] for e in range(2)]
        tick = f_ord[b][0:8, lanes[c]]
        emit_out(ordered, f_ord[b], b, j, c, o, s0)
        for _ in range(FT):
            tick = jnp.tanh(tick)
        fbuf[b][F_ROWS:F_ROWS + 8, 0:LANES] = tick
        st(at("tick", 0), tick)

    queue = []
    credit = [0]

    def fill(cycles):
        credit[0] += cycles
        while queue and credit[0] >= queue[0][2]:
            _, fn, cost = queue.pop(0)
            credit[0] -= cost
            fn()
        if not queue:
            credit[0] = min(credit[0], 128)

    def need(tag):
        while any(t == tag for t, _, _ in queue):
            queue.pop(0)[1]()

    marks = {}
    pieces = []
    cursor = [0]

    def weights(row, n):
        i = cursor[0]
        assert pieces[i][0] == row
        cursor[0] += 1
        for p in range(len(marks), min(i + 1 + LAG, len(pieces))):
            need(pieces[p][1])
            marks[p] = ordered[rows(pieces[p][0], 8), :]
            fill(pieces[p][2])
        return pltpu.bitcast(jnp.concatenate([marks[i], arena[rows(row + 8, n - 8), :]], axis=0), bf16)

    def mm1_op(b, j, s0, s1):
        need(("ln", b, j))
        w = jnp.concatenate([weights(at("w1", c) + s0 // 2, (s1 - s0) // 2) for c in range(nc)], axis=1)
        x = pltpu.bitcast(jnp.concatenate([wide("xn", b, 2 * j), wide("xn", b, 2 * j + 1)], axis=0), bf16)
        h = jax.lax.dot_general(x, w, (((1,), (1,)), ((), ())), preferred_element_type=f32) + b1s[0:1, s0:s1]
        u = h * (h * h * (_GC * 0.044715) + _GC)
        hh = 0.5 * h
        hbuf[b][j][:, s0:s1] = _packed(hh * jnp.tanh(u) + hh)

    def mm2_op(b, j, c, fused):
        def w():
            return jnp.concatenate([weights(at("w2", c) + s0 // 2, (min(s0 + KP, F) - s0) // 2)
                                    for s0 in range(0, F, KP)], axis=0)
        if M128:
            mlp = [jnp.dot(pltpu.bitcast(hbuf[b][j][e * H:(e + 1) * H, :], bf16), w(), preferred_element_type=f32)
                   for e in range(2)]
        else:
            mlp = jnp.dot(pltpu.bitcast(hbuf[b][j][...], bf16), w(), preferred_element_type=f32)
            mlp = [mlp[0:P], mlp[P:2 * P]]
        qw = q_words(arena, b, j, c)
        o = [mlp[0] + prm[5:6, lanes[c]] + _lo(qw), mlp[1] + prm[5:6, lanes[c]] + _hi(qw)]
        if fused:
            emit_out(arena, fbuf[b], b, j, c, o)
        else:
            for e in range(2):
                fbuf[b][(2 * j + e) * P:(2 * j + e + 1) * P, lanes[c]] = o[e]

    def fwd_op(b, r, src, dst):
        e = jnp.dot(pltpu.bitcast(fwd_ref[r], bf16), jnp.concatenate([weights(at(src, b, r, c), H) for c in range(nc)], axis=1),
                    preferred_element_type=f32)
        ebuf[b][(dst * R + r) * 2 * P:(dst * R + r + 1) * 2 * P, :] = e

    def inv_op(b, r):
        y = jnp.dot(pltpu.bitcast(inv_ref[r], bf16), jnp.concatenate([weights(at("z", b, r, c), P) for c in range(nc)], axis=1),
                    preferred_element_type=f32)
        fbuf[b][(R + r) * P:(R + r + 1) * P, :] = y

    part = functools.partial

    prog = []

    def push(units):
        prog.append(part(queue.extend, units))

    def ln(src, blocks, cost=C_LN):
        keys = [(b, r, s0) for b in blocks for r in range(R) for s0 in range(0, P, LR)]
        tag = lambda n: ("ln", keys[n][0], keys[n][1] // 2)
        return [(tag(max(n - 2, 0)), part(ln_unit, src, keys, n), cost) for n in range(len(keys) + 2)]

    def prep(blocks):
        ts = [(b, c, n) for b in blocks for c in range(nc) for n in range(R)]
        out = []
        for i in range(-TL - 1, len(ts)):
            tag = ("prep", ts[max(i, 0)][0])
            if i + TL + 1 < len(ts):
                out.append((tag, part(t_load, *ts[i + TL + 1]), 0))
            for j in range(2):
                if j == 1 and -1 <= i < len(ts) - 1:
                    out.append((tag, part(t_store, *ts[i + 1]), 0))
                if i >= 0:
                    out.append((tag, part(prep_unit, ts[i][0], j, ts[i][1], ts[i][2] * PR), C_PREP))
                else:
                    out.append((tag, lambda: None, C_PREP))
        return out

    def spectral(b):
        return [(("m", b), part(m_unit, b, g0, c), C_M[b]) for g0 in range(0, P, RG) for c in range(nc)]

    def fin(b, n=nc):
        return [(("fin", b), part(fin_gate, b), 0)] + [
            (("fin", b), part(fin_unit, b, j, c, s0), C_FIN)
            for c in range(n) for j in range(2) for s0 in range(0, P, FR)]

    def mix(main, extra):
        out = []
        for i, u in enumerate(main):
            out += extra[i * len(extra) // len(main):(i + 1) * len(extra) // len(main)] + [u]
        return out

    def mm1(b, lo=0, hi=None):
        for s0, j in [(s0, j) for s0 in range(0, F, FC) for j in range(2)][lo:hi]:
            s1 = min(s0 + FC, F)
            pieces.extend((at("w1", c) + s0 // 2, None, 64 * pl.cdiv(s1 - s0, LANES)) for c in range(nc))
            prog.append(part(mm1_op, b, j, s0, s1))

    def mm2(b, lo=0, hi=None, fused=False):
        for c, j in [(c, j) for c in range(nc) for j in range(2)][lo:hi]:
            pieces.extend((at("w2", c) + s0 // 2, None, pl.cdiv(min(KP, F - s0), LANES) * (32 if M128 else 64))
                          for _ in range(1 + M128) for s0 in range(0, F, KP))
            prog.append(part(mm2_op, b, j, c, fused))

    def fwd(b):
        for r in range(R):
            for dst, src in enumerate(("xu", "xk")):
                pieces.extend((at(src, b, r, c), ("prep", b), 64) for c in range(nc))
                prog.append(part(fwd_op, b, r, src, dst))

    def inv(b):
        for r in range(R):
            pieces.extend((at("z", b, r, c), ("m", b), 64) for c in range(nc))
            prog.append(part(inv_op, b, r))

    def run(then_wait=()):
        for step in prog:
            step()
        prog.clear(), pieces.clear(), marks.clear()
        cursor[0] = 0
        credit[0] = -256
        wait(then_wait)

    feed = [q_in(0), w1_in(0, 4 * FC, 0) + small_in, w1_in(4 * FC, F, 2) + q_in(1),
            q_in(2) + conv_in(0) + tables_in[:1], w2_in + conv_in(1) + q_in(3) + tables_in[1:],
            conv_in(2) + conv_in(3)]
    cuts = [pltpu.make_async_copy(q_hbm.at[0:16, 0:LANES], cut_buf.at[i], cut_sem.at[i]) for i in range(NCUT)]

    def params():
        prm[0:4, :] = shift_ref[...].astype(f32)
        prm[4:5, :] = sd_ref[...].astype(f32).reshape(1, D)
        prm[5:6, :] = b2_ref[...].astype(f32).reshape(1, D)
        b1s[...] = b1_ref[...].astype(f32).reshape(1, F)

    start(feed[0] + feed[1])
    for c in range(nc): st(at("k", c), jnp.zeros((8, LANES), u32))
    wait(feed[0])
    push(ln(arena, [0]))
    prog.append(part(need, ("ln", 0, 1)))
    run(feed[1])
    start(feed[2] + cuts)
    params()
    mm1(0, 0, 8)
    run(feed[2])
    start(feed[3])
    push(ln(ordered, [1], 160))
    mm1(0, 8)
    mm1(1, 0, 4)
    run(feed[3])
    start(feed[4])
    push(prep([0]))
    mm1(1, 4)
    push(ln(ordered, [2]))
    fwd(0)
    push(spectral(0))
    mm1(2)
    run(feed[4])
    start(feed[5])
    push(prep([1]))
    mm2(0, 0, 6)
    push(ln(ordered, [3]))
    fwd(1)
    push(spectral(1))
    mm1(3)
    mm2(0, 6, 8)
    run(feed[5])
    push(prep([2, 3]))
    mm2(0, 8)
    inv(0)
    mm2(1, 0, 3)
    fwd(2)
    mm2(1, 3, 5)
    run(cuts[0:1])
    push(spectral(2))
    fwd(3)
    mm2(1, 5)
    inv(1)
    mm2(2, 0, 2)
    run(cuts[1:2])
    push(spectral(3))
    mm2(2, 2)
    inv(2)
    mm2(3, 0, 2)
    inv(3)
    push(fin(0) + fin(1) + fin(2) + fin(3, 1))
    mm2(3, 2, fused=True)
    prog.append(part(need, ("fin", 3)))
    run()
    for b in range(nb):
        wait([out_copy(b, c) for c in range(nc)])


@jax.jit
def pallas_parallel_sum__ssm_conv_h3__dense_activation_gelu__prompt_kernel(
    A_q: jax.Array,
    A_k: jax.Array,
    A_v: jax.Array,
    A_shift_k: jax.Array,
    A_ssm_k: jax.Array,
    A_ssm_D: jax.Array,
    B_x: jax.Array,
    B_w1: jax.Array,
    B_b1: jax.Array,
    B_w2: jax.Array,
    B_b2: jax.Array,
):
    B, S, D = A_q.shape
    F = B_w1.shape[1]
    nc, nb = D // LANES, S // TB
    q, k, v = (a.reshape(S, D) for a in (A_q, A_k, A_v))
    hbm = pl.BlockSpec(memory_space=pltpu.HBM)
    out = pl.pallas_call(
        functools.partial(_kernel, nc=nc, nb=nb, D=D, F=F),
        in_specs=[pl.BlockSpec(memory_space=pltpu.SMEM)] + [hbm] * 12,
        out_specs=hbm,
        out_shape=jax.ShapeDtypeStruct((S, D), A_q.dtype),
        scratch_shapes=[
            pltpu.VMEM((4, D), bf16), pltpu.VMEM((D,), bf16), pltpu.VMEM((F,), bf16), pltpu.VMEM((D,), bf16),
            pltpu.VMEM(_FWD.shape, u32), pltpu.VMEM(_INV.shape, u32),
            pltpu.VMEM((2 * _layout(nb, nc, F)[1], LANES), bf16),
            [pltpu.VMEM((2 * R * 2 * P + 8, D), f32) for _ in range(nb)],
            [pltpu.VMEM((2 * R * P + 8, D), f32) for _ in range(nb)],
            [pltpu.VMEM((nc, TB, LANES), bf16) for _ in range(nb)],
            pltpu.VMEM((8, D), f32),
            pltpu.VMEM((1, F), f32),
            [[pltpu.VMEM((P, F), u32) for _ in range(2)] for _ in range(nb)],
            pltpu.SemaphoreType.DMA((4, nb)),
            pltpu.SemaphoreType.DMA((6,)),
            pltpu.SemaphoreType.DMA((nb,)),
            pltpu.VMEM((NCUT, 16, LANES), bf16),
            pltpu.SemaphoreType.DMA((NCUT,)),
        ],
        compiler_params=pltpu.CompilerParams(vmem_limit_bytes=120 * 1024 * 1024),
    )(jnp.asarray(np.zeros((1,), np.int32)), q, k, v, A_ssm_k, B_w1.T, B_w2, A_shift_k.T, A_ssm_D, B_b1, B_b2,
      jnp.asarray(_FWD), jnp.asarray(_INV))
    return out.reshape(B, S, D)
```

```python
import functools

import numpy as np
import jax
import jax.numpy as jnp
import jax.experimental.pallas as pl
import jax.experimental.pallas.tpu as pltpu

R = 4
P = 128
H = P // 2
TB = R * P
NFFT = 2 * TB
LANES = 128
IM, SR = P + 8, 2 * P + 24
RG = 8
import os
_E = lambda k, d: int(os.environ.get(k, d))
LAG = int(os.environ.get('LAG', 2))
C_LN, C_PREP, C_FIN = _E('CLN', 135), _E('CP', 115), _E('CF', 105)
PR, LR = _E('PR', 32), _E('LR', 32)
C_M = (_E('CM0', 120), _E('CM1', 125), _E('CM2', 125), _E('CM3', 130))
NT = int(os.environ.get('NT', 0))
PT = _E('PT', 7)
MB = [int(x) for x in os.environ.get('MB', '1').split(',')]
NCUT = _E('NCUT', 2)
M128, KP = _E('M128', 0), _E('KP', 256)
TL = _E('TL', 2)
FR, FT = _E('FR', 64), _E('FT', 7)
FC = 256


def _pack_rows(m):
    u = np.ascontiguousarray(m, np.float32).view(np.uint32).astype(np.uint64)
    h = ((u + 0x7FFF + ((u >> 16) & 1)) >> 16).astype(np.uint32)
    return h[..., 0::2, :] | (h[..., 1::2, :] << np.uint32(16))


def _dft_tables():
    g = np.concatenate([np.arange(0, P, 2), np.arange(1, P, 2)]).astype(np.float64)
    s = np.arange(P, dtype=np.float64)
    fwd, inv = [], []
    for r in range(R):
        th = 2.0 * np.pi * (g[:, None] + 0.5) * (R * s[None, :] + r) / NFFT
        fwd.append(np.concatenate([np.cos(th), -np.sin(th)], 0))
        inv.append(np.stack([np.cos(th).T, -np.sin(th).T], 2).reshape(P, 2 * P) * (2.0 / NFFT))
    return _pack_rows(np.stack(fwd)), _pack_rows(np.stack(inv))


_FWD, _INV = _dft_tables()
_GC = float(np.sqrt(2.0 / np.pi))
f32, bf16, u32 = jnp.float32, jnp.bfloat16, jnp.uint32


def _layout(nb, nc, F):
    spec = dict(q=(nb * nc, TB // 2), k=(nc, 8 + nb * TB // 2), v=(nb * nc, TB // 2), kt=(nb * nc, TB // 2),
                sk=(nb * R * nc, H),
                o=(nb * nc, TB // 2), w1=(nc, F // 2), w2=(nc, F // 2),
                xn=(nb * R * nc, H), xu=(nb * R * nc, H), xk=(nb * R * nc, H),
                u=((nb - 1) * R * nc, SR), kf=((nb - 1) * R * nc, SR), kp=((nb - 1) * R * nc, SR),
                z=(nb * R * nc, P + 8), tick=(1, 8))
    off, out = 0, {}
    for name, (n, rows) in spec.items():
        out[name] = (off, rows)
        off += n * rows
    return out, off


def _lo(w):
    return pltpu.bitcast(w << 16, f32)


def _hi(w):
    return pltpu.bitcast(w & np.uint32(0xFFFF0000), f32)


def _packed(x):
    return pltpu.bitcast(x.astype(bf16), u32)


def _pair(a, b):
    return pltpu.bitcast(pltpu.pack_elementwise([a, b], packed_dtype=bf16), u32)


def _kernel(zero_ref, q_hbm, k_hbm, v_hbm, sk_hbm, w1_hbm, w2_hbm,
            shift_hbm, sd_hbm, b1_hbm, b2_hbm, fwd_hbm, inv_hbm,
            o_hbm,
            shift_ref, sd_ref, b1_ref, b2_ref, fwd_ref, inv_ref,
            arena16, ebuf, fbuf, obuf, prm, b1s, hbuf, in_sem, w_sem, out_sem, cut_buf, cut_sem, *, nc, nb, D, F):
    lanes = [slice(c * LANES, (c + 1) * LANES) for c in range(nc)]
    lay, total = _layout(nb, nc, F)
    arena = arena16.bitcast(u32)
    zero = pl.multiple_of(zero_ref[0], 8)

    i0 = jnp.zeros((), jnp.int32)

    def rows(start, n):
        return pl.ds(pl.multiple_of(i0 + start, 8), n)

    def late(ref):
        return ref.at[pl.ds(zero, ref.shape[0]), :]

    ordered = late(arena)
    e_ord, f_ord = [late(r) for r in ebuf], [late(r) for r in fbuf]
    E_ROWS, F_ROWS = 2 * R * SR, 2 * R * P

    def at(name, *idx):
        n = 0
        for i in idx[:-1]:
            n = n * R + i
        return lay[name][0] + (n * nc + idx[-1]) * lay[name][1]

    def ld(row, n):
        return pltpu.bitcast(ordered[rows(row, n), :], f32)

    def st(row, val):
        arena[rows(row, val.shape[0]), :] = pltpu.bitcast(val, u32)

    def slab16(row, n):
        return arena16.at[2 * row:2 * (row + n), :]

    def wide(name, *idx):
        return jnp.concatenate([arena[rows(at(name, *idx, c), lay[name][1]), :] for c in range(nc)], axis=1)

    def cols_in(src, b, offs, sem):
        return [pltpu.make_async_copy(src.at[pl.ds(b * TB, TB), lanes[c]], slab16(offs[c], TB // 2), sem)
                for c in range(nc)]

    def conv_in(b):
        return (cols_in(k_hbm, b, [at("k", c) + 8 + b * TB // 2 for c in range(nc)], in_sem.at[0, b])
                + cols_in(v_hbm, b, [at("v", b, c) for c in range(nc)], in_sem.at[1, b])
                + [pltpu.make_async_copy(sk_hbm.at[lanes[c], pl.ds(b * TB + n * P, P)],
                                         slab16(at("sk", b, n, c), H), in_sem.at[2, b])
                   for c in range(nc) for n in range(R)])

    def q_in(b):
        return cols_in(q_hbm, b, [at("q", b, c) for c in range(nc)], in_sem.at[3, b])

    def out_copy(b, c, src=ordered):
        return pltpu.make_async_copy(slab16(at("o", b, c), TB // 2) if src is ordered else obuf[b].at[c],
                                     o_hbm.at[pl.ds(b * TB, TB), lanes[c]], out_sem.at[b])

    def w1_in(lo, hi, n):
        return [pltpu.make_async_copy(w1_hbm.at[lo:hi, lanes[c]], slab16(at("w1", c) + lo // 2, (hi - lo) // 2),
                                      w_sem.at[n]) for c in range(nc)]

    small_in = [pltpu.make_async_copy(src, dst, w_sem.at[3]) for src, dst in (
        (shift_hbm, shift_ref), (sd_hbm, sd_ref), (b1_hbm, b1_ref), (b2_hbm, b2_ref))]
    tables_in = [pltpu.make_async_copy(fwd_hbm, fwd_ref, w_sem.at[4]),
                 pltpu.make_async_copy(inv_hbm, inv_ref, w_sem.at[5])]
    w2_in = [pltpu.make_async_copy(w2_hbm.at[:, lanes[c]], slab16(at("w2", c), F // 2), w_sem.at[1])
             for c in range(nc)]

    def start(cs):
        for c in cs:
            c.start()

    def wait(cs):
        for c in cs:
            c.wait()

    tiles = {}

    def t_load(b, c, n):
        w = pltpu.bitcast(ordered[rows(at("sk", b, n, c), H), :], bf16)
        tiles[b, c, n] = pltpu.bitcast(w.T, u32)

    def t_store(b, c, n):
        st(at("kt", b, c) + n * H, tiles.pop((b, c, n)))

    def prep_unit(b, j, c, s0):
        base = at("k", c) + 8 + b * TB // 2 + j + 2 * s0
        t = ordered[rows(at("k", c), 8), :]
        if PT == 0:
            t = pltpu.roll(t, 1, 1)
        else:
            t = pltpu.bitcast(t, f32)
            for _ in range(PT):
                t = jnp.tanh(t)

        wa = ordered[pl.ds(base - 2, PR, stride=2), :]
        wb = ordered[pl.ds(base - 1, PR, stride=2), :]
        wc = ordered[pl.ds(base, PR, stride=2), :]
        ks = [_hi(wa), _lo(wb), _hi(wb), _lo(wc), _hi(wc)]
        vw = ordered[pl.ds(at("v", b, c) + j + 2 * s0, PR, stride=2), :]
        vs = [_lo(vw), _hi(vw)]
        tw = ordered[pl.ds(at("kt", b, c) + j + 2 * s0, PR, stride=2), :]
        ts = [_lo(tw), _hi(tw)]
        for e in range(2):
            acc = ks[3 + e] * prm[0:1, lanes[c]]
            for i in range(1, 4):
                acc = acc + ks[3 + e - i] * prm[i:i + 1, lanes[c]]
            st(at("xu", b, 2 * j + e, c) + s0 // 2, _packed(acc * vs[e]))
            st(at("xk", b, 2 * j + e, c) + s0 // 2, _packed(ts[e]))
        st(at("tick", 0), t)

    def m_unit(b, g0, c):
        def cld(name, slot, m):
            row = at(name, slot, m, c) + g0
            return ld(row, RG), ld(row + IM, RG)

        def cst(name, m, vr, vi):
            row = at(name, b, m, c) + g0
            st(row, vr)
            st(row + IM, vi)

        def bfly(which):
            offs = [(which * R + r) * SR + g0 for r in range(R)]
            er = [e_ord[b][rows(o, RG), lanes[c]] for o in offs]
            ei = [e_ord[b][rows(o + IM, RG), lanes[c]] for o in offs]
            ar, ai = er[0] + er[2], ei[0] + ei[2]
            br, bi = er[0] - er[2], ei[0] - ei[2]
            cr, ci = er[1] + er[3], ei[1] + ei[3]
            dr, di = er[1] - er[3], ei[1] - ei[3]
            return ([ar + cr, br + di, ar - cr, br - di],
                    [ai + ci, bi - dr, ai - ci, bi + dr])

        tick = pltpu.roll(e_ord[b][rows(g0, RG), lanes[c]], 1, 1)
        for _ in range(NT):
            tick = jnp.tanh(tick)
        ur, ui = bfly(0)
        kr, ki = bfly(1)
        if b == 0:
            kr = [x + prm[4:5, lanes[c]] for x in kr]
        keep = []
        for m in range(R):
            if b == 0:
                keep.append((kr[m], ki[m]))
            else:
                pr, pi = cld("kp", b - 1, m)
                keep.append((kr[m] - pi, ki[m] + pr) if g0 < P // 2 else (kr[m] + pi, ki[m] - pr))
        if b < nb - 1:
            for m in range(R):
                cst("kp", m, kr[m], ki[m])
                cst("u", m, ur[m], ui[m])
                cst("kf", m, *keep[m])
        else:
            st(at("tick", 0), keep[R - 1][1])
        yr, yi = [], []
        for m in range(R):
            accr = acci = None
            for jj in range(b + 1):
                a_r, a_i = (ur[m], ui[m]) if jj == b else cld("u", jj, m)
                b_r, b_i = keep[m] if jj == 0 else cld("kf", b - jj, m)
                pr_ = a_r * b_r - a_i * b_i
                pi_ = a_r * b_i + a_i * b_r
                accr = pr_ if accr is None else accr + pr_
                acci = pi_ if acci is None else acci + pi_
            yr.append(accr)
            yi.append(acci)
            if b >= 2 and m in MB:
                st(at("tick", 0), acci)
        ar, ai = yr[0] + yr[2], yi[0] + yi[2]
        br, bi = yr[0] - yr[2], yi[0] - yi[2]
        cr, ci = yr[1] + yr[3], yi[1] + yi[3]
        dr, di = yr[1] - yr[3], yi[1] - yi[3]
        zr = [ar + cr, br - di, ar - cr, br + di]
        zi = [ai + ci, bi + dr, ai - ci, bi - dr]
        for r in range(R):
            st(at("z", b, r, c) + g0, _pair(zr[r], zi[r]))
        ebuf[b][E_ROWS:E_ROWS + RG, 0:LANES] = tick
        st(at("tick", 0), tick)

    def q_words(src, b, j, c):
        return src[pl.ds(at("q", b, c) + j, P, stride=2), :]

    def ln_rows(src, b, r, s0):
        return jnp.concatenate([(_lo, _hi)[r % 2](src[pl.ds(at("q", b, c) + r // 2 + 2 * s0, LR, stride=2), :])
                                for c in range(nc)], axis=1)

    mean, rstd = {}, {}

    def ln_mean(src, key):
        mean[key] = jnp.mean(ln_rows(src, *key), axis=-1, keepdims=True)

    def ln_rstd(src, key):
        xc = ln_rows(src, *key) - mean[key]
        rstd[key] = jax.lax.rsqrt(jnp.mean(xc * xc, axis=-1, keepdims=True) + 1e-5)

    def ln_store(src, key):
        b, r, s0 = key
        xn = _packed((ln_rows(src, *key) - mean.pop(key)) * rstd.pop(key))
        for c in range(nc):
            st(at("xn", b, r, c) + s0 // 2, xn[:, lanes[c]])

    def ln_unit(src, keys, n):
        for stage, fn in enumerate((ln_mean, ln_rstd, ln_store)):
            if 0 <= n - stage < len(keys):
                fn(src, keys[n - stage])

    def emit_out(src, fsrc, b, j, c, o, s0=0):
        n = o[0].shape[0]
        outs = []
        for e in range(2):
            r = 2 * j + e
            xn = pltpu.bitcast(src[rows(at("xn", b, r, c) + s0 // 2, n // 2), :], bf16).astype(f32)
            outs.append(o[e] + xn * fsrc[(R + r) * P + s0:(R + r) * P + s0 + n, lanes[c]])
        if src is ordered:
            arena[pl.ds(at("o", b, c) + j + 2 * s0, n, stride=2), :] = _pair(*outs)
        else:
            obuf[b].at[c].bitcast(u32)[pl.ds(j + 2 * s0, n, stride=2), :] = _pair(*outs)
        if j == 1 and s0 + n == P:
            out_copy(b, c, src).start()

    def fin_gate(b):
        fbuf[b][F_ROWS:F_ROWS + 8, 0:LANES] = ld(at("k", 0), 8)

    def fin_unit(b, j, c, s0):
        o = [f_ord[b][(2 * j + e) * P + s0:(2 * j + e) * P + s0 + FR, lanes[c]] for e in range(2)]
        tick = f_ord[b][0:8, lanes[c]]
        emit_out(ordered, f_ord[b], b, j, c, o, s0)
        for _ in range(FT):
            tick = jnp.tanh(tick)
        fbuf[b][F_ROWS:F_ROWS + 8, 0:LANES] = tick
        st(at("tick", 0), tick)

    queue = []
    credit = [0]

    def fill(cycles):
        credit[0] += cycles
        while queue and credit[0] >= queue[0][2]:
            _, fn, cost = queue.pop(0)
            credit[0] -= cost
            fn()
        if not queue:
            credit[0] = min(credit[0], 128)

    def need(tag):
        while any(t == tag for t, _, _ in queue):
            queue.pop(0)[1]()

    marks = {}
    pieces = []
    cursor = [0]

    def weights(row, n):
        i = cursor[0]
        assert pieces[i][0] == row
        cursor[0] += 1
        for p in range(len(marks), min(i + 1 + LAG, len(pieces))):
            need(pieces[p][1])
            marks[p] = ordered[rows(pieces[p][0], 8), :]
            fill(pieces[p][2])
        return pltpu.bitcast(jnp.concatenate([marks[i], arena[rows(row + 8, n - 8), :]], axis=0), bf16)

    def mm1_op(b, j, s0, s1):
        need(("ln", b, j))
        w = jnp.concatenate([weights(at("w1", c) + s0 // 2, (s1 - s0) // 2) for c in range(nc)], axis=1)
        x = pltpu.bitcast(jnp.concatenate([wide("xn", b, 2 * j), wide("xn", b, 2 * j + 1)], axis=0), bf16)
        h = jax.lax.dot_general(x, w, (((1,), (1,)), ((), ())), preferred_element_type=f32) + b1s[0:1, s0:s1]
        u = h * (h * h * (_GC * 0.044715) + _GC)
        hh = 0.5 * h
        hbuf[b][j][:, s0:s1] = _packed(hh * jnp.tanh(u) + hh)

    def mm2_op(b, j, c, fused):
        def w():
            return jnp.concatenate([weights(at("w2", c) + s0 // 2, (min(s0 + KP, F) - s0) // 2)
                                    for s0 in range(0, F, KP)], axis=0)
        if M128:
            mlp = [jnp.dot(pltpu.bitcast(hbuf[b][j][e * H:(e + 1) * H, :], bf16), w(), preferred_element_type=f32)
                   for e in range(2)]
        else:
            mlp = jnp.dot(pltpu.bitcast(hbuf[b][j][...], bf16), w(), preferred_element_type=f32)
            mlp = [mlp[0:P], mlp[P:2 * P]]
        qw = q_words(arena, b, j, c)
        o = [mlp[0] + prm[5:6, lanes[c]] + _lo(qw), mlp[1] + prm[5:6, lanes[c]] + _hi(qw)]
        if fused:
            emit_out(arena, fbuf[b], b, j, c, o)
        else:
            for e in range(2):
                fbuf[b][(2 * j + e) * P:(2 * j + e + 1) * P, lanes[c]] = o[e]

    def fwd_op(b, r, src, dst):
        e = jnp.dot(pltpu.bitcast(fwd_ref[r], bf16), jnp.concatenate([weights(at(src, b, r, c), H) for c in range(nc)], axis=1),
                    preferred_element_type=f32)
        row = (dst * R + r) * SR
        ebuf[b][row:row + P, :] = e[0:P]
        ebuf[b][row + IM:row + IM + P, :] = e[P:2 * P]

    def inv_op(b, r):
        y = jnp.dot(pltpu.bitcast(inv_ref[r], bf16), jnp.concatenate([weights(at("z", b, r, c), P) for c in range(nc)], axis=1),
                    preferred_element_type=f32)
        fbuf[b][(R + r) * P:(R + r + 1) * P, :] = y

    part = functools.partial

    prog = []

    def push(units):
        prog.append(part(queue.extend, units))

    def ln(src, blocks, cost=C_LN):
        keys = [(b, r, s0) for b in blocks for r in range(R) for s0 in range(0, P, LR)]
        tag = lambda n: ("ln", keys[n][0], keys[n][1] // 2)
        return [(tag(max(n - 2, 0)), part(ln_unit, src, keys, n), cost) for n in range(len(keys) + 2)]

    def prep(blocks):
        ts = [(b, c, n) for b in blocks for c in range(nc) for n in range(R)]
        out = []
        for i in range(-TL - 1, len(ts)):
            tag = ("prep", ts[max(i, 0)][0])
            if i + TL + 1 < len(ts):
                out.append((tag, part(t_load, *ts[i + TL + 1]), 0))
            for j in range(2):
                if j == 1 and -1 <= i < len(ts) - 1:
                    out.append((tag, part(t_store, *ts[i + 1]), 0))
                if i >= 0:
                    out.append((tag, part(prep_unit, ts[i][0], j, ts[i][1], ts[i][2] * PR), C_PREP))
                else:
                    out.append((tag, lambda: None, C_PREP))
        return out

    def spectral(b):
        return [(("m", b), part(m_unit, b, g0, c), C_M[b]) for g0 in range(0, P, RG) for c in range(nc)]

    def fin(b, n=nc):
        return [(("fin", b), part(fin_gate, b), 0)] + [
            (("fin", b), part(fin_unit, b, j, c, s0), C_FIN)
            for c in range(n) for j in range(2) for s0 in range(0, P, FR)]

    def mix(main, extra):
        out = []
        for i, u in enumerate(main):
            out += extra[i * len(extra) // len(main):(i + 1) * len(extra) // len(main)] + [u]
        return out

    def mm1(b, lo=0, hi=None):
        for s0, j in [(s0, j) for s0 in range(0, F, FC) for j in range(2)][lo:hi]:
            s1 = min(s0 + FC, F)
            pieces.extend((at("w1", c) + s0 // 2, None, 64 * pl.cdiv(s1 - s0, LANES)) for c in range(nc))
            prog.append(part(mm1_op, b, j, s0, s1))

    def mm2(b, lo=0, hi=None, fused=False):
        for c, j in [(c, j) for c in range(nc) for j in range(2)][lo:hi]:
            pieces.extend((at("w2", c) + s0 // 2, None, pl.cdiv(min(KP, F - s0), LANES) * (32 if M128 else 64))
                          for _ in range(1 + M128) for s0 in range(0, F, KP))
            prog.append(part(mm2_op, b, j, c, fused))

    def fwd(b):
        for r in range(R):
            for dst, src in enumerate(("xu", "xk")):
                pieces.extend((at(src, b, r, c), ("prep", b), 64) for c in range(nc))
                prog.append(part(fwd_op, b, r, src, dst))

    def inv(b):
        for r in range(R):
            pieces.extend((at("z", b, r, c), ("m", b), 64) for c in range(nc))
            prog.append(part(inv_op, b, r))

    def run(then_wait=()):
        for step in prog:
            step()
        prog.clear(), pieces.clear(), marks.clear()
        cursor[0] = 0
        credit[0] = -256
        wait(then_wait)

    feed = [q_in(0), w1_in(0, 4 * FC, 0) + small_in, w1_in(4 * FC, F, 2) + q_in(1),
            q_in(2) + conv_in(0) + tables_in[:1], w2_in + conv_in(1) + q_in(3) + tables_in[1:],
            conv_in(2) + conv_in(3)]
    cuts = [pltpu.make_async_copy(q_hbm.at[0:16, 0:LANES], cut_buf.at[i], cut_sem.at[i]) for i in range(NCUT)]

    def params():
        prm[0:4, :] = shift_ref[...].astype(f32)
        prm[4:5, :] = sd_ref[...].astype(f32).reshape(1, D)
        prm[5:6, :] = b2_ref[...].astype(f32).reshape(1, D)
        b1s[...] = b1_ref[...].astype(f32).reshape(1, F)

    start(feed[0] + feed[1])
    for c in range(nc): st(at("k", c), jnp.zeros((8, LANES), u32))
    wait(feed[0])
    push(ln(arena, [0]))
    prog.append(part(need, ("ln", 0, 1)))
    run(feed[1])
    start(feed[2] + cuts)
    params()
    mm1(0, 0, 8)
    run(feed[2])
    start(feed[3])
    push(ln(ordered, [1], 160))
    mm1(0, 8)
    mm1(1, 0, 4)
    run(feed[3])
    start(feed[4])
    push(prep([0]))
    mm1(1, 4)
    push(ln(ordered, [2]))
    fwd(0)
    push(spectral(0))
    mm1(2)
    run(feed[4])
    start(feed[5])
    push(prep([1]))
    mm2(0, 0, 6)
    push(ln(ordered, [3]))
    fwd(1)
    push(spectral(1))
    mm1(3)
    mm2(0, 6, 8)
    run(feed[5])
    push(prep([2, 3]))
    mm2(0, 8)
    inv(0)
    mm2(1, 0, 3)
    fwd(2)
    mm2(1, 3, 6)
    run(cuts[0:1])
    push(spectral(2))
    fwd(3)
    mm2(1, 6)
    inv(1)
    mm2(2, 0, 2)
    run(cuts[1:2])
    push(spectral(3))
    mm2(2, 2)
    inv(2)
    mm2(3, 0, 2)
    inv(3)
    push(fin(0) + fin(1) + fin(2) + fin(3, 1))
    mm2(3, 2, fused=True)
    prog.append(part(need, ("fin", 3)))
    run()
    for b in range(nb):
        wait([out_copy(b, c) for c in range(nc)])


@jax.jit
def pallas_parallel_sum__ssm_conv_h3__dense_activation_gelu__prompt_kernel(
    A_q: jax.Array,
    A_k: jax.Array,
    A_v: jax.Array,
    A_shift_k: jax.Array,
    A_ssm_k: jax.Array,
    A_ssm_D: jax.Array,
    B_x: jax.Array,
    B_w1: jax.Array,
    B_b1: jax.Array,
    B_w2: jax.Array,
    B_b2: jax.Array,
):
    B, S, D = A_q.shape
    F = B_w1.shape[1]
    nc, nb = D // LANES, S // TB
    q, k, v = (a.reshape(S, D) for a in (A_q, A_k, A_v))
    hbm = pl.BlockSpec(memory_space=pltpu.HBM)
    out = pl.pallas_call(
        functools.partial(_kernel, nc=nc, nb=nb, D=D, F=F),
        in_specs=[pl.BlockSpec(memory_space=pltpu.SMEM)] + [hbm] * 12,
        out_specs=hbm,
        out_shape=jax.ShapeDtypeStruct((S, D), A_q.dtype),
        scratch_shapes=[
            pltpu.VMEM((4, D), bf16), pltpu.VMEM((D,), bf16), pltpu.VMEM((F,), bf16), pltpu.VMEM((D,), bf16),
            pltpu.VMEM(_FWD.shape, u32), pltpu.VMEM(_INV.shape, u32),
            pltpu.VMEM((2 * _layout(nb, nc, F)[1], LANES), bf16),
            [pltpu.VMEM((2 * R * SR + 8, D), f32) for _ in range(nb)],
            [pltpu.VMEM((2 * R * P + 8, D), f32) for _ in range(nb)],
            [pltpu.VMEM((nc, TB, LANES), bf16) for _ in range(nb)],
            pltpu.VMEM((8, D), f32),
            pltpu.VMEM((1, F), f32),
            [[pltpu.VMEM((P, F), u32) for _ in range(2)] for _ in range(nb)],
            pltpu.SemaphoreType.DMA((4, nb)),
            pltpu.SemaphoreType.DMA((6,)),
            pltpu.SemaphoreType.DMA((nb,)),
            pltpu.VMEM((NCUT, 16, LANES), bf16),
            pltpu.SemaphoreType.DMA((NCUT,)),
        ],
        compiler_params=pltpu.CompilerParams(vmem_limit_bytes=120 * 1024 * 1024),
    )(jnp.asarray(np.zeros((1,), np.int32)), q, k, v, A_ssm_k, B_w1.T, B_w2, A_shift_k.T, A_ssm_D, B_b1, B_b2,
      jnp.asarray(_FWD), jnp.asarray(_INV))
    return out.reshape(B, S, D)
```

```python
import functools

import numpy as np
import jax
import jax.numpy as jnp
import jax.experimental.pallas as pl
import jax.experimental.pallas.tpu as pltpu

R = 4
P = 128
H = P // 2
TB = R * P
NFFT = 2 * TB
LANES = 128
IM, SR = P + 8, 2 * P + 24
RG = 8
PR, LR, FR = 32, 32, 64
C_LN, C_PREP, C_FIN, C_M = 135, 115, 105, (124, 125, 125, 130)
LAG, TL, NCUT = 2, 2, 2
FC = 256


def _pack_rows(m):
    u = np.ascontiguousarray(m, np.float32).view(np.uint32).astype(np.uint64)
    h = ((u + 0x7FFF + ((u >> 16) & 1)) >> 16).astype(np.uint32)
    return h[..., 0::2, :] | (h[..., 1::2, :] << np.uint32(16))


def _dft_tables():
    g = np.concatenate([np.arange(0, P, 2), np.arange(1, P, 2)]).astype(np.float64)
    s = np.arange(P, dtype=np.float64)
    fwd, inv = [], []
    for r in range(R):
        th = 2.0 * np.pi * (g[:, None] + 0.5) * (R * s[None, :] + r) / NFFT
        fwd.append(np.concatenate([np.cos(th), -np.sin(th)], 0))
        inv.append(np.stack([np.cos(th).T, -np.sin(th).T], 2).reshape(P, 2 * P) * (2.0 / NFFT))
    return _pack_rows(np.stack(fwd)), _pack_rows(np.stack(inv))


_FWD, _INV = _dft_tables()
_GC = float(np.sqrt(2.0 / np.pi))
f32, bf16, u32 = jnp.float32, jnp.bfloat16, jnp.uint32


def _layout(nb, nc, F):
    spec = dict(q=(nb * nc, TB // 2), k=(nc, 8 + nb * TB // 2), v=(nb * nc, TB // 2), kt=(nb * nc, TB // 2),
                sk=(nb * R * nc, H),
                o=(nb * nc, TB // 2), w1=(nc, F // 2), w2=(nc, F // 2),
                xn=(nb * R * nc, H), xu=(nb * R * nc, H), xk=(nb * R * nc, H),
                u=((nb - 1) * R * nc, SR), kf=((nb - 1) * R * nc, SR), kp=((nb - 1) * R * nc, SR),
                z=(nb * R * nc, P + 8), tick=(1, 8))
    off, out = 0, {}
    for name, (n, rows) in spec.items():
        out[name] = (off, rows)
        off += n * rows
    return out, off


def _lo(w):
    return pltpu.bitcast(w << 16, f32)


def _hi(w):
    return pltpu.bitcast(w & np.uint32(0xFFFF0000), f32)


def _packed(x):
    return pltpu.bitcast(x.astype(bf16), u32)


def _pair(a, b):
    return pltpu.bitcast(pltpu.pack_elementwise([a, b], packed_dtype=bf16), u32)


def _kernel(zero_ref, q_hbm, k_hbm, v_hbm, sk_hbm, w1_hbm, w2_hbm,
            shift_hbm, sd_hbm, b1_hbm, b2_hbm, fwd_hbm, inv_hbm,
            o_hbm,
            shift_ref, sd_ref, b1_ref, b2_ref, fwd_ref, inv_ref,
            arena16, ebuf, fbuf, obuf, prm, b1s, hbuf, in_sem, w_sem, out_sem, cut_buf, cut_sem, *, nc, nb, D, F):
    lanes = [slice(c * LANES, (c + 1) * LANES) for c in range(nc)]
    lay, total = _layout(nb, nc, F)
    arena = arena16.bitcast(u32)
    zero = pl.multiple_of(zero_ref[0], 8)

    i0 = jnp.zeros((), jnp.int32)

    def rows(start, n):
        return pl.ds(pl.multiple_of(i0 + start, 8), n)

    def late(ref):
        return ref.at[pl.ds(zero, ref.shape[0]), :]

    ordered = late(arena)
    e_ord, f_ord = [late(r) for r in ebuf], [late(r) for r in fbuf]
    E_ROWS, F_ROWS = 2 * R * SR, 2 * R * P

    def at(name, *idx):
        n = 0
        for i in idx[:-1]:
            n = n * R + i
        return lay[name][0] + (n * nc + idx[-1]) * lay[name][1]

    def ld(row, n):
        return pltpu.bitcast(ordered[rows(row, n), :], f32)

    def st(row, val):
        arena[rows(row, val.shape[0]), :] = pltpu.bitcast(val, u32)

    def slab16(row, n):
        return arena16.at[2 * row:2 * (row + n), :]

    def wide(name, *idx):
        return jnp.concatenate([arena[rows(at(name, *idx, c), lay[name][1]), :] for c in range(nc)], axis=1)

    def cols_in(src, b, offs, sem):
        return [pltpu.make_async_copy(src.at[pl.ds(b * TB, TB), lanes[c]], slab16(offs[c], TB // 2), sem)
                for c in range(nc)]

    def conv_in(b):
        return (cols_in(k_hbm, b, [at("k", c) + 8 + b * TB // 2 for c in range(nc)], in_sem.at[0, b])
                + cols_in(v_hbm, b, [at("v", b, c) for c in range(nc)], in_sem.at[1, b])
                + [pltpu.make_async_copy(sk_hbm.at[lanes[c], pl.ds(b * TB + n * P, P)],
                                         slab16(at("sk", b, n, c), H), in_sem.at[2, b])
                   for c in range(nc) for n in range(R)])

    def q_in(b):
        return cols_in(q_hbm, b, [at("q", b, c) for c in range(nc)], in_sem.at[3, b])

    out_copies = []

    def out_copy(b, c, src):
        return pltpu.make_async_copy(slab16(at("o", b, c), TB // 2) if src is ordered else obuf.at[c, 0:TB, :],
                                     o_hbm.at[pl.ds(b * TB, TB), lanes[c]], out_sem.at[b])

    def w1_in(lo, hi, n):
        return [pltpu.make_async_copy(w1_hbm.at[lo:hi, lanes[c]], slab16(at("w1", c) + lo // 2, (hi - lo) // 2),
                                      w_sem.at[n]) for c in range(nc)]

    small_in = [pltpu.make_async_copy(src, dst, w_sem.at[3]) for src, dst in (
        (shift_hbm, shift_ref), (sd_hbm, sd_ref), (b1_hbm, b1_ref), (b2_hbm, b2_ref))]
    tables_in = [pltpu.make_async_copy(fwd_hbm, fwd_ref, w_sem.at[4]),
                 pltpu.make_async_copy(inv_hbm, inv_ref, w_sem.at[5])]
    w2_in = [pltpu.make_async_copy(w2_hbm.at[:, lanes[c]], slab16(at("w2", c), F // 2), w_sem.at[1])
             for c in range(nc)]

    def start(cs):
        for c in cs:
            c.start()

    def wait(cs):
        for c in cs:
            c.wait()

    def delayed(x):
        for _ in range(7):
            x = jnp.tanh(x)
        return x

    tiles = {}

    def t_load(b, c, n):
        w = pltpu.bitcast(ordered[rows(at("sk", b, n, c), H), :], bf16)
        tiles[b, c, n] = pltpu.bitcast(w.T, u32)

    def t_store(b, c, n):
        st(at("kt", b, c) + n * H, tiles.pop((b, c, n)))

    def prep_unit(b, j, c, s0):
        base = at("k", c) + 8 + b * TB // 2 + j + 2 * s0
        t = ordered[rows(at("k", c), 8), :]
        t = delayed(pltpu.bitcast(t, f32))

        wa = ordered[pl.ds(base - 2, PR, stride=2), :]
        wb = ordered[pl.ds(base - 1, PR, stride=2), :]
        wc = ordered[pl.ds(base, PR, stride=2), :]
        ks = [_hi(wa), _lo(wb), _hi(wb), _lo(wc), _hi(wc)]
        vw = ordered[pl.ds(at("v", b, c) + j + 2 * s0, PR, stride=2), :]
        vs = [_lo(vw), _hi(vw)]
        tw = ordered[pl.ds(at("kt", b, c) + j + 2 * s0, PR, stride=2), :]
        ts = [_lo(tw), _hi(tw)]
        for e in range(2):
            acc = ks[3 + e] * prm[0:1, lanes[c]]
            for i in range(1, 4):
                acc = acc + ks[3 + e - i] * prm[i:i + 1, lanes[c]]
            st(at("xu", b, 2 * j + e, c) + s0 // 2, _packed(acc * vs[e]))
            st(at("xk", b, 2 * j + e, c) + s0 // 2, _packed(ts[e]))
        st(at("tick", 0), t)

    def m_unit(b, g0, c):
        def cld(name, slot, m):
            row = at(name, slot, m, c) + g0
            return ld(row, RG), ld(row + IM, RG)

        def cst(name, m, vr, vi):
            row = at(name, b, m, c) + g0
            st(row, vr)
            st(row + IM, vi)

        def bfly(which):
            offs = [(which * R + r) * SR + g0 for r in range(R)]
            er = [e_ord[b][rows(o, RG), lanes[c]] for o in offs]
            ei = [e_ord[b][rows(o + IM, RG), lanes[c]] for o in offs]
            ar, ai = er[0] + er[2], ei[0] + ei[2]
            br, bi = er[0] - er[2], ei[0] - ei[2]
            cr, ci = er[1] + er[3], ei[1] + ei[3]
            dr, di = er[1] - er[3], ei[1] - ei[3]
            return ([ar + cr, br + di, ar - cr, br - di],
                    [ai + ci, bi - dr, ai - ci, bi + dr])

        tick = pltpu.roll(e_ord[b][rows(g0, RG), lanes[c]], 1, 1)
        ur, ui = bfly(0)
        kr, ki = bfly(1)
        if b == 0:
            kr = [x + prm[4:5, lanes[c]] for x in kr]
        keep = []
        for m in range(R):
            if b == 0:
                keep.append((kr[m], ki[m]))
            else:
                pr, pi = cld("kp", b - 1, m)
                keep.append((kr[m] - pi, ki[m] + pr) if g0 < P // 2 else (kr[m] + pi, ki[m] - pr))
        if b < nb - 1:
            for m in range(R):
                cst("kp", m, kr[m], ki[m])
                cst("u", m, ur[m], ui[m])
                cst("kf", m, *keep[m])
        else:
            st(at("tick", 0), keep[R - 1][1])
        yr, yi = [], []
        for m in range(R):
            accr = acci = None
            for jj in range(b + 1):
                a_r, a_i = (ur[m], ui[m]) if jj == b else cld("u", jj, m)
                b_r, b_i = keep[m] if jj == 0 else cld("kf", b - jj, m)
                pr_ = a_r * b_r - a_i * b_i
                pi_ = a_r * b_i + a_i * b_r
                accr = pr_ if accr is None else accr + pr_
                acci = pi_ if acci is None else acci + pi_
            yr.append(accr)
            yi.append(acci)
            if b >= 2 and m == 1:
                st(at("tick", 0), acci)
        ar, ai = yr[0] + yr[2], yi[0] + yi[2]
        br, bi = yr[0] - yr[2], yi[0] - yi[2]
        cr, ci = yr[1] + yr[3], yi[1] + yi[3]
        dr, di = yr[1] - yr[3], yi[1] - yi[3]
        zr = [ar + cr, br - di, ar - cr, br + di]
        zi = [ai + ci, bi + dr, ai - ci, bi - dr]
        for r in range(R):
            st(at("z", b, r, c) + g0, _pair(zr[r], zi[r]))
        ebuf[b][E_ROWS:E_ROWS + RG, 0:LANES] = tick
        st(at("tick", 0), tick)

    def q_words(src, b, j, c):
        return src[pl.ds(at("q", b, c) + j, P, stride=2), :]

    def ln_rows(src, b, r, s0):
        return jnp.concatenate([(_lo, _hi)[r % 2](src[pl.ds(at("q", b, c) + r // 2 + 2 * s0, LR, stride=2), :])
                                for c in range(nc)], axis=1)

    mean, rstd = {}, {}

    def ln_mean(src, key):
        mean[key] = jnp.mean(ln_rows(src, *key), axis=-1, keepdims=True)

    def ln_rstd(src, key):
        xc = ln_rows(src, *key) - mean[key]
        rstd[key] = jax.lax.rsqrt(jnp.mean(xc * xc, axis=-1, keepdims=True) + 1e-5)

    def ln_store(src, key):
        b, r, s0 = key
        xn = _packed((ln_rows(src, *key) - mean.pop(key)) * rstd.pop(key))
        for c in range(nc):
            st(at("xn", b, r, c) + s0 // 2, xn[:, lanes[c]])

    def ln_unit(src, keys, n):
        for stage, fn in enumerate((ln_mean, ln_rstd, ln_store)):
            if 0 <= n - stage < len(keys):
                fn(src, keys[n - stage])

    def emit_out(src, fsrc, b, j, c, o, s0=0):
        n = o[0].shape[0]
        outs = []
        for e in range(2):
            r = 2 * j + e
            xn = pltpu.bitcast(src[rows(at("xn", b, r, c) + s0 // 2, n // 2), :], bf16).astype(f32)
            outs.append(o[e] + xn * fsrc[(R + r) * P + s0:(R + r) * P + s0 + n, lanes[c]])
        if src is ordered:
            arena[pl.ds(at("o", b, c) + j + 2 * s0, n, stride=2), :] = _pair(*outs)
        else:
            obuf.at[c].bitcast(u32)[pl.ds(j + 2 * s0, n, stride=2), :] = _pair(*outs)
        if j == 1 and s0 + n == P:
            out_copies.append(out_copy(b, c, src))
            out_copies[-1].start()

    def fin_gate(b):
        fbuf[b][F_ROWS:F_ROWS + 8, 0:LANES] = ld(at("k", 0), 8)

    def fin_unit(b, j, c, s0):
        o = [f_ord[b][(2 * j + e) * P + s0:(2 * j + e) * P + s0 + FR, lanes[c]] for e in range(2)]
        tick = delayed(f_ord[b][0:8, lanes[c]])
        emit_out(ordered, f_ord[b], b, j, c, o, s0)
        fbuf[b][F_ROWS:F_ROWS + 8, 0:LANES] = tick
        st(at("tick", 0), tick)

    queue = []
    credit = [0]

    def fill(cycles):
        credit[0] += cycles
        while queue and credit[0] >= queue[0][2]:
            _, fn, cost = queue.pop(0)
            credit[0] -= cost
            fn()
        if not queue:
            credit[0] = min(credit[0], 128)

    def need(tag):
        while any(t == tag for t, _, _ in queue):
            queue.pop(0)[1]()

    marks = {}
    pieces = []
    cursor = [0]

    def weights(row, n):
        i = cursor[0]
        assert pieces[i][0] == row
        cursor[0] += 1
        for p in range(len(marks), min(i + 1 + LAG, len(pieces))):
            need(pieces[p][1])
            marks[p] = ordered[rows(pieces[p][0], 8), :]
            fill(pieces[p][2])
        return pltpu.bitcast(jnp.concatenate([marks[i], arena[rows(row + 8, n - 8), :]], axis=0), bf16)

    def mm1_op(b, j, s0, s1):
        need(("ln", b, j))
        w = jnp.concatenate([weights(at("w1", c) + s0 // 2, (s1 - s0) // 2) for c in range(nc)], axis=1)
        x = pltpu.bitcast(jnp.concatenate([wide("xn", b, 2 * j), wide("xn", b, 2 * j + 1)], axis=0), bf16)
        h = jax.lax.dot_general(x, w, (((1,), (1,)), ((), ())), preferred_element_type=f32) + b1s[0:1, s0:s1]
        u = h * (h * h * (_GC * 0.044715) + _GC)
        hh = 0.5 * h
        hbuf[b][j][:, s0:s1] = _packed(hh * jnp.tanh(u) + hh)

    def mm2_op(b, j, c, fused):
        w = jnp.concatenate([weights(at("w2", c) + s0 // 2, (min(s0 + FC, F) - s0) // 2)
                             for s0 in range(0, F, FC)], axis=0)
        mlp = jnp.dot(pltpu.bitcast(hbuf[b][j][...], bf16), w, preferred_element_type=f32)
        mlp = [mlp[0:P], mlp[P:2 * P]]
        qw = q_words(arena, b, j, c)
        o = [mlp[0] + prm[5:6, lanes[c]] + _lo(qw), mlp[1] + prm[5:6, lanes[c]] + _hi(qw)]
        if fused:
            emit_out(arena, fbuf[b], b, j, c, o)
        else:
            for e in range(2):
                fbuf[b][(2 * j + e) * P:(2 * j + e + 1) * P, lanes[c]] = o[e]

    def fwd_op(b, r, src, dst):
        e = jnp.dot(pltpu.bitcast(fwd_ref[r], bf16), jnp.concatenate([weights(at(src, b, r, c), H) for c in range(nc)], axis=1),
                    preferred_element_type=f32)
        row = (dst * R + r) * SR
        ebuf[b][row:row + P, :] = e[0:P]
        ebuf[b][row + IM:row + IM + P, :] = e[P:2 * P]

    def inv_op(b, r):
        y = jnp.dot(pltpu.bitcast(inv_ref[r], bf16), jnp.concatenate([weights(at("z", b, r, c), P) for c in range(nc)], axis=1),
                    preferred_element_type=f32)
        fbuf[b][(R + r) * P:(R + r + 1) * P, :] = y

    part = functools.partial

    prog = []

    def push(units):
        prog.append(part(queue.extend, units))

    def ln(src, blocks, cost=C_LN):
        keys = [(b, r, s0) for b in blocks for r in range(R) for s0 in range(0, P, LR)]
        tag = lambda n: ("ln", keys[n][0], keys[n][1] // 2)
        return [(tag(max(n - 2, 0)), part(ln_unit, src, keys, n), cost) for n in range(len(keys) + 2)]

    def prep(blocks):
        ts = [(b, c, n) for b in blocks for c in range(nc) for n in range(R)]
        out = []
        for i in range(-TL - 1, len(ts)):
            tag = ("prep", ts[max(i, 0)][0])
            if i + TL + 1 < len(ts):
                out.append((tag, part(t_load, *ts[i + TL + 1]), 0))
            for j in range(2):
                if j == 1 and -1 <= i < len(ts) - 1:
                    out.append((tag, part(t_store, *ts[i + 1]), 0))
                if i >= 0:
                    out.append((tag, part(prep_unit, ts[i][0], j, ts[i][1], ts[i][2] * PR), C_PREP))
                else:
                    out.append((tag, lambda: None, C_PREP))
        return out

    def spectral(b):
        return [(("m", b), part(m_unit, b, g0, c), C_M[b]) for g0 in range(0, P, RG) for c in range(nc)]

    def fin(b, n=nc):
        return [(("fin", b), part(fin_gate, b), 0)] + [
            (("fin", b), part(fin_unit, b, j, c, s0), C_FIN)
            for c in range(n) for j in range(2) for s0 in range(0, P, FR)]

    def mix(main, extra):
        out = []
        for i, u in enumerate(main):
            out += extra[i * len(extra) // len(main):(i + 1) * len(extra) // len(main)] + [u]
        return out

    def mm1(b, lo=0, hi=None):
        for s0, j in [(s0, j) for s0 in range(0, F, FC) for j in range(2)][lo:hi]:
            s1 = min(s0 + FC, F)
            pieces.extend((at("w1", c) + s0 // 2, None, 64 * pl.cdiv(s1 - s0, LANES)) for c in range(nc))
            prog.append(part(mm1_op, b, j, s0, s1))

    def mm2(b, lo=0, hi=None, fused=False):
        for c, j in [(c, j) for c in range(nc) for j in range(2)][lo:hi]:
            pieces.extend((at("w2", c) + s0 // 2, None, 128) for s0 in range(0, F, FC))
            prog.append(part(mm2_op, b, j, c, fused))

    def fwd(b):
        for r in range(R):
            for dst, src in enumerate(("xu", "xk")):
                pieces.extend((at(src, b, r, c), ("prep", b), 64) for c in range(nc))
                prog.append(part(fwd_op, b, r, src, dst))

    def inv(b):
        for r in range(R):
            pieces.extend((at("z", b, r, c), ("m", b), 64) for c in range(nc))
            prog.append(part(inv_op, b, r))

    def run(then_wait=()):
        for step in prog:
            step()
        prog.clear(), pieces.clear(), marks.clear()
        cursor[0] = 0
        credit[0] = -256
        wait(then_wait)

    feed = [q_in(0), q_in(1), w1_in(0, 2 * FC, 0) + small_in, w1_in(2 * FC, F, 2),
            q_in(2) + conv_in(0) + tables_in[:1], w2_in + conv_in(1) + q_in(3) + tables_in[1:],
            conv_in(2) + conv_in(3)]
    cuts = [pltpu.make_async_copy(q_hbm.at[0:16, 0:LANES], cut_buf.at[i], cut_sem.at[i]) for i in range(NCUT)]

    def params():
        prm[0:4, :] = shift_ref[...].astype(f32)
        prm[4:5, :] = sd_ref[...].astype(f32).reshape(1, D)
        prm[5:6, :] = b2_ref[...].astype(f32).reshape(1, D)
        b1s[...] = b1_ref[...].astype(f32).reshape(1, F)

    start(feed[0] + feed[1])
    for c in range(nc): st(at("k", c), jnp.zeros((8, LANES), u32))
    wait(feed[0])
    start(feed[2])
    push(ln(arena, [0]))
    prog.append(part(need, ("ln", 0, 1)))
    run(feed[1])
    push(ln(arena, [1]))
    prog.append(part(need, ("ln", 1, 1)))
    run(feed[2])
    start(feed[3] + cuts)
    params()
    mm1(0, 0, 4)
    mm1(1, 0, 4)
    run(feed[3])
    start(feed[4])
    mm1(0, 4)
    mm1(1, 4, 6)
    run(feed[4])
    start(feed[5])
    push(prep([0]))
    mm1(1, 6)
    push(ln(ordered, [2]))
    fwd(0)
    push(spectral(0))
    mm1(2)
    run(feed[5])
    start(feed[6])
    push(prep([1]))
    mm2(0, 0, 6)
    push(ln(ordered, [3]))
    fwd(1)
    push(spectral(1))
    mm1(3)
    mm2(0, 6, 8)
    run(feed[6])
    push(prep([2, 3]))
    mm2(0, 8)
    inv(0)
    mm2(1, 0, 3)
    fwd(2)
    mm2(1, 3, 6)
    run(cuts[0:1])
    push(spectral(2))
    fwd(3)
    mm2(1, 6)
    inv(1)
    mm2(2, 0, 2)
    run(cuts[1:2])
    push(spectral(3))
    mm2(2, 2)
    inv(2)
    mm2(3, 0, 2)
    inv(3)
    push(fin(0) + fin(1) + fin(2) + fin(3, 1))
    mm2(3, 2, fused=True)
    prog.append(part(need, ("fin", 3)))
    run()
    wait(out_copies)


@jax.jit
def pallas_parallel_sum__ssm_conv_h3__dense_activation_gelu__prompt_kernel(
    A_q: jax.Array,
    A_k: jax.Array,
    A_v: jax.Array,
    A_shift_k: jax.Array,
    A_ssm_k: jax.Array,
    A_ssm_D: jax.Array,
    B_x: jax.Array,
    B_w1: jax.Array,
    B_b1: jax.Array,
    B_w2: jax.Array,
    B_b2: jax.Array,
):
    B, S, D = A_q.shape
    F = B_w1.shape[1]
    nc, nb = D // LANES, S // TB
    q, k, v = (a.reshape(S, D) for a in (A_q, A_k, A_v))
    hbm = pl.BlockSpec(memory_space=pltpu.HBM)
    out = pl.pallas_call(
        functools.partial(_kernel, nc=nc, nb=nb, D=D, F=F),
        in_specs=[pl.BlockSpec(memory_space=pltpu.SMEM)] + [hbm] * 12,
        out_specs=hbm,
        out_shape=jax.ShapeDtypeStruct((S, D), A_q.dtype),
        scratch_shapes=[
            pltpu.VMEM((4, D), bf16), pltpu.VMEM((D,), bf16), pltpu.VMEM((F,), bf16), pltpu.VMEM((D,), bf16),
            pltpu.VMEM(_FWD.shape, u32), pltpu.VMEM(_INV.shape, u32),
            pltpu.VMEM((2 * _layout(nb, nc, F)[1], LANES), bf16),
            [pltpu.VMEM((2 * R * SR + 8, D), f32) for _ in range(nb)],
            [pltpu.VMEM((2 * R * P + 8, D), f32) for _ in range(nb)],
            pltpu.VMEM((nc, TB + 16, LANES), bf16),
            pltpu.VMEM((8, D), f32),
            pltpu.VMEM((1, F), f32),
            [[pltpu.VMEM((P, F), u32) for _ in range(2)] for _ in range(nb)],
            pltpu.SemaphoreType.DMA((4, nb)),
            pltpu.SemaphoreType.DMA((6,)),
            pltpu.SemaphoreType.DMA((nb,)),
            pltpu.VMEM((NCUT, 16, LANES), bf16),
            pltpu.SemaphoreType.DMA((NCUT,)),
        ],
        compiler_params=pltpu.CompilerParams(vmem_limit_bytes=120 * 1024 * 1024),
    )(jnp.asarray(np.zeros((1,), np.int32)), q, k, v, A_ssm_k, B_w1.T, B_w2, A_shift_k.T, A_ssm_D, B_b1, B_b2,
      jnp.asarray(_FWD), jnp.asarray(_INV))
    return out.reshape(B, S, D)
```

```python
import functools

import numpy as np
import jax
import jax.numpy as jnp
import jax.experimental.pallas as pl
import jax.experimental.pallas.tpu as pltpu

R = 4
P = 128
H = P // 2
TB = R * P
NFFT = 2 * TB
LANES = 128
IM, SR = P + 8, 2 * P + 24
RG = 8
PT = 5
PR, LR, FR = 16, 32, 64
C_LN, C_PREP, C_FIN, C_M = 135, 72, 105, (132, 134, 125, 130)
LAG, TL, NCUT = 2, 2, 2
FC = 256


def _pack_rows(m):
    u = np.ascontiguousarray(m, np.float32).view(np.uint32).astype(np.uint64)
    h = ((u + 0x7FFF + ((u >> 16) & 1)) >> 16).astype(np.uint32)
    return h[..., 0::2, :] | (h[..., 1::2, :] << np.uint32(16))


def _dft_tables():
    g = np.concatenate([np.arange(0, P, 2), np.arange(1, P, 2)]).astype(np.float64)
    s = np.arange(P, dtype=np.float64)
    fwd, inv = [], []
    for r in range(R):
        th = 2.0 * np.pi * (g[:, None] + 0.5) * (R * s[None, :] + r) / NFFT
        fwd.append(np.concatenate([np.cos(th), -np.sin(th)], 0))
        inv.append(np.stack([np.cos(th).T, -np.sin(th).T], 2).reshape(P, 2 * P) * (2.0 / NFFT))
    return _pack_rows(np.stack(fwd)), _pack_rows(np.stack(inv))


_FWD, _INV = _dft_tables()
_GC = float(np.sqrt(2.0 / np.pi))
f32, bf16, u32 = jnp.float32, jnp.bfloat16, jnp.uint32


def _layout(nb, nc, F):
    spec = dict(q=(nb * nc, TB // 2), k=(nc, 8 + nb * TB // 2), v=(nb * nc, TB // 2), kt=(nb * nc, TB // 2),
                sk=(nb * R * nc, H),
                o=(nb * nc, TB // 2), w1=(nc, F // 2), w2=(nc, F // 2),
                xn=(nb * R * nc, H), xu=(nb * R * nc, H), xk=(nb * R * nc, H),
                u=((nb - 1) * R * nc, SR), kf=((nb - 1) * R * nc, SR), kp=((nb - 1) * R * nc, SR),
                z=(nb * R * nc, P + 8), tick=(1, 8))
    off, out = 0, {}
    for name, (n, rows) in spec.items():
        out[name] = (off, rows)
        off += n * rows
    return out, off


def _lo(w):
    return pltpu.bitcast(w << 16, f32)


def _hi(w):
    return pltpu.bitcast(w & np.uint32(0xFFFF0000), f32)


def _packed(x):
    return pltpu.bitcast(x.astype(bf16), u32)


def _pair(a, b):
    return pltpu.bitcast(pltpu.pack_elementwise([a, b], packed_dtype=bf16), u32)


def _kernel(zero_ref, q_hbm, k_hbm, v_hbm, sk_hbm, w1_hbm, w2_hbm,
            shift_hbm, sd_hbm, b1_hbm, b2_hbm, fwd_hbm, inv_hbm,
            o_hbm,
            shift_ref, sd_ref, b1_ref, b2_ref, fwd_ref, inv_ref,
            arena16, ebuf, fbuf, obuf, prm, b1s, hbuf, in_sem, w_sem, out_sem, cut_buf, cut_sem, *, nc, nb, D, F):
    lanes = [slice(c * LANES, (c + 1) * LANES) for c in range(nc)]
    lay, total = _layout(nb, nc, F)
    arena = arena16.bitcast(u32)
    zero = pl.multiple_of(zero_ref[0], 8)

    i0 = jnp.zeros((), jnp.int32)

    def rows(start, n):
        return pl.ds(pl.multiple_of(i0 + start, 8), n)

    def late(ref):
        return ref.at[pl.ds(zero, ref.shape[0]), :]

    ordered = late(arena)
    e_ord, f_ord = [late(r) for r in ebuf], [late(r) for r in fbuf]
    E_ROWS, F_ROWS = 2 * R * SR, 2 * R * P

    def at(name, *idx):
        n = 0
        for i in idx[:-1]:
            n = n * R + i
        return lay[name][0] + (n * nc + idx[-1]) * lay[name][1]

    def ld(row, n):
        return pltpu.bitcast(ordered[rows(row, n), :], f32)

    def st(row, val):
        arena[rows(row, val.shape[0]), :] = pltpu.bitcast(val, u32)

    def slab16(row, n):
        return arena16.at[2 * row:2 * (row + n), :]

    def wide(name, *idx):
        return jnp.concatenate([arena[rows(at(name, *idx, c), lay[name][1]), :] for c in range(nc)], axis=1)

    def cols_in(src, b, offs, sem):
        return [pltpu.make_async_copy(src.at[pl.ds(b * TB, TB), lanes[c]], slab16(offs[c], TB // 2), sem)
                for c in range(nc)]

    def conv_in(b):
        return (cols_in(k_hbm, b, [at("k", c) + 8 + b * TB // 2 for c in range(nc)], in_sem.at[0, b])
                + cols_in(v_hbm, b, [at("v", b, c) for c in range(nc)], in_sem.at[1, b])
                + [pltpu.make_async_copy(sk_hbm.at[lanes[c], pl.ds(b * TB + n * P, P)],
                                         slab16(at("sk", b, n, c), H), in_sem.at[2, b])
                   for c in range(nc) for n in range(R)])

    def q_in(b):
        return cols_in(q_hbm, b, [at("q", b, c) for c in range(nc)], in_sem.at[3, b])

    out_copies = []

    def out_copy(b, c, src):
        return pltpu.make_async_copy(slab16(at("o", b, c), TB // 2) if src is ordered else obuf.at[c, 0:TB, :],
                                     o_hbm.at[pl.ds(b * TB, TB), lanes[c]], out_sem.at[b])

    def w1_in(lo, hi, n):
        return [pltpu.make_async_copy(w1_hbm.at[lo:hi, lanes[c]], slab16(at("w1", c) + lo // 2, (hi - lo) // 2),
                                      w_sem.at[n]) for c in range(nc)]

    small_in = [pltpu.make_async_copy(src, dst, w_sem.at[3]) for src, dst in (
        (shift_hbm, shift_ref), (sd_hbm, sd_ref), (b1_hbm, b1_ref), (b2_hbm, b2_ref))]
    tables_in = [pltpu.make_async_copy(fwd_hbm, fwd_ref, w_sem.at[4]),
                 pltpu.make_async_copy(inv_hbm, inv_ref, w_sem.at[5])]
    w2_in = [pltpu.make_async_copy(w2_hbm.at[:, lanes[c]], slab16(at("w2", c), F // 2), w_sem.at[1])
             for c in range(nc)]

    def start(cs):
        for c in cs:
            c.start()

    def wait(cs):
        for c in cs:
            c.wait()

    def delayed(x, n):
        for _ in range(n):
            x = jnp.tanh(x)
        return x

    tiles = {}

    def t_load(b, c, n):
        w = pltpu.bitcast(ordered[rows(at("sk", b, n, c), H), :], bf16)
        tiles[b, c, n] = pltpu.bitcast(w.T, u32)

    def t_store(b, c, n):
        st(at("kt", b, c) + n * H, tiles.pop((b, c, n)))

    def prep_unit(b, j, c, s0):
        base = at("k", c) + 8 + b * TB // 2 + j + 2 * s0
        t = ordered[rows(at("k", c), 8), :]
        t = delayed(pltpu.bitcast(t, f32), PT)

        wa = ordered[pl.ds(base - 2, PR, stride=2), :]
        wb = ordered[pl.ds(base - 1, PR, stride=2), :]
        wc = ordered[pl.ds(base, PR, stride=2), :]
        ks = [_hi(wa), _lo(wb), _hi(wb), _lo(wc), _hi(wc)]
        vw = ordered[pl.ds(at("v", b, c) + j + 2 * s0, PR, stride=2), :]
        vs = [_lo(vw), _hi(vw)]
        tw = ordered[pl.ds(at("kt", b, c) + j + 2 * s0, PR, stride=2), :]
        ts = [_lo(tw), _hi(tw)]
        for e in range(2):
            acc = ks[3 + e] * prm[0:1, lanes[c]]
            for i in range(1, 4):
                acc = acc + ks[3 + e - i] * prm[i:i + 1, lanes[c]]
            st(at("xu", b, 2 * j + e, c) + s0 // 2, _packed(acc * vs[e]))
            st(at("xk", b, 2 * j + e, c) + s0 // 2, _packed(ts[e]))
        st(at("tick", 0), t)

    def m_unit(b, g0, c):
        def cld(name, slot, m):
            row = at(name, slot, m, c) + g0
            return ld(row, RG), ld(row + IM, RG)

        def cst(name, m, vr, vi):
            row = at(name, b, m, c) + g0
            st(row, vr)
            st(row + IM, vi)

        def bfly(which):
            offs = [(which * R + r) * SR + g0 for r in range(R)]
            er = [e_ord[b][rows(o, RG), lanes[c]] for o in offs]
            ei = [e_ord[b][rows(o + IM, RG), lanes[c]] for o in offs]
            ar, ai = er[0] + er[2], ei[0] + ei[2]
            br, bi = er[0] - er[2], ei[0] - ei[2]
            cr, ci = er[1] + er[3], ei[1] + ei[3]
            dr, di = er[1] - er[3], ei[1] - ei[3]
            return ([ar + cr, br + di, ar - cr, br - di],
                    [ai + ci, bi - dr, ai - ci, bi + dr])

        tick = pltpu.roll(e_ord[b][rows(g0, RG), lanes[c]], 1, 1)
        ur, ui = bfly(0)
        kr, ki = bfly(1)
        if b == 0:
            kr = [x + prm[4:5, lanes[c]] for x in kr]
        keep = []
        for m in range(R):
            if b == 0:
                keep.append((kr[m], ki[m]))
            else:
                pr, pi = cld("kp", b - 1, m)
                keep.append((kr[m] - pi, ki[m] + pr) if g0 < P // 2 else (kr[m] + pi, ki[m] - pr))
        if b < nb - 1:
            for m in range(R):
                cst("kp", m, kr[m], ki[m])
                cst("u", m, ur[m], ui[m])
                cst("kf", m, *keep[m])
        else:
            st(at("tick", 0), keep[R - 1][1])
        yr, yi = [], []
        for m in range(R):
            accr = acci = None
            for jj in range(b + 1):
                a_r, a_i = (ur[m], ui[m]) if jj == b else cld("u", jj, m)
                b_r, b_i = keep[m] if jj == 0 else cld("kf", b - jj, m)
                pr_ = a_r * b_r - a_i * b_i
                pi_ = a_r * b_i + a_i * b_r
                accr = pr_ if accr is None else accr + pr_
                acci = pi_ if acci is None else acci + pi_
            yr.append(accr)
            yi.append(acci)
            if b >= 2 and m == 1:
                st(at("tick", 0), acci)
        ar, ai = yr[0] + yr[2], yi[0] + yi[2]
        br, bi = yr[0] - yr[2], yi[0] - yi[2]
        cr, ci = yr[1] + yr[3], yi[1] + yi[3]
        dr, di = yr[1] - yr[3], yi[1] - yi[3]
        zr = [ar + cr, br - di, ar - cr, br + di]
        zi = [ai + ci, bi + dr, ai - ci, bi - dr]
        for r in range(R):
            st(at("z", b, r, c) + g0, _pair(zr[r], zi[r]))
        ebuf[b][E_ROWS:E_ROWS + RG, 0:LANES] = tick
        st(at("tick", 0), tick)

    def q_words(src, b, j, c):
        return src[pl.ds(at("q", b, c) + j, P, stride=2), :]

    def ln_rows(src, b, r, s0):
        return jnp.concatenate([(_lo, _hi)[r % 2](src[pl.ds(at("q", b, c) + r // 2 + 2 * s0, LR, stride=2), :])
                                for c in range(nc)], axis=1)

    mean, rstd = {}, {}

    def ln_mean(src, key):
        mean[key] = jnp.mean(ln_rows(src, *key), axis=-1, keepdims=True)

    def ln_rstd(src, key):
        xc = ln_rows(src, *key) - mean[key]
        rstd[key] = jax.lax.rsqrt(jnp.mean(xc * xc, axis=-1, keepdims=True) + 1e-5)

    def ln_store(src, key):
        b, r, s0 = key
        xn = _packed((ln_rows(src, *key) - mean.pop(key)) * rstd.pop(key))
        for c in range(nc):
            st(at("xn", b, r, c) + s0 // 2, xn[:, lanes[c]])

    def ln_unit(src, keys, n):
        for stage, fn in enumerate((ln_mean, ln_rstd, ln_store)):
            if 0 <= n - stage < len(keys):
                fn(src, keys[n - stage])

    def emit_out(src, fsrc, b, j, c, o, s0=0):
        n = o[0].shape[0]
        outs = []
        for e in range(2):
            r = 2 * j + e
            xn = pltpu.bitcast(src[rows(at("xn", b, r, c) + s0 // 2, n // 2), :], bf16).astype(f32)
            outs.append(o[e] + xn * fsrc[(R + r) * P + s0:(R + r) * P + s0 + n, lanes[c]])
        if src is ordered:
            arena[pl.ds(at("o", b, c) + j + 2 * s0, n, stride=2), :] = _pair(*outs)
        else:
            obuf.at[c].bitcast(u32)[pl.ds(j + 2 * s0, n, stride=2), :] = _pair(*outs)
        if j == 1 and s0 + n == P:
            out_copies.append(out_copy(b, c, src))
            out_copies[-1].start()

    def fin_gate(b):
        fbuf[b][F_ROWS:F_ROWS + 8, 0:LANES] = ld(at("k", 0), 8)

    def fin_unit(b, j, c, s0):
        o = [f_ord[b][(2 * j + e) * P + s0:(2 * j + e) * P + s0 + FR, lanes[c]] for e in range(2)]
        tick = delayed(f_ord[b][0:8, lanes[c]], 7)
        emit_out(ordered, f_ord[b], b, j, c, o, s0)
        fbuf[b][F_ROWS:F_ROWS + 8, 0:LANES] = tick
        st(at("tick", 0), tick)

    queue = []
    credit = [0]

    def fill(cycles):
        credit[0] += cycles
        while queue and credit[0] >= queue[0][2]:
            _, fn, cost = queue.pop(0)
            credit[0] -= cost
            fn()
        if not queue:
            credit[0] = min(credit[0], 128)

    def need(tag):
        while any(t == tag for t, _, _ in queue):
            queue.pop(0)[1]()

    marks = {}
    pieces = []
    cursor = [0]

    def weights(row, n):
        i = cursor[0]
        assert pieces[i][0] == row
        cursor[0] += 1
        for p in range(len(marks), min(i + 1 + LAG, len(pieces))):
            need(pieces[p][1])
            marks[p] = ordered[rows(pieces[p][0], 8), :]
            fill(pieces[p][2])
        return pltpu.bitcast(jnp.concatenate([marks[i], arena[rows(row + 8, n - 8), :]], axis=0), bf16)

    def mm1_op(b, j, s0, s1):
        need(("ln", b, j))
        w = jnp.concatenate([weights(at("w1", c) + s0 // 2, (s1 - s0) // 2) for c in range(nc)], axis=1)
        x = pltpu.bitcast(jnp.concatenate([wide("xn", b, 2 * j), wide("xn", b, 2 * j + 1)], axis=0), bf16)
        h = jax.lax.dot_general(x, w, (((1,), (1,)), ((), ())), preferred_element_type=f32) + b1s[0:1, s0:s1]
        u = h * (h * h * (_GC * 0.044715) + _GC)
        hh = 0.5 * h
        hbuf[b][j][:, s0:s1] = _packed(hh * jnp.tanh(u) + hh)

    def mm2_op(b, j, c, fused):
        w = jnp.concatenate([weights(at("w2", c) + s0 // 2, (min(s0 + FC, F) - s0) // 2)
                             for s0 in range(0, F, FC)], axis=0)
        mlp = jnp.dot(pltpu.bitcast(hbuf[b][j][...], bf16), w, preferred_element_type=f32)
        mlp = [mlp[0:P], mlp[P:2 * P]]
        qw = q_words(arena, b, j, c)
        o = [mlp[0] + prm[5:6, lanes[c]] + _lo(qw), mlp[1] + prm[5:6, lanes[c]] + _hi(qw)]
        if fused:
            emit_out(arena, fbuf[b], b, j, c, o)
        else:
            for e in range(2):
                fbuf[b][(2 * j + e) * P:(2 * j + e + 1) * P, lanes[c]] = o[e]

    def fwd_op(b, r, src, dst):
        e = jnp.dot(pltpu.bitcast(fwd_ref[r], bf16), jnp.concatenate([weights(at(src, b, r, c), H) for c in range(nc)], axis=1),
                    preferred_element_type=f32)
        row = (dst * R + r) * SR
        ebuf[b][row:row + P, :] = e[0:P]
        ebuf[b][row + IM:row + IM + P, :] = e[P:2 * P]

    def inv_op(b, r):
        y = jnp.dot(pltpu.bitcast(inv_ref[r], bf16), jnp.concatenate([weights(at("z", b, r, c), P) for c in range(nc)], axis=1),
                    preferred_element_type=f32)
        fbuf[b][(R + r) * P:(R + r + 1) * P, :] = y

    part = functools.partial

    prog = []

    def push(units):
        prog.append(part(queue.extend, units))

    def ln(src, blocks, cost=C_LN):
        keys = [(b, r, s0) for b in blocks for r in range(R) for s0 in range(0, P, LR)]
        tag = lambda n: ("ln", keys[n][0], keys[n][1] // 2)
        return [(tag(max(n - 2, 0)), part(ln_unit, src, keys, n), cost) for n in range(len(keys) + 2)]

    def prep(blocks):
        ts = [(b, c, n) for b in blocks for c in range(nc) for n in range(R)]
        lead, out = [], []
        for i in range(-TL - 1, len(ts)):
            tag, dst = ("prep", ts[max(i, 0)][0]), lead if i < 0 else out
            if i + TL + 1 < len(ts):
                dst.append((tag, part(t_load, *ts[i + TL + 1]), 0))
            for j in range(2):
                if j == 1 and -1 <= i < len(ts) - 1:
                    dst.append((tag, part(t_store, *ts[i + 1]), 0))
                if i >= 0:
                    b, c, n = ts[i]
                    dst += [(tag, part(prep_unit, b, j, c, s0), C_PREP)
                            for s0 in range(n * P // R, (n + 1) * P // R, PR)]

        def enqueue():
            n = 2 * TL + 2
            tail = queue[-n:]
            tail += [(lead[0][0], lambda: None, C_LN)] * (n - len(tail))
            queue[-n:] = mix(tail, lead) + out

        prog.append(enqueue)

    def spectral(b):
        return [(("m", b), part(m_unit, b, g0, c), C_M[b]) for g0 in range(0, P, RG) for c in range(nc)]

    def fin(b, n=nc):
        return [(("fin", b), part(fin_gate, b), 0)] + [
            (("fin", b), part(fin_unit, b, j, c, s0), C_FIN)
            for c in range(n) for j in range(2) for s0 in range(0, P, FR)]

    def mix(main, extra):
        out = []
        for i, u in enumerate(main):
            out += extra[i * len(extra) // len(main):(i + 1) * len(extra) // len(main)] + [u]
        return out

    def mm1(b, lo=0, hi=None):
        for s0, j in [(s0, j) for s0 in range(0, F, FC) for j in range(2)][lo:hi]:
            s1 = min(s0 + FC, F)
            pieces.extend((at("w1", c) + s0 // 2, None, 64 * pl.cdiv(s1 - s0, LANES)) for c in range(nc))
            prog.append(part(mm1_op, b, j, s0, s1))

    def mm2(b, lo=0, hi=None, fused=False):
        for c, j in [(c, j) for c in range(nc) for j in range(2)][lo:hi]:
            pieces.extend((at("w2", c) + s0 // 2, None, 128) for s0 in range(0, F, FC))
            prog.append(part(mm2_op, b, j, c, fused))

    def fwd(b):
        for r in range(R):
            for dst, src in enumerate(("xu", "xk")):
                pieces.extend((at(src, b, r, c), ("prep", b), 64) for c in range(nc))
                prog.append(part(fwd_op, b, r, src, dst))

    def inv(b):
        for r in range(R):
            pieces.extend((at("z", b, r, c), ("m", b), 64) for c in range(nc))
            prog.append(part(inv_op, b, r))

    def run(then_wait=()):
        for step in prog:
            step()
        prog.clear(), pieces.clear(), marks.clear()
        cursor[0] = 0
        credit[0] = -256
        wait(then_wait)

    feed = [q_in(0), q_in(1), w1_in(0, 2 * FC, 0) + small_in, w1_in(2 * FC, F, 2),
            q_in(2) + conv_in(0) + tables_in[:1], w2_in + conv_in(1) + q_in(3) + tables_in[1:],
            conv_in(2) + conv_in(3)]
    cuts = [pltpu.make_async_copy(q_hbm.at[0:16, 0:LANES], cut_buf.at[i], cut_sem.at[i]) for i in range(NCUT)]

    def params():
        prm[0:4, :] = shift_ref[...].astype(f32)
        prm[4:5, :] = sd_ref[...].astype(f32).reshape(1, D)
        prm[5:6, :] = b2_ref[...].astype(f32).reshape(1, D)
        b1s[...] = b1_ref[...].astype(f32).reshape(1, F)

    start(feed[0] + feed[1])
    for c in range(nc): st(at("k", c), jnp.zeros((8, LANES), u32))
    wait(feed[0])
    start(feed[2])
    push(ln(arena, [0]))
    prog.append(part(need, ("ln", 0, 1)))
    run(feed[1])
    push(ln(arena, [1]))
    prog.append(part(need, ("ln", 1, 1)))
    run(feed[2])
    start(feed[3] + cuts)
    params()
    mm1(0, 0, 4)
    mm1(1, 0, 4)
    run(feed[3])
    start(feed[4])
    mm1(0, 4)
    mm1(1, 4, 6)
    run(feed[4])
    start(feed[5])
    prep([0])
    mm1(1, 6)
    push(ln(ordered, [2]))
    fwd(0)
    push(spectral(0))
    mm1(2)
    run(feed[5])
    start(feed[6])
    prep([1])
    mm2(0, 0, 6)
    push(ln(ordered, [3]))
    fwd(1)
    push(spectral(1))
    mm1(3, 0, 10)
    mm2(0, 6, 8)
    run(feed[6])
    prep([2, 3])
    mm1(3, 10)
    mm2(0, 8)
    inv(0)
    mm2(1, 0, 4)
    fwd(2)
    run(cuts[0:1])
    push(spectral(2))
    mm2(1, 4, 6)
    fwd(3)
    mm2(1, 6)
    mm2(2, 0, 2)
    inv(1)
    run(cuts[1:2])
    push(spectral(3))
    mm2(2, 2)
    inv(2)
    mm2(3, 0, 2)
    inv(3)
    push(fin(0) + fin(1) + fin(2) + fin(3, 1))
    mm2(3, 2, fused=True)
    prog.append(part(need, ("fin", 3)))
    run()
    wait(out_copies)


@jax.jit
def pallas_parallel_sum__ssm_conv_h3__dense_activation_gelu__prompt_kernel(
    A_q: jax.Array,
    A_k: jax.Array,
    A_v: jax.Array,
    A_shift_k: jax.Array,
    A_ssm_k: jax.Array,
    A_ssm_D: jax.Array,
    B_x: jax.Array,
    B_w1: jax.Array,
    B_b1: jax.Array,
    B_w2: jax.Array,
    B_b2: jax.Array,
):
    B, S, D = A_q.shape
    F = B_w1.shape[1]
    nc, nb = D // LANES, S // TB
    q, k, v = (a.reshape(S, D) for a in (A_q, A_k, A_v))
    hbm = pl.BlockSpec(memory_space=pltpu.HBM)
    out = pl.pallas_call(
        functools.partial(_kernel, nc=nc, nb=nb, D=D, F=F),
        in_specs=[pl.BlockSpec(memory_space=pltpu.SMEM)] + [hbm] * 12,
        out_specs=hbm,
        out_shape=jax.ShapeDtypeStruct((S, D), A_q.dtype),
        scratch_shapes=[
            pltpu.VMEM((4, D), bf16), pltpu.VMEM((D,), bf16), pltpu.VMEM((F,), bf16), pltpu.VMEM((D,), bf16),
            pltpu.VMEM(_FWD.shape, u32), pltpu.VMEM(_INV.shape, u32),
            pltpu.VMEM((2 * _layout(nb, nc, F)[1], LANES), bf16),
            [pltpu.VMEM((2 * R * SR + 8, D), f32) for _ in range(nb)],
            [pltpu.VMEM((2 * R * P + 8, D), f32) for _ in range(nb)],
            pltpu.VMEM((nc, TB + 16, LANES), bf16),
            pltpu.VMEM((8, D), f32),
            pltpu.VMEM((1, F), f32),
            [[pltpu.VMEM((P, F), u32) for _ in range(2)] for _ in range(nb)],
            pltpu.SemaphoreType.DMA((4, nb)),
            pltpu.SemaphoreType.DMA((6,)),
            pltpu.SemaphoreType.DMA((nb,)),
            pltpu.VMEM((NCUT, 16, LANES), bf16),
            pltpu.SemaphoreType.DMA((NCUT,)),
        ],
        compiler_params=pltpu.CompilerParams(vmem_limit_bytes=120 * 1024 * 1024),
    )(jnp.asarray(np.zeros((1,), np.int32)), q, k, v, A_ssm_k, B_w1.T, B_w2, A_shift_k.T, A_ssm_D, B_b1, B_b2,
      jnp.asarray(_FWD), jnp.asarray(_INV))
    return out.reshape(B, S, D)
```

```python
import functools

import numpy as np
import jax
import jax.numpy as jnp
import jax.experimental.pallas as pl
import jax.experimental.pallas.tpu as pltpu

R = 4
P = 128
H = P // 2
TB = R * P
NFFT = 2 * TB
LANES = 128
IM, SR = P + 8, 2 * P + 24
RG = 8
PT = 5
PR, LR, FR = 16, 32, 64
C_LN, C_PREP, C_FIN, C_M = 135, 72, 105, (132, 134, 125, 130)
LAG, TL, NCUT = 2, 2, 2
FC = 256


def _pack_rows(m):
    u = np.ascontiguousarray(m, np.float32).view(np.uint32).astype(np.uint64)
    h = ((u + 0x7FFF + ((u >> 16) & 1)) >> 16).astype(np.uint32)
    return h[..., 0::2, :] | (h[..., 1::2, :] << np.uint32(16))


def _dft_tables():
    g = np.concatenate([np.arange(0, P, 2), np.arange(1, P, 2)]).astype(np.float64)
    s = np.arange(P, dtype=np.float64)
    fwd, inv = [], []
    for r in range(R):
        th = 2.0 * np.pi * (g[:, None] + 0.5) * (R * s[None, :] + r) / NFFT
        fwd.append(np.concatenate([np.cos(th), -np.sin(th)], 0))
        inv.append(np.stack([np.cos(th).T, -np.sin(th).T], 2).reshape(P, 2 * P) * (2.0 / NFFT))
    return _pack_rows(np.stack(fwd)), _pack_rows(np.stack(inv))


_FWD, _INV = _dft_tables()
_GC = float(np.sqrt(2.0 / np.pi))
f32, bf16, u32 = jnp.float32, jnp.bfloat16, jnp.uint32


def _layout(nb, nc, F):
    spec = dict(q=(nb * nc, TB // 2 + 8), k=(nb * nc, 8 + TB // 2 + 8),
                v=(nb * nc, TB // 2 + 8), kt=(nb * nc, TB // 2 + 8),
                sk=(nb * R * nc, H),
                o=(nb * nc, TB // 2 + 8), w1=(nc, F // 2), w2=(nc, F // 2),
                xn=(nb * R * nc, H), xu=(nb * R * nc, H), xk=(nb * R * nc, H),
                u=((nb - 1) * R * nc, SR), kf=((nb - 1) * R * nc, SR), kp=((nb - 1) * R * nc, SR),
                z=(nb * R * nc, P + 8), tick=(1, 8))
    off, out = 0, {}
    for name, (n, rows) in spec.items():
        out[name] = (off, rows)
        off += n * rows
    return out, off


def _lo(w):
    return pltpu.bitcast(w << 16, f32)


def _hi(w):
    return pltpu.bitcast(w & np.uint32(0xFFFF0000), f32)


def _packed(x):
    return pltpu.bitcast(x.astype(bf16), u32)


def _pair(a, b):
    return pltpu.bitcast(pltpu.pack_elementwise([a, b], packed_dtype=bf16), u32)


def _kernel(zero_ref, q_hbm, k_hbm, v_hbm, sk_hbm, w1_hbm, w2_hbm,
            shift_hbm, sd_hbm, b1_hbm, b2_hbm, fwd_hbm, inv_hbm,
            o_hbm,
            shift_ref, sd_ref, b1_ref, b2_ref, fwd_ref, inv_ref,
            arena16, ebuf, fbuf, obuf, prm, b1s, hbuf, in_sem, w_sem, out_sem, cut_buf, cut_sem, *, nc, nb, D, F):
    lanes = [slice(c * LANES, (c + 1) * LANES) for c in range(nc)]
    lay, total = _layout(nb, nc, F)
    arena = arena16.bitcast(u32)
    zero = pl.multiple_of(zero_ref[0], 8)

    i0 = jnp.zeros((), jnp.int32)

    def rows(start, n):
        return pl.ds(pl.multiple_of(i0 + start, 8), n)

    def late(ref):
        return ref.at[pl.ds(zero, ref.shape[0]), :]

    ordered = late(arena)
    e_ord, f_ord = [late(r) for r in ebuf], [late(r) for r in fbuf]
    E_ROWS, F_ROWS = 2 * R * SR, 2 * R * P

    def at(name, *idx):
        n = 0
        for i in idx[:-1]:
            n = n * R + i
        return lay[name][0] + (n * nc + idx[-1]) * lay[name][1]

    def ld(row, n):
        return pltpu.bitcast(ordered[rows(row, n), :], f32)

    def st(row, val):
        arena[rows(row, val.shape[0]), :] = pltpu.bitcast(val, u32)

    def slab16(row, n):
        return arena16.at[2 * row:2 * (row + n), :]

    def wide(name, *idx):
        return jnp.concatenate([arena[rows(at(name, *idx, c), lay[name][1]), :] for c in range(nc)], axis=1)

    def cols_in(src, b, offs, sem, history=0):
        return [pltpu.make_async_copy(src.at[pl.ds(b * TB - 2 * history, TB + 2 * history), lanes[c]],
                                      slab16(offs[c] - history, TB // 2 + history), sem) for c in range(nc)]

    def conv_in(b):
        return (cols_in(k_hbm, b, [at("k", b, c) + 8 for c in range(nc)], in_sem.at[0, b], 8 if b else 0)
                + cols_in(v_hbm, b, [at("v", b, c) for c in range(nc)], in_sem.at[1, b])
                + [pltpu.make_async_copy(sk_hbm.at[lanes[c], pl.ds(b * TB + n * P, P)],
                                         slab16(at("sk", b, n, c), H), in_sem.at[2, b])
                   for c in range(nc) for n in range(R)])

    def q_in(b):
        return cols_in(q_hbm, b, [at("q", b, c) for c in range(nc)], in_sem.at[3, b])

    out_copies = []

    def out_copy(b, c, src):
        return pltpu.make_async_copy(slab16(at("o", b, c), TB // 2) if src is ordered else obuf.at[c, 0:TB, :],
                                     o_hbm.at[pl.ds(b * TB, TB), lanes[c]], out_sem.at[b])

    def w1_in(lo, hi, n):
        return [pltpu.make_async_copy(w1_hbm.at[lo:hi, lanes[c]], slab16(at("w1", c) + lo // 2, (hi - lo) // 2),
                                      w_sem.at[n]) for c in range(nc)]

    small_in = [pltpu.make_async_copy(src, dst, w_sem.at[3]) for src, dst in (
        (shift_hbm, shift_ref), (sd_hbm, sd_ref), (b1_hbm, b1_ref), (b2_hbm, b2_ref))]
    tables_in = [pltpu.make_async_copy(fwd_hbm, fwd_ref, w_sem.at[4]),
                 pltpu.make_async_copy(inv_hbm, inv_ref, w_sem.at[5])]
    w2_in = [pltpu.make_async_copy(w2_hbm.at[:, lanes[c]], slab16(at("w2", c), F // 2), w_sem.at[1])
             for c in range(nc)]

    def start(cs):
        for c in cs:
            c.start()

    def wait(cs):
        for c in cs:
            c.wait()

    def delayed(x, n):
        for _ in range(n):
            x = jnp.tanh(x)
        return x

    tiles = {}

    def t_load(b, c, n):
        w = pltpu.bitcast(ordered[rows(at("sk", b, n, c), H), :], bf16)
        tiles[b, c, n] = pltpu.bitcast(w.T, u32)

    def t_store(b, c, n):
        st(at("kt", b, c) + n * H, tiles.pop((b, c, n)))

    def prep_unit(b, j, c, s0):
        base = at("k", b, c) + 8 + j + 2 * s0
        t = ordered[rows(at("k", b, c), 8), :]
        t = delayed(pltpu.bitcast(t, f32), PT)

        wa = ordered[pl.ds(base - 2, PR, stride=2), :]
        wb = ordered[pl.ds(base - 1, PR, stride=2), :]
        wc = ordered[pl.ds(base, PR, stride=2), :]
        ks = [_hi(wa), _lo(wb), _hi(wb), _lo(wc), _hi(wc)]
        vw = ordered[pl.ds(at("v", b, c) + j + 2 * s0, PR, stride=2), :]
        vs = [_lo(vw), _hi(vw)]
        tw = ordered[pl.ds(at("kt", b, c) + j + 2 * s0, PR, stride=2), :]
        ts = [_lo(tw), _hi(tw)]
        for e in range(2):
            acc = ks[3 + e] * prm[0:1, lanes[c]]
            for i in range(1, 4):
                acc = acc + ks[3 + e - i] * prm[i:i + 1, lanes[c]]
            st(at("xu", b, 2 * j + e, c) + s0 // 2, _packed(acc * vs[e]))
            st(at("xk", b, 2 * j + e, c) + s0 // 2, _packed(ts[e]))
        st(at("tick", 0), t)

    def m_unit(b, g0, c):
        def cld(name, slot, m):
            row = at(name, slot, m, c) + g0
            return ld(row, RG), ld(row + IM, RG)

        def cst(name, m, vr, vi):
            row = at(name, b, m, c) + g0
            st(row, vr)
            st(row + IM, vi)

        def bfly(which):
            offs = [(which * R + r) * SR + g0 for r in range(R)]
            er = [e_ord[b][rows(o, RG), lanes[c]] for o in offs]
            ei = [e_ord[b][rows(o + IM, RG), lanes[c]] for o in offs]
            ar, ai = er[0] + er[2], ei[0] + ei[2]
            br, bi = er[0] - er[2], ei[0] - ei[2]
            cr, ci = er[1] + er[3], ei[1] + ei[3]
            dr, di = er[1] - er[3], ei[1] - ei[3]
            return ([ar + cr, br + di, ar - cr, br - di],
                    [ai + ci, bi - dr, ai - ci, bi + dr])

        tick = pltpu.roll(e_ord[b][rows(g0, RG), lanes[c]], 1, 1)
        ur, ui = bfly(0)
        kr, ki = bfly(1)
        if b == 0:
            kr = [x + prm[4:5, lanes[c]] for x in kr]
        keep = []
        for m in range(R):
            if b == 0:
                keep.append((kr[m], ki[m]))
            else:
                pr, pi = cld("kp", b - 1, m)
                keep.append((kr[m] - pi, ki[m] + pr) if g0 < P // 2 else (kr[m] + pi, ki[m] - pr))
        if b < nb - 1:
            for m in range(R):
                cst("kp", m, kr[m], ki[m])
                cst("u", m, ur[m], ui[m])
                cst("kf", m, *keep[m])
        else:
            st(at("tick", 0), keep[R - 1][1])
        yr, yi = [], []
        for m in range(R):
            accr = acci = None
            for jj in range(b + 1):
                a_r, a_i = (ur[m], ui[m]) if jj == b else cld("u", jj, m)
                b_r, b_i = keep[m] if jj == 0 else cld("kf", b - jj, m)
                pr_ = a_r * b_r - a_i * b_i
                pi_ = a_r * b_i + a_i * b_r
                accr = pr_ if accr is None else accr + pr_
                acci = pi_ if acci is None else acci + pi_
            yr.append(accr)
            yi.append(acci)
            if b >= 2 and m == 1:
                st(at("tick", 0), acci)
        ar, ai = yr[0] + yr[2], yi[0] + yi[2]
        br, bi = yr[0] - yr[2], yi[0] - yi[2]
        cr, ci = yr[1] + yr[3], yi[1] + yi[3]
        dr, di = yr[1] - yr[3], yi[1] - yi[3]
        zr = [ar + cr, br - di, ar - cr, br + di]
        zi = [ai + ci, bi + dr, ai - ci, bi - dr]
        for r in range(R):
            st(at("z", b, r, c) + g0, _pair(zr[r], zi[r]))
        ebuf[b][E_ROWS:E_ROWS + RG, 0:LANES] = tick
        st(at("tick", 0), tick)

    def q_words(src, b, j, c):
        return src[pl.ds(at("q", b, c) + j, P, stride=2), :]

    def ln_rows(src, b, r, s0):
        return jnp.concatenate([(_lo, _hi)[r % 2](src[pl.ds(at("q", b, c) + r // 2 + 2 * s0, LR, stride=2), :])
                                for c in range(nc)], axis=1)

    mean, rstd = {}, {}

    def ln_mean(src, key):
        mean[key] = jnp.mean(ln_rows(src, *key), axis=-1, keepdims=True)

    def ln_rstd(src, key):
        xc = ln_rows(src, *key) - mean[key]
        rstd[key] = jax.lax.rsqrt(jnp.mean(xc * xc, axis=-1, keepdims=True) + 1e-5)

    def ln_store(src, key):
        b, r, s0 = key
        xn = _packed((ln_rows(src, *key) - mean.pop(key)) * rstd.pop(key))
        for c in range(nc):
            st(at("xn", b, r, c) + s0 // 2, xn[:, lanes[c]])

    def ln_unit(src, keys, n):
        for stage, fn in enumerate((ln_mean, ln_rstd, ln_store)):
            if 0 <= n - stage < len(keys):
                fn(src, keys[n - stage])

    def emit_out(src, fsrc, b, j, c, o, s0=0):
        n = o[0].shape[0]
        outs = []
        for e in range(2):
            r = 2 * j + e
            xn = pltpu.bitcast(src[rows(at("xn", b, r, c) + s0 // 2, n // 2), :], bf16).astype(f32)
            outs.append(o[e] + xn * fsrc[(R + r) * P + s0:(R + r) * P + s0 + n, lanes[c]])
        if src is ordered:
            arena[pl.ds(at("o", b, c) + j + 2 * s0, n, stride=2), :] = _pair(*outs)
        else:
            obuf.at[c].bitcast(u32)[pl.ds(j + 2 * s0, n, stride=2), :] = _pair(*outs)
        if j == 1 and s0 + n == P:
            out_copies.append(out_copy(b, c, src))
            out_copies[-1].start()

    def fin_gate(b):
        fbuf[b][F_ROWS:F_ROWS + 8, 0:LANES] = ld(at("k", 0, 0), 8)

    def fin_unit(b, j, c, s0):
        o = [f_ord[b][(2 * j + e) * P + s0:(2 * j + e) * P + s0 + FR, lanes[c]] for e in range(2)]
        tick = delayed(f_ord[b][0:8, lanes[c]], 7)
        emit_out(ordered, f_ord[b], b, j, c, o, s0)
        fbuf[b][F_ROWS:F_ROWS + 8, 0:LANES] = tick
        st(at("tick", 0), tick)

    queue = []
    credit = [0]

    def fill(cycles):
        credit[0] += cycles
        while queue and credit[0] >= queue[0][2]:
            _, fn, cost = queue.pop(0)
            credit[0] -= cost
            fn()
        if not queue:
            credit[0] = min(credit[0], 128)

    def need(tag):
        while any(t == tag for t, _, _ in queue):
            queue.pop(0)[1]()

    marks = {}
    pieces = []
    cursor = [0]

    def weights(row, n):
        i = cursor[0]
        assert pieces[i][0] == row
        cursor[0] += 1
        for p in range(len(marks), min(i + 1 + LAG, len(pieces))):
            need(pieces[p][1])
            marks[p] = ordered[rows(pieces[p][0], 8), :]
            fill(pieces[p][2])
        return pltpu.bitcast(jnp.concatenate([marks[i], arena[rows(row + 8, n - 8), :]], axis=0), bf16)

    def mm1_op(b, j, s0, s1):
        need(("ln", b, j))
        w = jnp.concatenate([weights(at("w1", c) + s0 // 2, (s1 - s0) // 2) for c in range(nc)], axis=1)
        x = pltpu.bitcast(jnp.concatenate([wide("xn", b, 2 * j), wide("xn", b, 2 * j + 1)], axis=0), bf16)
        h = jax.lax.dot_general(x, w, (((1,), (1,)), ((), ())), preferred_element_type=f32) + b1s[0:1, s0:s1]
        u = h * (h * h * (_GC * 0.044715) + _GC)
        hh = 0.5 * h
        hbuf[b][j][:, s0:s1] = _packed(hh * jnp.tanh(u) + hh)

    def mm2_op(b, j, c, fused):
        w = jnp.concatenate([weights(at("w2", c) + s0 // 2, (min(s0 + FC, F) - s0) // 2)
                             for s0 in range(0, F, FC)], axis=0)
        mlp = jnp.dot(pltpu.bitcast(hbuf[b][j][...], bf16), w, preferred_element_type=f32)
        mlp = [mlp[0:P], mlp[P:2 * P]]
        qw = q_words(arena, b, j, c)
        o = [mlp[0] + prm[5:6, lanes[c]] + _lo(qw), mlp[1] + prm[5:6, lanes[c]] + _hi(qw)]
        if fused:
            emit_out(arena, fbuf[b], b, j, c, o)
        else:
            for e in range(2):
                fbuf[b][(2 * j + e) * P:(2 * j + e + 1) * P, lanes[c]] = o[e]

    def fwd_op(b, r, src, dst):
        e = jnp.dot(pltpu.bitcast(fwd_ref[r], bf16), jnp.concatenate([weights(at(src, b, r, c), H) for c in range(nc)], axis=1),
                    preferred_element_type=f32)
        row = (dst * R + r) * SR
        ebuf[b][row:row + P, :] = e[0:P]
        ebuf[b][row + IM:row + IM + P, :] = e[P:2 * P]

    def inv_op(b, r):
        y = jnp.dot(pltpu.bitcast(inv_ref[r], bf16), jnp.concatenate([weights(at("z", b, r, c), P) for c in range(nc)], axis=1),
                    preferred_element_type=f32)
        fbuf[b][(R + r) * P:(R + r + 1) * P, :] = y

    part = functools.partial

    prog = []

    def push(units):
        prog.append(part(queue.extend, units))

    def ln(src, blocks, cost=C_LN):
        keys = [(b, r, s0) for b in blocks for r in range(R) for s0 in range(0, P, LR)]
        tag = lambda n: ("ln", keys[n][0], keys[n][1] // 2)
        return [(tag(max(n - 2, 0)), part(ln_unit, src, keys, n), cost) for n in range(len(keys) + 2)]

    def prep(blocks):
        ts = [(b, c, n) for b in blocks for c in range(nc) for n in range(R)]
        lead, out = [], []
        for i in range(-TL - 1, len(ts)):
            tag, dst = ("prep", ts[max(i, 0)][0]), lead if i < 0 else out
            if i + TL + 1 < len(ts):
                dst.append((tag, part(t_load, *ts[i + TL + 1]), 0))
            for j in range(2):
                if j == 1 and -1 <= i < len(ts) - 1:
                    dst.append((tag, part(t_store, *ts[i + 1]), 0))
                if i >= 0:
                    b, c, n = ts[i]
                    dst += [(tag, part(prep_unit, b, j, c, s0), C_PREP)
                            for s0 in range(n * P // R, (n + 1) * P // R, PR)]

        def enqueue():
            n = 2 * TL + 2
            tail = queue[-n:]
            tail += [(lead[0][0], lambda: None, C_LN)] * (n - len(tail))
            queue[-n:] = mix(tail, lead) + out

        prog.append(enqueue)

    def spectral(b):
        return [(("m", b), part(m_unit, b, g0, c), C_M[b]) for g0 in range(0, P, RG) for c in range(nc)]

    def fin(b, n=nc):
        return [(("fin", b), part(fin_gate, b), 0)] + [
            (("fin", b), part(fin_unit, b, j, c, s0), C_FIN)
            for c in range(n) for j in range(2) for s0 in range(0, P, FR)]

    def mix(main, extra):
        out = []
        for i, u in enumerate(main):
            out += extra[i * len(extra) // len(main):(i + 1) * len(extra) // len(main)] + [u]
        return out

    def mm1(b, lo=0, hi=None):
        for s0, j in [(s0, j) for s0 in range(0, F, FC) for j in range(2)][lo:hi]:
            s1 = min(s0 + FC, F)
            pieces.extend((at("w1", c) + s0 // 2, None, 64 * pl.cdiv(s1 - s0, LANES)) for c in range(nc))
            prog.append(part(mm1_op, b, j, s0, s1))

    def mm2(b, lo=0, hi=None, fused=False):
        for c, j in [(c, j) for c in range(nc) for j in range(2)][lo:hi]:
            pieces.extend((at("w2", c) + s0 // 2, None, 128) for s0 in range(0, F, FC))
            prog.append(part(mm2_op, b, j, c, fused))

    def fwd(b):
        for r in range(R):
            for dst, src in enumerate(("xu", "xk")):
                pieces.extend((at(src, b, r, c), ("prep", b), 64) for c in range(nc))
                prog.append(part(fwd_op, b, r, src, dst))

    def inv(b):
        for r in range(R):
            pieces.extend((at("z", b, r, c), ("m", b), 64) for c in range(nc))
            prog.append(part(inv_op, b, r))

    def run(then_wait=()):
        for step in prog:
            step()
        prog.clear(), pieces.clear(), marks.clear()
        cursor[0] = 0
        credit[0] = -256
        wait(then_wait)

    feed = [q_in(0), q_in(1), w1_in(0, 2 * FC, 0) + small_in, w1_in(2 * FC, F, 2),
            q_in(2) + conv_in(0) + tables_in[:1], w2_in + conv_in(1) + q_in(3) + tables_in[1:],
            conv_in(2) + conv_in(3)]
    cuts = [pltpu.make_async_copy(q_hbm.at[0:16, 0:LANES], cut_buf.at[i], cut_sem.at[i]) for i in range(NCUT)]

    def params():
        prm[0:4, :] = shift_ref[...].astype(f32)
        prm[4:5, :] = sd_ref[...].astype(f32).reshape(1, D)
        prm[5:6, :] = b2_ref[...].astype(f32).reshape(1, D)
        b1s[...] = b1_ref[...].astype(f32).reshape(1, F)

    start(feed[0] + feed[1])
    for c in range(nc):
        st(at("k", 0, c), jnp.zeros((8, LANES), u32))
    wait(feed[0])
    start(feed[2])
    push(ln(arena, [0]))
    prog.append(part(need, ("ln", 0, 1)))
    run(feed[1])
    push(ln(arena, [1]))
    prog.append(part(need, ("ln", 1, 1)))
    run(feed[2])
    start(feed[3] + cuts)
    params()
    mm1(0, 0, 4)
    mm1(1, 0, 4)
    run(feed[3])
    start(feed[4])
    mm1(0, 4)
    mm1(1, 4, 6)
    run(feed[4])
    start(feed[5])
    prep([0])
    mm1(1, 6)
    push(ln(ordered, [2]))
    fwd(0)
    push(spectral(0))
    mm1(2)
    run(feed[5])
    start(feed[6])
    prep([1])
    mm2(0, 0, 6)
    push(ln(ordered, [3]))
    fwd(1)
    push(spectral(1))
    mm1(3, 0, 10)
    mm2(0, 6, 8)
    run(feed[6])
    prep([2, 3])
    mm1(3, 10)
    mm2(0, 8)
    inv(0)
    mm2(1, 0, 4)
    fwd(2)
    run(cuts[0:1])
    push(spectral(2))
    mm2(1, 4, 6)
    fwd(3)
    mm2(1, 6)
    mm2(2, 0, 2)
    inv(1)
    run(cuts[1:2])
    push(spectral(3))
    mm2(2, 2)
    inv(2)
    mm2(3, 0, 2)
    inv(3)
    push(fin(0) + fin(1) + fin(2) + fin(3, 1))
    mm2(3, 2, fused=True)
    prog.append(part(need, ("fin", 3)))
    run()
    wait(out_copies)


@jax.jit
def pallas_parallel_sum__ssm_conv_h3__dense_activation_gelu__prompt_kernel(
    A_q: jax.Array,
    A_k: jax.Array,
    A_v: jax.Array,
    A_shift_k: jax.Array,
    A_ssm_k: jax.Array,
    A_ssm_D: jax.Array,
    B_x: jax.Array,
    B_w1: jax.Array,
    B_b1: jax.Array,
    B_w2: jax.Array,
    B_b2: jax.Array,
):
    B, S, D = A_q.shape
    F = B_w1.shape[1]
    nc, nb = D // LANES, S // TB
    q, k, v = (a.reshape(S, D) for a in (A_q, A_k, A_v))
    hbm = pl.BlockSpec(memory_space=pltpu.HBM)
    out = pl.pallas_call(
        functools.partial(_kernel, nc=nc, nb=nb, D=D, F=F),
        in_specs=[pl.BlockSpec(memory_space=pltpu.SMEM)] + [hbm] * 12,
        out_specs=hbm,
        out_shape=jax.ShapeDtypeStruct((S, D), A_q.dtype),
        scratch_shapes=[
            pltpu.VMEM((4, D), bf16), pltpu.VMEM((D,), bf16), pltpu.VMEM((F,), bf16), pltpu.VMEM((D,), bf16),
            pltpu.VMEM(_FWD.shape, u32), pltpu.VMEM(_INV.shape, u32),
            pltpu.VMEM((2 * _layout(nb, nc, F)[1], LANES), bf16),
            [pltpu.VMEM((2 * R * SR + 8, D), f32) for _ in range(nb)],
            [pltpu.VMEM((2 * R * P + 8, D), f32) for _ in range(nb)],
            pltpu.VMEM((nc, TB + 16, LANES), bf16),
            pltpu.VMEM((8, D), f32),
            pltpu.VMEM((1, F), f32),
            [[pltpu.VMEM((P, F), u32) for _ in range(2)] for _ in range(nb)],
            pltpu.SemaphoreType.DMA((4, nb)),
            pltpu.SemaphoreType.DMA((6,)),
            pltpu.SemaphoreType.DMA((nb,)),
            pltpu.VMEM((NCUT, 16, LANES), bf16),
            pltpu.SemaphoreType.DMA((NCUT,)),
        ],
        compiler_params=pltpu.CompilerParams(vmem_limit_bytes=120 * 1024 * 1024),
    )(jnp.asarray(np.zeros((1,), np.int32)), q, k, v, A_ssm_k, B_w1.T, B_w2, A_shift_k.T, A_ssm_D, B_b1, B_b2,
      jnp.asarray(_FWD), jnp.asarray(_INV))
    return out.reshape(B, S, D)
```

```python
import functools

import numpy as np
import jax
import jax.numpy as jnp
import jax.experimental.pallas as pl
import jax.experimental.pallas.tpu as pltpu

R = 4
P = 128
H = P // 2
TB = R * P
NFFT = 2 * TB
LANES = 128
IM, SR = P + 8, 2 * P + 24
RG = 8
PT = 5
PR, LR, FR = 16, 32, 64
C_LN, C_PREP, C_FIN, C_M = 135, 72, 105, (132, 134, 125, 130)
LAG, TL, NCUT = 2, 2, 2
FC = 256


def _pack_rows(m):
    u = np.ascontiguousarray(m, np.float32).view(np.uint32).astype(np.uint64)
    h = ((u + 0x7FFF + ((u >> 16) & 1)) >> 16).astype(np.uint32)
    return h[..., 0::2, :] | (h[..., 1::2, :] << np.uint32(16))


def _dft_tables():
    g = np.concatenate([np.arange(0, P, 2), np.arange(1, P, 2)]).astype(np.float64)
    s = np.arange(P, dtype=np.float64)
    fwd, inv = [], []
    for r in range(R):
        th = 2.0 * np.pi * (g[:, None] + 0.5) * (R * s[None, :] + r) / NFFT
        fwd.append(np.concatenate([np.cos(th), -np.sin(th)], 0))
        inv.append(np.stack([np.cos(th).T, -np.sin(th).T], 2).reshape(P, 2 * P) * (2.0 / NFFT))
    return _pack_rows(np.stack(fwd)), _pack_rows(np.stack(inv))


_FWD, _INV = _dft_tables()
_GC = float(np.sqrt(2.0 / np.pi))
f32, bf16, u32 = jnp.float32, jnp.bfloat16, jnp.uint32


def _layout(nb, nc, F):
    spec = dict(q=(nb * nc, TB // 2 + 8), k=(nb * nc, 8 + TB // 2 + 8),
                v=(nb * nc, TB // 2 + 8), kt=(nb * nc, TB // 2 + 8),
                sk=(nb * R * nc, H),
                o=(nb * nc, TB // 2 + 8), w1=(nc, F // 2), w2=(nc, F // 2),
                xn=(nb * R * nc, H), xu=(nb * R * nc, H), xk=(nb * R * nc, H),
                u=((nb - 1) * R * nc, SR), kf=((nb - 1) * R * nc, SR), kp=((nb - 1) * R * nc, SR),
                z=(nb * R * nc, P + 8), tick=(1, 8))
    off, out = 0, {}
    for name, (n, rows) in spec.items():
        out[name] = (off, rows)
        off += n * rows
    return out, off


def _lo(w):
    return pltpu.bitcast(w << 16, f32)


def _hi(w):
    return pltpu.bitcast(w & np.uint32(0xFFFF0000), f32)


def _packed(x):
    return pltpu.bitcast(x.astype(bf16), u32)


def _pair(a, b):
    return pltpu.bitcast(pltpu.pack_elementwise([a, b], packed_dtype=bf16), u32)


def _kernel(zero_ref, q_hbm, k_hbm, v_hbm, sk_hbm, w1_hbm, w2_hbm,
            shift_hbm, sd_hbm, b1_hbm, b2_hbm, fwd_hbm, inv_hbm,
            o_hbm,
            shift_ref, sd_ref, b1_ref, b2_ref, fwd_ref, inv_ref,
            arena16, ebuf, fbuf, obuf, prm, b1s, hbuf, in_sem, w_sem, out_sem, cut_buf, cut_sem, *, nc, nb, D, F):
    lanes = [slice(c * LANES, (c + 1) * LANES) for c in range(nc)]
    lay, total = _layout(nb, nc, F)
    arena = arena16.bitcast(u32)
    zero = pl.multiple_of(zero_ref[0], 8)

    i0 = jnp.zeros((), jnp.int32)

    def rows(start, n):
        return pl.ds(pl.multiple_of(i0 + start, 8), n)

    def late(ref):
        return ref.at[pl.ds(zero, ref.shape[0]), :]

    ordered = late(arena)
    e_ord, f_ord = [late(r) for r in ebuf], [late(r) for r in fbuf]
    E_ROWS, F_ROWS = 2 * R * SR, 2 * R * P

    def at(name, *idx):
        n = 0
        for i in idx[:-1]:
            n = n * R + i
        return lay[name][0] + (n * nc + idx[-1]) * lay[name][1]

    def ld(row, n):
        return pltpu.bitcast(ordered[rows(row, n), :], f32)

    def st(row, val):
        arena[rows(row, val.shape[0]), :] = pltpu.bitcast(val, u32)

    def slab16(row, n):
        return arena16.at[2 * row:2 * (row + n), :]

    def wide(name, *idx):
        return jnp.concatenate([arena[rows(at(name, *idx, c), lay[name][1]), :] for c in range(nc)], axis=1)

    def cols_in(src, b, offs, sem, history=0):
        return [pltpu.make_async_copy(src.at[pl.ds(b * TB - 2 * history, TB + 2 * history), lanes[c]],
                                      slab16(offs[c] - history, TB // 2 + history), sem) for c in range(nc)]

    def conv_in(b):
        return (cols_in(k_hbm, b, [at("k", b, c) + 8 for c in range(nc)], in_sem.at[0, b], 8 if b else 0)
                + cols_in(v_hbm, b, [at("v", b, c) for c in range(nc)], in_sem.at[1, b])
                + [pltpu.make_async_copy(sk_hbm.at[lanes[c], pl.ds(b * TB + n * P, P)],
                                         slab16(at("sk", b, n, c), H), in_sem.at[2, b])
                   for c in range(nc) for n in range(R)])

    def q_in(b):
        return cols_in(q_hbm, b, [at("q", b, c) for c in range(nc)], in_sem.at[3, b])

    out_copies = []

    def out_copy(b, c, src):
        return pltpu.make_async_copy(slab16(at("o", b, c), TB // 2) if src is ordered else obuf.at[c, 0:TB, :],
                                     o_hbm.at[pl.ds(b * TB, TB), lanes[c]], out_sem.at[b])

    def w1_in(lo, hi, n):
        return [pltpu.make_async_copy(w1_hbm.at[lo:hi, lanes[c]], slab16(at("w1", c) + lo // 2, (hi - lo) // 2),
                                      w_sem.at[n]) for c in range(nc)]

    small_in = [pltpu.make_async_copy(src, dst, w_sem.at[3]) for src, dst in (
        (shift_hbm, shift_ref), (sd_hbm, sd_ref), (b1_hbm, b1_ref), (b2_hbm, b2_ref))]
    tables_in = [pltpu.make_async_copy(fwd_hbm, fwd_ref, w_sem.at[4]),
                 pltpu.make_async_copy(inv_hbm, inv_ref, w_sem.at[5])]
    w2_in = [pltpu.make_async_copy(w2_hbm.at[:, lanes[c]], slab16(at("w2", c), F // 2), w_sem.at[1])
             for c in range(nc)]

    def start(cs):
        for c in cs:
            c.start()

    def wait(cs):
        for c in cs:
            c.wait()

    def delayed(x, n):
        for _ in range(n):
            x = jnp.tanh(x)
        return x

    tiles = {}

    def t_load(b, c, n):
        w = pltpu.bitcast(ordered[rows(at("sk", b, n, c), H), :], bf16)
        tiles[b, c, n] = pltpu.bitcast(w.T, u32)

    def t_store(b, c, n):
        st(at("kt", b, c) + n * H, tiles.pop((b, c, n)))

    def prep_unit(b, j, c, s0):
        base = at("k", b, c) + 8 + j + 2 * s0
        t = ordered[rows(at("k", b, c), 8), :]
        t = delayed(pltpu.bitcast(t, f32), PT)

        wa = ordered[pl.ds(base - 2, PR, stride=2), :]
        wb = ordered[pl.ds(base - 1, PR, stride=2), :]
        wc = ordered[pl.ds(base, PR, stride=2), :]
        ks = [_hi(wa), _lo(wb), _hi(wb), _lo(wc), _hi(wc)]
        vw = ordered[pl.ds(at("v", b, c) + j + 2 * s0, PR, stride=2), :]
        vs = [_lo(vw), _hi(vw)]
        tw = ordered[pl.ds(at("kt", b, c) + j + 2 * s0, PR, stride=2), :]
        ts = [_lo(tw), _hi(tw)]
        for e in range(2):
            acc = ks[3 + e] * prm[0:1, lanes[c]]
            for i in range(1, 4):
                acc = acc + ks[3 + e - i] * prm[i:i + 1, lanes[c]]
            st(at("xu", b, 2 * j + e, c) + s0 // 2, _packed(acc * vs[e]))
            st(at("xk", b, 2 * j + e, c) + s0 // 2, _packed(ts[e]))
        st(at("tick", 0), t)

    def m_unit(b, g0, c):
        def cld(name, slot, m):
            row = at(name, slot, m, c) + g0
            return ld(row, RG), ld(row + IM, RG)

        def cst(name, m, vr, vi):
            row = at(name, b, m, c) + g0
            st(row, vr)
            st(row + IM, vi)

        def bfly(which):
            offs = [(which * R + r) * SR + g0 for r in range(R)]
            er = [e_ord[b][rows(o, RG), lanes[c]] for o in offs]
            ei = [e_ord[b][rows(o + IM, RG), lanes[c]] for o in offs]
            ar, ai = er[0] + er[2], ei[0] + ei[2]
            br, bi = er[0] - er[2], ei[0] - ei[2]
            cr, ci = er[1] + er[3], ei[1] + ei[3]
            dr, di = er[1] - er[3], ei[1] - ei[3]
            return ([ar + cr, br + di, ar - cr, br - di],
                    [ai + ci, bi - dr, ai - ci, bi + dr])

        tick = pltpu.roll(e_ord[b][rows(g0, RG), lanes[c]], 1, 1)
        ur, ui = bfly(0)
        kr, ki = bfly(1)
        if b == 0:
            kr = [x + prm[4:5, lanes[c]] for x in kr]
        keep = []
        for m in range(R):
            if b == 0:
                keep.append((kr[m], ki[m]))
            else:
                pr, pi = cld("kp", b - 1, m)
                keep.append((kr[m] - pi, ki[m] + pr) if g0 < P // 2 else (kr[m] + pi, ki[m] - pr))
        if b < nb - 1:
            for m in range(R):
                cst("kp", m, kr[m], ki[m])
                cst("u", m, ur[m], ui[m])
                cst("kf", m, *keep[m])
        else:
            st(at("tick", 0), keep[R - 1][1])
        yr, yi = [], []
        for m in range(R):
            accr = acci = None
            for jj in range(b + 1):
                a_r, a_i = (ur[m], ui[m]) if jj == b else cld("u", jj, m)
                b_r, b_i = keep[m] if jj == 0 else cld("kf", b - jj, m)
                pr_ = a_r * b_r - a_i * b_i
                pi_ = a_r * b_i + a_i * b_r
                accr = pr_ if accr is None else accr + pr_
                acci = pi_ if acci is None else acci + pi_
            yr.append(accr)
            yi.append(acci)
            if b >= 2 and m == 1:
                st(at("tick", 0), acci)
        ar, ai = yr[0] + yr[2], yi[0] + yi[2]
        br, bi = yr[0] - yr[2], yi[0] - yi[2]
        cr, ci = yr[1] + yr[3], yi[1] + yi[3]
        dr, di = yr[1] - yr[3], yi[1] - yi[3]
        zr = [ar + cr, br - di, ar - cr, br + di]
        zi = [ai + ci, bi + dr, ai - ci, bi - dr]
        for r in range(R):
            st(at("z", b, r, c) + g0, _pair(zr[r], zi[r]))
        ebuf[b][E_ROWS:E_ROWS + RG, 0:LANES] = tick
        st(at("tick", 0), tick)

    def q_words(src, b, j, c):
        return src[pl.ds(at("q", b, c) + j, P, stride=2), :]

    def ln_rows(src, b, r, s0):
        return jnp.concatenate([(_lo, _hi)[r % 2](src[pl.ds(at("q", b, c) + r // 2 + 2 * s0, LR, stride=2), :])
                                for c in range(nc)], axis=1)

    mean, rstd = {}, {}

    def ln_mean(src, key):
        mean[key] = jnp.mean(ln_rows(src, *key), axis=-1, keepdims=True)

    def ln_rstd(src, key):
        xc = ln_rows(src, *key) - mean[key]
        rstd[key] = jax.lax.rsqrt(jnp.mean(xc * xc, axis=-1, keepdims=True) + 1e-5)

    def ln_store(src, key):
        b, r, s0 = key
        xn = _packed((ln_rows(src, *key) - mean.pop(key)) * rstd.pop(key))
        for c in range(nc):
            st(at("xn", b, r, c) + s0 // 2, xn[:, lanes[c]])

    def ln_unit(src, keys, n):
        for stage, fn in enumerate((ln_mean, ln_rstd, ln_store)):
            if 0 <= n - stage < len(keys):
                fn(src, keys[n - stage])

    def emit_out(src, fsrc, b, j, c, o, s0=0):
        n = o[0].shape[0]
        outs = []
        for e in range(2):
            r = 2 * j + e
            xn = pltpu.bitcast(src[rows(at("xn", b, r, c) + s0 // 2, n // 2), :], bf16).astype(f32)
            outs.append(o[e] + xn * fsrc[(R + r) * P + s0:(R + r) * P + s0 + n, lanes[c]])
        if src is ordered:
            arena[pl.ds(at("o", b, c) + j + 2 * s0, n, stride=2), :] = _pair(*outs)
        else:
            obuf.at[c].bitcast(u32)[pl.ds(j + 2 * s0, n, stride=2), :] = _pair(*outs)
        if j == 1 and s0 + n == P:
            out_copies.append(out_copy(b, c, src))
            out_copies[-1].start()

    def fin_gate(b):
        fbuf[b][F_ROWS:F_ROWS + 8, 0:LANES] = ld(at("k", 0, 0), 8)

    def fin_unit(b, j, c, s0):
        o = [f_ord[b][(2 * j + e) * P + s0:(2 * j + e) * P + s0 + FR, lanes[c]] for e in range(2)]
        tick = delayed(f_ord[b][0:8, lanes[c]], 7)
        emit_out(ordered, f_ord[b], b, j, c, o, s0)
        fbuf[b][F_ROWS:F_ROWS + 8, 0:LANES] = tick
        st(at("tick", 0), tick)

    queue = []
    credit = [0]

    def fill(cycles):
        credit[0] += cycles
        while queue and credit[0] >= queue[0][2]:
            _, fn, cost = queue.pop(0)
            credit[0] -= cost
            fn()
        if not queue:
            credit[0] = min(credit[0], 128)

    def need(tag):
        while any(t == tag for t, _, _ in queue):
            queue.pop(0)[1]()

    marks = {}
    pieces = []
    cursor = [0]

    def weights(row, n):
        i = cursor[0]
        assert pieces[i][0] == row
        cursor[0] += 1
        for p in range(len(marks), min(i + 1 + LAG, len(pieces))):
            need(pieces[p][1])
            marks[p] = ordered[rows(pieces[p][0], 8), :]
            fill(pieces[p][2])
        return pltpu.bitcast(jnp.concatenate([marks[i], arena[rows(row + 8, n - 8), :]], axis=0), bf16)

    def mm1_op(b, j, s0, s1):
        need(("ln", b, j))
        w = jnp.concatenate([weights(at("w1", c) + s0 // 2, (s1 - s0) // 2) for c in range(nc)], axis=1)
        x = pltpu.bitcast(jnp.concatenate([wide("xn", b, 2 * j), wide("xn", b, 2 * j + 1)], axis=0), bf16)
        h = jax.lax.dot_general(x, w, (((1,), (1,)), ((), ())), preferred_element_type=f32) + b1s[0:1, s0:s1]
        u = h * (h * h * (_GC * 0.044715) + _GC)
        hh = 0.5 * h
        hbuf[b][j][:, s0:s1] = _packed(hh * jnp.tanh(u) + hh)

    def mm2_op(b, j, c, fused):
        w = jnp.concatenate([weights(at("w2", c) + s0 // 2, (min(s0 + FC, F) - s0) // 2)
                             for s0 in range(0, F, FC)], axis=0)
        mlp = jnp.dot(pltpu.bitcast(hbuf[b][j][...], bf16), w, preferred_element_type=f32)
        mlp = [mlp[0:P], mlp[P:2 * P]]
        qw = q_words(arena, b, j, c)
        o = [mlp[0] + prm[5:6, lanes[c]] + _lo(qw), mlp[1] + prm[5:6, lanes[c]] + _hi(qw)]
        if fused:
            emit_out(arena, fbuf[b], b, j, c, o)
        else:
            for e in range(2):
                fbuf[b][(2 * j + e) * P:(2 * j + e + 1) * P, lanes[c]] = o[e]

    def fwd_op(b, r, src, dst):
        e = jnp.dot(pltpu.bitcast(fwd_ref[r], bf16), jnp.concatenate([weights(at(src, b, r, c), H) for c in range(nc)], axis=1),
                    preferred_element_type=f32)
        row = (dst * R + r) * SR
        ebuf[b][row:row + P, :] = e[0:P]
        ebuf[b][row + IM:row + IM + P, :] = e[P:2 * P]

    def inv_op(b, r):
        y = jnp.dot(pltpu.bitcast(inv_ref[r], bf16), jnp.concatenate([weights(at("z", b, r, c), P) for c in range(nc)], axis=1),
                    preferred_element_type=f32)
        fbuf[b][(R + r) * P:(R + r + 1) * P, :] = y

    part = functools.partial

    prog = []

    def push(units):
        prog.append(part(queue.extend, units))

    def ln(src, blocks, cost=C_LN):
        keys = [(b, r, s0) for b in blocks for r in range(R) for s0 in range(0, P, LR)]
        tag = lambda n: ("ln", keys[n][0], keys[n][1] // 2)
        return [(tag(max(n - 2, 0)), part(ln_unit, src, keys, n), cost) for n in range(len(keys) + 2)]

    def prep(blocks):
        ts = [(b, c, n) for b in blocks for c in range(nc) for n in range(R)]
        lead, out = [], []
        for i in range(-TL - 1, len(ts)):
            tag, dst = ("prep", ts[max(i, 0)][0]), lead if i < 0 else out
            if i + TL + 1 < len(ts):
                dst.append((tag, part(t_load, *ts[i + TL + 1]), 0))
            for j in range(2):
                if j == 1 and -1 <= i < len(ts) - 1:
                    dst.append((tag, part(t_store, *ts[i + 1]), 0))
                if i >= 0:
                    b, c, n = ts[i]
                    dst += [(tag, part(prep_unit, b, j, c, s0), C_PREP)
                            for s0 in range(n * P // R, (n + 1) * P // R, PR)]

        def enqueue():
            n = 2 * TL + 2
            tail = queue[-n:]
            tail += [(lead[0][0], lambda: None, C_LN)] * (n - len(tail))
            queue[-n:] = mix(tail, lead) + out

        prog.append(enqueue)

    def spectral(b):
        return [(("m", b), part(m_unit, b, g0, c), C_M[b]) for g0 in range(0, P, RG) for c in range(nc)]

    def fin(b, n=nc):
        return [(("fin", b), part(fin_gate, b), 0)] + [
            (("fin", b), part(fin_unit, b, j, c, s0), C_FIN)
            for c in range(n) for j in range(2) for s0 in range(0, P, FR)]

    def mix(main, extra):
        out = []
        for i, u in enumerate(main):
            out += extra[i * len(extra) // len(main):(i + 1) * len(extra) // len(main)] + [u]
        return out

    def mm1(b, lo=0, hi=None):
        for s0, j in [(s0, j) for s0 in range(0, F, FC) for j in range(2)][lo:hi]:
            s1 = min(s0 + FC, F)
            pieces.extend((at("w1", c) + s0 // 2, None, 64 * pl.cdiv(s1 - s0, LANES)) for c in range(nc))
            prog.append(part(mm1_op, b, j, s0, s1))

    def mm2(b, lo=0, hi=None, fused=False):
        for c, j in [(c, j) for c in range(nc) for j in range(2)][lo:hi]:
            pieces.extend((at("w2", c) + s0 // 2, None, 128) for s0 in range(0, F, FC))
            prog.append(part(mm2_op, b, j, c, fused))

    def fwd(b):
        for r in range(R):
            for dst, src in enumerate(("xu", "xk")):
                pieces.extend((at(src, b, r, c), ("prep", b), 64) for c in range(nc))
                prog.append(part(fwd_op, b, r, src, dst))

    def inv(b):
        for r in range(R):
            pieces.extend((at("z", b, r, c), ("m", b), 64) for c in range(nc))
            prog.append(part(inv_op, b, r))

    def run(then_wait=(), then_start=()):
        for step in prog:
            step()
        prog.clear(), pieces.clear(), marks.clear()
        cursor[0] = 0
        credit[0] = -256
        start(then_start)
        wait(then_wait)

    feed = [q_in(0), q_in(1), w1_in(0, 2 * FC, 0) + small_in, w1_in(2 * FC, F, 2),
            q_in(2) + conv_in(0) + tables_in[:1], w2_in + conv_in(1) + q_in(3) + tables_in[1:],
            conv_in(2) + conv_in(3)]
    cuts = [pltpu.make_async_copy(q_hbm.at[0:16, 0:LANES], cut_buf.at[i], cut_sem.at[i]) for i in range(NCUT)]

    def params():
        prm[0:4, :] = shift_ref[...].astype(f32)
        prm[4:5, :] = sd_ref[...].astype(f32).reshape(1, D)
        prm[5:6, :] = b2_ref[...].astype(f32).reshape(1, D)
        b1s[...] = b1_ref[...].astype(f32).reshape(1, F)

    start(feed[0] + feed[1])
    for c in range(nc):
        st(at("k", 0, c), jnp.zeros((8, LANES), u32))
    wait(feed[0])
    start(feed[2])
    push(ln(arena, [0]))
    prog.append(part(need, ("ln", 0, 1)))
    run(feed[1])
    push(ln(arena, [1]))
    prog.append(part(need, ("ln", 1, 1)))
    run(feed[2])
    start(feed[3])
    params()
    mm1(0, 0, 4)
    mm1(1, 0, 4)
    run(feed[3], feed[4] + cuts)
    mm1(0, 4)
    mm1(1, 4, 6)
    run(feed[4], feed[5])
    prep([0])
    mm1(1, 6)
    push(ln(ordered, [2]))
    fwd(0)
    push(spectral(0))
    mm1(2)
    run(feed[5], feed[6])
    prep([1])
    mm2(0, 0, 6)
    push(ln(ordered, [3]))
    fwd(1)
    push(spectral(1))
    mm2(0, 6)
    inv(0)
    mm2(1, 0, 4)
    run(feed[6])
    prep([2, 3])
    mm1(3)
    fwd(2)
    run(cuts[0:1])
    push(spectral(2))
    mm2(1, 4, 6)
    fwd(3)
    mm2(1, 6)
    mm2(2, 0, 2)
    inv(1)
    run(cuts[1:2])
    push(spectral(3))
    mm2(2, 2)
    inv(2)
    mm2(3, 0, 2)
    inv(3)
    push(fin(0) + fin(1) + fin(2) + fin(3, 1))
    mm2(3, 2, fused=True)
    prog.append(part(need, ("fin", 3)))
    run()
    wait(out_copies)


@jax.jit
def pallas_parallel_sum__ssm_conv_h3__dense_activation_gelu__prompt_kernel(
    A_q: jax.Array,
    A_k: jax.Array,
    A_v: jax.Array,
    A_shift_k: jax.Array,
    A_ssm_k: jax.Array,
    A_ssm_D: jax.Array,
    B_x: jax.Array,
    B_w1: jax.Array,
    B_b1: jax.Array,
    B_w2: jax.Array,
    B_b2: jax.Array,
):
    B, S, D = A_q.shape
    F = B_w1.shape[1]
    nc, nb = D // LANES, S // TB
    q, k, v = (a.reshape(S, D) for a in (A_q, A_k, A_v))
    hbm = pl.BlockSpec(memory_space=pltpu.HBM)
    out = pl.pallas_call(
        functools.partial(_kernel, nc=nc, nb=nb, D=D, F=F),
        in_specs=[pl.BlockSpec(memory_space=pltpu.SMEM)] + [hbm] * 12,
        out_specs=hbm,
        out_shape=jax.ShapeDtypeStruct((S, D), A_q.dtype),
        scratch_shapes=[
            pltpu.VMEM((4, D), bf16), pltpu.VMEM((D,), bf16), pltpu.VMEM((F,), bf16), pltpu.VMEM((D,), bf16),
            pltpu.VMEM(_FWD.shape, u32), pltpu.VMEM(_INV.shape, u32),
            pltpu.VMEM((2 * _layout(nb, nc, F)[1], LANES), bf16),
            [pltpu.VMEM((2 * R * SR + 8, D), f32) for _ in range(nb)],
            [pltpu.VMEM((2 * R * P + 8, D), f32) for _ in range(nb)],
            pltpu.VMEM((nc, TB + 16, LANES), bf16),
            pltpu.VMEM((8, D), f32),
            pltpu.VMEM((1, F), f32),
            [[pltpu.VMEM((P, F), u32) for _ in range(2)] for _ in range(nb)],
            pltpu.SemaphoreType.DMA((4, nb)),
            pltpu.SemaphoreType.DMA((6,)),
            pltpu.SemaphoreType.DMA((nb,)),
            pltpu.VMEM((NCUT, 16, LANES), bf16),
            pltpu.SemaphoreType.DMA((NCUT,)),
        ],
        compiler_params=pltpu.CompilerParams(vmem_limit_bytes=120 * 1024 * 1024),
    )(jnp.asarray(np.zeros((1,), np.int32)), q, k, v, A_ssm_k, B_w1.T, B_w2, A_shift_k.T, A_ssm_D, B_b1, B_b2,
      jnp.asarray(_FWD), jnp.asarray(_INV))
    return out.reshape(B, S, D)
```

```python
import functools

import numpy as np
import jax
import jax.numpy as jnp
import jax.experimental.pallas as pl
import jax.experimental.pallas.tpu as pltpu

R = 4
P = 128
H = P // 2
TB = R * P
NFFT = 2 * TB
LANES = 128
IM, SR = P + 8, 2 * P + 24
RG = 8
PR, LR, FR = 16, 32, 64
C_LN, C_PREP, C_FIN, C_M = 135, 72, 105, (132, 134, 125, 130)
LAG, TL, PT, NCUT = 2, 2, 5, 2
FC = 256


def _pack_rows(m):
    u = np.ascontiguousarray(m, np.float32).view(np.uint32).astype(np.uint64)
    h = ((u + 0x7FFF + ((u >> 16) & 1)) >> 16).astype(np.uint32)
    return h[..., 0::2, :] | (h[..., 1::2, :] << np.uint32(16))


def _dft_tables():
    g = np.concatenate([np.arange(0, P, 2), np.arange(1, P, 2)]).astype(np.float64)
    s = np.arange(P, dtype=np.float64)
    fwd, inv = [], []
    for r in range(R):
        th = 2.0 * np.pi * (g[:, None] + 0.5) * (R * s[None, :] + r) / NFFT
        fwd.append(np.concatenate([np.cos(th), -np.sin(th)], 0))
        inv.append(np.stack([np.cos(th).T, -np.sin(th).T], 2).reshape(P, 2 * P) * (2.0 / NFFT))
    return _pack_rows(np.stack(fwd)), _pack_rows(np.stack(inv))


_FWD, _INV = _dft_tables()
_GC = float(np.sqrt(2.0 / np.pi))
f32, bf16, u32 = jnp.float32, jnp.bfloat16, jnp.uint32


def _layout(nb, nc, F):
    spec = dict(q=(nb * nc, TB // 2 + 8), k=(nb * nc, 8 + TB // 2 + 8),
                v=(nb * nc, TB // 2 + 8), kt=(nb * nc, TB // 2 + 8),
                sk=(nb * R * nc, H),
                o=(nb * nc, TB // 2 + 8), w1=(nc, F // 2), w2=(nc, F // 2),
                xn=(nb * R * nc, H), xu=(nb * R * nc, H), xk=(nb * R * nc, H),
                u=((nb - 1) * R * nc, SR), kf=((nb - 1) * R * nc, SR), kp=((nb - 1) * R * nc, SR),
                z=(nb * R * nc, P + 8), tick=(1, 8))
    off, out = 0, {}
    for name, (n, rows) in spec.items():
        out[name] = (off, rows)
        off += n * rows
    return out, off


def _lo(w):
    return pltpu.bitcast(w << 16, f32)


def _hi(w):
    return pltpu.bitcast(w & np.uint32(0xFFFF0000), f32)


def _packed(x):
    return pltpu.bitcast(x.astype(bf16), u32)


def _pair(a, b):
    return pltpu.bitcast(pltpu.pack_elementwise([a, b], packed_dtype=bf16), u32)


def _kernel(zero_ref, q_hbm, k_hbm, v_hbm, sk_hbm, w1_hbm, w2_hbm,
            shift_hbm, sd_hbm, b1_hbm, b2_hbm, fwd_hbm, inv_hbm,
            o_hbm,
            shift_ref, sd_ref, b1_ref, b2_ref, fwd_ref, inv_ref,
            arena16, ebuf, fbuf, obuf, prm, b1s, hbuf, in_sem, w_sem, out_sem, cut_buf, cut_sem, *, nc, nb, D, F):
    lanes = [slice(c * LANES, (c + 1) * LANES) for c in range(nc)]
    lay, _ = _layout(nb, nc, F)
    arena = arena16.bitcast(u32)
    zero = pl.multiple_of(zero_ref[0], 8)

    i0 = jnp.zeros((), jnp.int32)

    def rows(start, n):
        return pl.ds(pl.multiple_of(i0 + start, 8), n)

    def late(ref):
        return ref.at[pl.ds(zero, ref.shape[0]), :]

    ordered = late(arena)
    e_ord, f_ord = [late(r) for r in ebuf], [late(r) for r in fbuf]
    E_ROWS, F_ROWS = 2 * R * SR, 2 * R * P

    def at(name, *idx):
        n = 0
        for i in idx[:-1]:
            n = n * R + i
        return lay[name][0] + (n * nc + idx[-1]) * lay[name][1]

    def ld(row, n):
        return pltpu.bitcast(ordered[rows(row, n), :], f32)

    def st(row, val):
        arena[rows(row, val.shape[0]), :] = pltpu.bitcast(val, u32)

    def slab16(row, n):
        return arena16.at[2 * row:2 * (row + n), :]

    def wide(name, *idx):
        return jnp.concatenate([arena[rows(at(name, *idx, c), lay[name][1]), :] for c in range(nc)], axis=1)

    def cols_in(src, b, offs, sem, history=0):
        return [pltpu.make_async_copy(src.at[pl.ds(b * TB - 2 * history, TB + 2 * history), lanes[c]],
                                      slab16(offs[c] - history, TB // 2 + history), sem) for c in range(nc)]

    def conv_in(b):
        return (cols_in(k_hbm, b, [at("k", b, c) + 8 for c in range(nc)], in_sem.at[0, b], 8 if b else 0)
                + cols_in(v_hbm, b, [at("v", b, c) for c in range(nc)], in_sem.at[1, b])
                + [pltpu.make_async_copy(sk_hbm.at[lanes[c], pl.ds(b * TB + n * P, P)],
                                         slab16(at("sk", b, n, c), H), in_sem.at[2, b])
                   for c in range(nc) for n in range(R)])

    def q_in(b):
        return cols_in(q_hbm, b, [at("q", b, c) for c in range(nc)], in_sem.at[3, b])

    out_copies = []

    def out_copy(b, c, src):
        return pltpu.make_async_copy(slab16(at("o", b, c), TB // 2) if src is ordered else obuf.at[c, 0:TB, :],
                                     o_hbm.at[pl.ds(b * TB, TB), lanes[c]], out_sem.at[b])

    def w1_in(lo, hi, n):
        return [pltpu.make_async_copy(w1_hbm.at[lo:hi, lanes[c]], slab16(at("w1", c) + lo // 2, (hi - lo) // 2),
                                      w_sem.at[n]) for c in range(nc)]

    small_in = [pltpu.make_async_copy(src, dst, w_sem.at[3]) for src, dst in (
        (shift_hbm, shift_ref), (sd_hbm, sd_ref), (b1_hbm, b1_ref), (b2_hbm, b2_ref))]
    tables_in = [pltpu.make_async_copy(fwd_hbm, fwd_ref, w_sem.at[4]),
                 pltpu.make_async_copy(inv_hbm, inv_ref, w_sem.at[5])]
    w2_in = [pltpu.make_async_copy(w2_hbm.at[:, lanes[c]], slab16(at("w2", c), F // 2), w_sem.at[1])
             for c in range(nc)]

    def start(cs):
        for c in cs:
            c.start()

    def wait(cs):
        for c in cs:
            c.wait()

    def delayed(x, n):
        for _ in range(n):
            x = jnp.tanh(x)
        return x

    tiles = {}

    def t_load(b, c, n):
        w = pltpu.bitcast(ordered[rows(at("sk", b, n, c), H), :], bf16)
        tiles[b, c, n] = pltpu.bitcast(w.T, u32)

    def t_store(b, c, n):
        st(at("kt", b, c) + n * H, tiles.pop((b, c, n)))

    def prep_unit(b, j, c, s0):
        base = at("k", b, c) + 8 + j + 2 * s0
        t = ordered[rows(at("k", b, c), 8), :]
        t = delayed(pltpu.bitcast(t, f32), PT)

        wa = ordered[pl.ds(base - 2, PR, stride=2), :]
        wb = ordered[pl.ds(base - 1, PR, stride=2), :]
        wc = ordered[pl.ds(base, PR, stride=2), :]
        ks = [_hi(wa), _lo(wb), _hi(wb), _lo(wc), _hi(wc)]
        vw = ordered[pl.ds(at("v", b, c) + j + 2 * s0, PR, stride=2), :]
        vs = [_lo(vw), _hi(vw)]
        tw = ordered[pl.ds(at("kt", b, c) + j + 2 * s0, PR, stride=2), :]
        ts = [_lo(tw), _hi(tw)]
        for e in range(2):
            acc = ks[3 + e] * prm[0:1, lanes[c]]
            for i in range(1, 4):
                acc = acc + ks[3 + e - i] * prm[i:i + 1, lanes[c]]
            st(at("xu", b, 2 * j + e, c) + s0 // 2, _packed(acc * vs[e]))
            st(at("xk", b, 2 * j + e, c) + s0 // 2, _packed(ts[e]))
        st(at("tick", 0), t)

    def m_unit(b, g0, c):
        def cld(name, slot, m):
            row = at(name, slot, m, c) + g0
            return ld(row, RG), ld(row + IM, RG)

        def cst(name, m, vr, vi):
            row = at(name, b, m, c) + g0
            st(row, vr)
            st(row + IM, vi)

        def bfly(which):
            offs = [(which * R + r) * SR + g0 for r in range(R)]
            er = [e_ord[b][rows(o, RG), lanes[c]] for o in offs]
            ei = [e_ord[b][rows(o + IM, RG), lanes[c]] for o in offs]
            ar, ai = er[0] + er[2], ei[0] + ei[2]
            br, bi = er[0] - er[2], ei[0] - ei[2]
            cr, ci = er[1] + er[3], ei[1] + ei[3]
            dr, di = er[1] - er[3], ei[1] - ei[3]
            return ([ar + cr, br + di, ar - cr, br - di],
                    [ai + ci, bi - dr, ai - ci, bi + dr])

        tick = pltpu.roll(e_ord[b][rows(g0, RG), lanes[c]], 1, 1)
        ur, ui = bfly(0)
        kr, ki = bfly(1)
        if b == 0:
            kr = [x + prm[4:5, lanes[c]] for x in kr]
        keep = []
        for m in range(R):
            if b == 0:
                keep.append((kr[m], ki[m]))
            else:
                pr, pi = cld("kp", b - 1, m)
                keep.append((kr[m] - pi, ki[m] + pr) if g0 < P // 2 else (kr[m] + pi, ki[m] - pr))
        if b < nb - 1:
            for m in range(R):
                cst("kp", m, kr[m], ki[m])
                cst("u", m, ur[m], ui[m])
                cst("kf", m, *keep[m])
        else:
            st(at("tick", 0), keep[R - 1][1])
        yr, yi = [], []
        for m in range(R):
            accr = acci = None
            for jj in range(b + 1):
                a_r, a_i = (ur[m], ui[m]) if jj == b else cld("u", jj, m)
                b_r, b_i = keep[m] if jj == 0 else cld("kf", b - jj, m)
                pr_ = a_r * b_r - a_i * b_i
                pi_ = a_r * b_i + a_i * b_r
                accr = pr_ if accr is None else accr + pr_
                acci = pi_ if acci is None else acci + pi_
            yr.append(accr)
            yi.append(acci)
            if b >= 2 and m == 1:
                st(at("tick", 0), acci)
        ar, ai = yr[0] + yr[2], yi[0] + yi[2]
        br, bi = yr[0] - yr[2], yi[0] - yi[2]
        cr, ci = yr[1] + yr[3], yi[1] + yi[3]
        dr, di = yr[1] - yr[3], yi[1] - yi[3]
        zr = [ar + cr, br - di, ar - cr, br + di]
        zi = [ai + ci, bi + dr, ai - ci, bi - dr]
        for r in range(R):
            st(at("z", b, r, c) + g0, _pair(zr[r], zi[r]))
        ebuf[b][E_ROWS:E_ROWS + RG, 0:LANES] = tick
        st(at("tick", 0), tick)

    def q_words(src, b, j, c):
        return src[pl.ds(at("q", b, c) + j, P, stride=2), :]

    def ln_rows(src, b, r, s0):
        return jnp.concatenate([(_lo, _hi)[r % 2](src[pl.ds(at("q", b, c) + r // 2 + 2 * s0, LR, stride=2), :])
                                for c in range(nc)], axis=1)

    mean, rstd = {}, {}

    def ln_mean(src, key):
        mean[key] = jnp.mean(ln_rows(src, *key), axis=-1, keepdims=True)

    def ln_rstd(src, key):
        xc = ln_rows(src, *key) - mean[key]
        rstd[key] = jax.lax.rsqrt(jnp.mean(xc * xc, axis=-1, keepdims=True) + 1e-5)

    def ln_store(src, key):
        b, r, s0 = key
        xn = _packed((ln_rows(src, *key) - mean.pop(key)) * rstd.pop(key))
        for c in range(nc):
            st(at("xn", b, r, c) + s0 // 2, xn[:, lanes[c]])

    def ln_unit(src, keys, n):
        for stage, fn in enumerate((ln_mean, ln_rstd, ln_store)):
            if 0 <= n - stage < len(keys):
                fn(src, keys[n - stage])

    def emit_out(src, fsrc, b, j, c, o, s0=0):
        n = o[0].shape[0]
        outs = []
        for e in range(2):
            r = 2 * j + e
            xn = pltpu.bitcast(src[rows(at("xn", b, r, c) + s0 // 2, n // 2), :], bf16).astype(f32)
            outs.append(o[e] + xn * fsrc[(R + r) * P + s0:(R + r) * P + s0 + n, lanes[c]])
        if src is ordered:
            arena[pl.ds(at("o", b, c) + j + 2 * s0, n, stride=2), :] = _pair(*outs)
        else:
            obuf.at[c].bitcast(u32)[pl.ds(j + 2 * s0, n, stride=2), :] = _pair(*outs)
        if j == 1 and s0 + n == P:
            out_copies.append(out_copy(b, c, src))
            out_copies[-1].start()

    def fin_gate(b):
        fbuf[b][F_ROWS:F_ROWS + 8, 0:LANES] = ld(at("k", 0, 0), 8)

    def fin_unit(b, j, c, s0):
        o = [f_ord[b][(2 * j + e) * P + s0:(2 * j + e) * P + s0 + FR, lanes[c]] for e in range(2)]
        tick = delayed(f_ord[b][0:8, lanes[c]], 7)
        emit_out(ordered, f_ord[b], b, j, c, o, s0)
        fbuf[b][F_ROWS:F_ROWS + 8, 0:LANES] = tick
        st(at("tick", 0), tick)

    queue = []
    credit = [0]

    def fill(cycles):
        credit[0] += cycles
        while queue and credit[0] >= queue[0][2]:
            _, fn, cost = queue.pop(0)
            credit[0] -= cost
            fn()
        if not queue:
            credit[0] = min(credit[0], 128)

    def need(tag):
        while any(t == tag for t, _, _ in queue):
            queue.pop(0)[1]()

    marks = {}
    pieces = []
    cursor = [0]

    def weights(row, n):
        i = cursor[0]
        assert pieces[i][0] == row
        cursor[0] += 1
        for p in range(len(marks), min(i + 1 + LAG, len(pieces))):
            need(pieces[p][1])
            marks[p] = ordered[rows(pieces[p][0], 8), :]
            fill(pieces[p][2])
        return pltpu.bitcast(jnp.concatenate([marks[i], arena[rows(row + 8, n - 8), :]], axis=0), bf16)

    def mm1_op(b, j, s0, s1):
        need(("ln", b, j))
        w = jnp.concatenate([weights(at("w1", c) + s0 // 2, (s1 - s0) // 2) for c in range(nc)], axis=1)
        x = pltpu.bitcast(jnp.concatenate([wide("xn", b, 2 * j), wide("xn", b, 2 * j + 1)], axis=0), bf16)
        h = jax.lax.dot_general(x, w, (((1,), (1,)), ((), ())), preferred_element_type=f32) + b1s[0:1, s0:s1]
        u = h * (h * h * (_GC * 0.044715) + _GC)
        hh = 0.5 * h
        hbuf[b][j][:, s0:s1] = _packed(hh * jnp.tanh(u) + hh)

    def mm2_op(b, j, c, fused):
        w = jnp.concatenate([weights(at("w2", c) + s0 // 2, (min(s0 + FC, F) - s0) // 2)
                             for s0 in range(0, F, FC)], axis=0)
        mlp = jnp.dot(pltpu.bitcast(hbuf[b][j][...], bf16), w, preferred_element_type=f32)
        mlp = [mlp[0:P], mlp[P:2 * P]]
        qw = q_words(arena, b, j, c)
        o = [mlp[0] + prm[5:6, lanes[c]] + _lo(qw), mlp[1] + prm[5:6, lanes[c]] + _hi(qw)]
        if fused:
            emit_out(arena, fbuf[b], b, j, c, o)
        else:
            for e in range(2):
                fbuf[b][(2 * j + e) * P:(2 * j + e + 1) * P, lanes[c]] = o[e]

    def fwd_op(b, r, src, dst):
        x = jnp.concatenate([weights(at(src, b, r, c), H) for c in range(nc)], axis=1)
        e = jnp.dot(pltpu.bitcast(fwd_ref[r], bf16), x, preferred_element_type=f32)
        row = (dst * R + r) * SR
        ebuf[b][row:row + P, :] = e[0:P]
        ebuf[b][row + IM:row + IM + P, :] = e[P:2 * P]

    def inv_op(b, r):
        z = jnp.concatenate([weights(at("z", b, r, c), P) for c in range(nc)], axis=1)
        fbuf[b][(R + r) * P:(R + r + 1) * P, :] = jnp.dot(pltpu.bitcast(inv_ref[r], bf16), z,
                                                         preferred_element_type=f32)

    part = functools.partial

    prog = []

    def push(units):
        prog.append(part(queue.extend, units))

    def ln(src, blocks):
        keys = [(b, r, s0) for b in blocks for r in range(R) for s0 in range(0, P, LR)]
        tag = lambda n: ("ln", keys[n][0], keys[n][1] // 2)
        return [(tag(max(n - 2, 0)), part(ln_unit, src, keys, n), C_LN) for n in range(len(keys) + 2)]

    def prep(blocks):
        ts = [(b, c, n) for b in blocks for c in range(nc) for n in range(R)]
        lead, out = [], []
        for i in range(-TL - 1, len(ts)):
            tag, dst = ("prep", ts[max(i, 0)][0]), lead if i < 0 else out
            if i + TL + 1 < len(ts):
                dst.append((tag, part(t_load, *ts[i + TL + 1]), 0))
            for j in range(2):
                if j == 1 and -1 <= i < len(ts) - 1:
                    dst.append((tag, part(t_store, *ts[i + 1]), 0))
                if i >= 0:
                    b, c, n = ts[i]
                    dst += [(tag, part(prep_unit, b, j, c, s0), C_PREP)
                            for s0 in range(n * P // R, (n + 1) * P // R, PR)]

        def enqueue():
            n = 2 * TL + 2
            tail = queue[-n:]
            tail += [(lead[0][0], lambda: None, C_LN)] * (n - len(tail))
            queue[-n:] = mix(tail, lead) + out

        prog.append(enqueue)

    def spectral(b):
        return [(("m", b), part(m_unit, b, g0, c), C_M[b]) for g0 in range(0, P, RG) for c in range(nc)]

    def fin(b, n=nc):
        return [(("fin", b), part(fin_gate, b), 0)] + [
            (("fin", b), part(fin_unit, b, j, c, s0), C_FIN)
            for c in range(n) for j in range(2) for s0 in range(0, P, FR)]

    def mix(main, extra):
        out = []
        for i, u in enumerate(main):
            out += extra[i * len(extra) // len(main):(i + 1) * len(extra) // len(main)] + [u]
        return out

    def mm1(b, lo=0, hi=None):
        for s0, j in [(s0, j) for s0 in range(0, F, FC) for j in range(2)][lo:hi]:
            s1 = min(s0 + FC, F)
            pieces.extend((at("w1", c) + s0 // 2, None, 64 * pl.cdiv(s1 - s0, LANES)) for c in range(nc))
            prog.append(part(mm1_op, b, j, s0, s1))

    def mm2(b, lo=0, hi=None, fused=False):
        for c, j in [(c, j) for c in range(nc) for j in range(2)][lo:hi]:
            pieces.extend((at("w2", c) + s0 // 2, None, 128) for s0 in range(0, F, FC))
            prog.append(part(mm2_op, b, j, c, fused))

    def fwd(b):
        for r in range(R):
            for dst, src in enumerate(("xu", "xk")):
                pieces.extend((at(src, b, r, c), ("prep", b), 64) for c in range(nc))
                prog.append(part(fwd_op, b, r, src, dst))

    def inv(b):
        for r in range(R):
            pieces.extend((at("z", b, r, c), ("m", b), 64) for c in range(nc))
            prog.append(part(inv_op, b, r))

    def run(then_wait=(), then_start=()):
        for step in prog:
            step()
        prog.clear(), pieces.clear(), marks.clear()
        cursor[0] = 0
        credit[0] = -256
        start(then_start)
        wait(then_wait)

    feed = [q_in(0), q_in(1), w1_in(0, 2 * FC, 0) + small_in, w1_in(2 * FC, F, 2),
            q_in(2) + conv_in(0) + tables_in[:1], w2_in + conv_in(1) + q_in(3) + tables_in[1:],
            conv_in(2) + conv_in(3)]
    cuts = [pltpu.make_async_copy(q_hbm.at[0:16, 0:LANES], cut_buf.at[i], cut_sem.at[i]) for i in range(NCUT)]

    def params():
        prm[0:4, :] = shift_ref[...].astype(f32)
        prm[4:5, :] = sd_ref[...].astype(f32).reshape(1, D)
        prm[5:6, :] = b2_ref[...].astype(f32).reshape(1, D)
        b1s[...] = b1_ref[...].astype(f32).reshape(1, F)

    start(feed[0] + feed[1])
    for c in range(nc):
        st(at("k", 0, c), jnp.zeros((8, LANES), u32))
    wait(feed[0])
    start(feed[2])
    push(ln(arena, [0]))
    prog.append(part(need, ("ln", 0, 1)))
    run(feed[1])
    push(ln(arena, [1]))
    prog.append(part(need, ("ln", 1, 1)))
    run(feed[2])
    start(feed[3])
    params()
    mm1(0, 0, 4)
    mm1(1, 0, 4)
    run(feed[3], feed[4] + cuts)
    mm1(0, 4)
    mm1(1, 4, 6)
    run(feed[4], feed[5])
    prep([0])
    mm1(1, 6)
    push(ln(ordered, [2]))
    fwd(0)
    push(spectral(0))
    mm1(2)
    run(feed[5], feed[6])
    prep([1])
    mm2(0, 0, 6)
    push(ln(ordered, [3]))
    fwd(1)
    push(spectral(1))
    mm2(0, 6)
    inv(0)
    mm2(1, 0, 4)
    run(feed[6])
    prep([2, 3])
    mm1(3)
    fwd(2)
    run(cuts[0:1])
    push(spectral(2))
    mm2(1, 4, 6)
    fwd(3)
    mm2(1, 6)
    mm2(2, 0, 2)
    inv(1)
    run(cuts[1:2])
    push(spectral(3))
    mm2(2, 2)
    inv(2)
    mm2(3, 0, 2)
    inv(3)
    push(fin(0) + fin(1) + fin(2) + fin(3, 1))
    mm2(3, 2, fused=True)
    prog.append(part(need, ("fin", 3)))
    run()
    wait(out_copies)


@jax.jit
def pallas_parallel_sum__ssm_conv_h3__dense_activation_gelu__prompt_kernel(
    A_q: jax.Array,
    A_k: jax.Array,
    A_v: jax.Array,
    A_shift_k: jax.Array,
    A_ssm_k: jax.Array,
    A_ssm_D: jax.Array,
    B_x: jax.Array,
    B_w1: jax.Array,
    B_b1: jax.Array,
    B_w2: jax.Array,
    B_b2: jax.Array,
):
    B, S, D = A_q.shape
    F = B_w1.shape[1]
    nc, nb = D // LANES, S // TB
    assert (B, nb, D % LANES, F // FC, A_shift_k.shape[1]) == (1, 4, 0, 6, 4)
    q, k, v = (a.reshape(S, D) for a in (A_q, A_k, A_v))
    hbm = pl.BlockSpec(memory_space=pltpu.HBM)
    out = pl.pallas_call(
        functools.partial(_kernel, nc=nc, nb=nb, D=D, F=F),
        in_specs=[pl.BlockSpec(memory_space=pltpu.SMEM)] + [hbm] * 12,
        out_specs=hbm,
        out_shape=jax.ShapeDtypeStruct((S, D), A_q.dtype),
        scratch_shapes=[
            pltpu.VMEM((4, D), bf16), pltpu.VMEM((D,), bf16), pltpu.VMEM((F,), bf16), pltpu.VMEM((D,), bf16),
            pltpu.VMEM(_FWD.shape, u32), pltpu.VMEM(_INV.shape, u32),
            pltpu.VMEM((2 * _layout(nb, nc, F)[1], LANES), bf16),
            [pltpu.VMEM((2 * R * SR + 8, D), f32) for _ in range(nb)],
            [pltpu.VMEM((2 * R * P + 8, D), f32) for _ in range(nb)],
            pltpu.VMEM((nc, TB + 16, LANES), bf16),
            pltpu.VMEM((8, D), f32),
            pltpu.VMEM((1, F), f32),
            [[pltpu.VMEM((P, F), u32) for _ in range(2)] for _ in range(nb)],
            pltpu.SemaphoreType.DMA((4, nb)),
            pltpu.SemaphoreType.DMA((6,)),
            pltpu.SemaphoreType.DMA((nb,)),
            pltpu.VMEM((NCUT, 16, LANES), bf16),
            pltpu.SemaphoreType.DMA((NCUT,)),
        ],
        compiler_params=pltpu.CompilerParams(vmem_limit_bytes=120 * 1024 * 1024),
    )(jnp.asarray(np.zeros((1,), np.int32)), q, k, v, A_ssm_k, B_w1.T, B_w2, A_shift_k.T, A_ssm_D, B_b1, B_b2,
      jnp.asarray(_FWD), jnp.asarray(_INV))
    return out.reshape(B, S, D)
```

```python
import functools

import numpy as np
import jax
import jax.numpy as jnp
import jax.experimental.pallas as pl
import jax.experimental.pallas.tpu as pltpu

R = 4
P = 128
H = P // 2
TB = R * P
NFFT = 2 * TB
LANES = 128
IM, SR = P + 8, 2 * P + 24
RG = 8
PR, LR, FR = 16, 32, 64
C_LN, C_PREP, C_FIN, C_M = 135, 72, 105, (132, 134, 125, 130)
LAG, TL, PT, NCUT = 2, 2, 5, 2
FC = 256


def _pack_rows(m):
    u = np.ascontiguousarray(m, np.float32).view(np.uint32).astype(np.uint64)
    h = ((u + 0x7FFF + ((u >> 16) & 1)) >> 16).astype(np.uint32)
    return h[..., 0::2, :] | (h[..., 1::2, :] << np.uint32(16))


def _dft_tables():
    g = np.concatenate([np.arange(0, P, 2), np.arange(1, P, 2)]).astype(np.float64)
    s = np.arange(P, dtype=np.float64)
    fwd, inv = [], []
    for r in range(R):
        th = 2.0 * np.pi * (g[:, None] + 0.5) * (R * s[None, :] + r) / NFFT
        fwd.append(np.concatenate([np.cos(th), -np.sin(th)], 0))
        inv.append(np.stack([np.cos(th).T, -np.sin(th).T], 2).reshape(P, 2 * P) * (2.0 / NFFT))
    return _pack_rows(np.stack(fwd)), _pack_rows(np.stack(inv))


_FWD, _INV = _dft_tables()
_GC = float(np.sqrt(2.0 / np.pi))
f32, bf16, u32 = jnp.float32, jnp.bfloat16, jnp.uint32


def _layout(nb, nc, F):
    spec = dict(q=(nb * nc, TB // 2 + 8), k=(nb * nc, 8 + TB // 2 + 8),
                v=(nb * nc, TB // 2 + 8), kt=(nb * nc, TB // 2 + 8),
                sk=(nb * R * nc, H),
                o=(nb * nc, TB // 2 + 8), w1=(nc, F // 2), w2=(nc, F // 2),
                xn=(nb * R * nc, H), xu=(nb * R * nc, H), xk=(nb * R * nc, H),
                u=((nb - 1) * R * nc, SR), kf=((nb - 1) * R * nc, SR), kp=((nb - 1) * R * nc, SR),
                z=(nb * R * nc, P + 8), tick=(1, 8))
    off, out = 0, {}
    for name, (n, rows) in spec.items():
        out[name] = (off, rows)
        off += n * rows
    return out, off


def _lo(w):
    return pltpu.bitcast(w << 16, f32)


def _hi(w):
    return pltpu.bitcast(w & np.uint32(0xFFFF0000), f32)


def _packed(x):
    return pltpu.bitcast(x.astype(bf16), u32)


def _pair(a, b):
    return pltpu.bitcast(pltpu.pack_elementwise([a, b], packed_dtype=bf16), u32)


def _kernel(zero_ref, q_hbm, k_hbm, v_hbm, sk_hbm, w1_hbm, w2_hbm,
            shift_hbm, sd_hbm, b1_hbm, b2_hbm, fwd_hbm, inv_hbm,
            o_hbm,
            shift_ref, sd_ref, b1_ref, b2_ref, fwd_ref, inv_ref,
            arena16, ebuf, fbuf, obuf, prm, b1s, hbuf, in_sem, w_sem, out_sem, cut_buf, cut_sem, *, nc, nb, D, F):
    lanes = [slice(c * LANES, (c + 1) * LANES) for c in range(nc)]
    lay, _ = _layout(nb, nc, F)
    arena = arena16.bitcast(u32)
    zero = pl.multiple_of(zero_ref[0], 8)

    i0 = jnp.zeros((), jnp.int32)

    def rows(start, n):
        return pl.ds(pl.multiple_of(i0 + start, 8), n)

    def late(ref):
        return ref.at[pl.ds(zero, ref.shape[0]), :]

    ordered = late(arena)
    e_ord, f_ord = [late(r) for r in ebuf], [late(r) for r in fbuf]
    E_ROWS, F_ROWS = 2 * R * SR, 2 * R * P

    def at(name, *idx):
        n = 0
        for i in idx[:-1]:
            n = n * R + i
        return lay[name][0] + (n * nc + idx[-1]) * lay[name][1]

    def ld(row, n):
        return pltpu.bitcast(ordered[rows(row, n), :], f32)

    def st(row, val):
        arena[rows(row, val.shape[0]), :] = pltpu.bitcast(val, u32)

    def slab16(row, n):
        return arena16.at[2 * row:2 * (row + n), :]

    def wide(name, *idx):
        return jnp.concatenate([arena[rows(at(name, *idx, c), lay[name][1]), :] for c in range(nc)], axis=1)

    def cols_in(src, b, offs, sem, history=0):
        return [pltpu.make_async_copy(src.at[pl.ds(b * TB - 2 * history, TB + 2 * history), lanes[c]],
                                      slab16(offs[c] - history, TB // 2 + history), sem) for c in range(nc)]

    def conv_in(b):
        return (cols_in(k_hbm, b, [at("k", b, c) + 8 for c in range(nc)], in_sem.at[0, b], 8 if b else 0)
                + cols_in(v_hbm, b, [at("v", b, c) for c in range(nc)], in_sem.at[1, b])
                + [pltpu.make_async_copy(sk_hbm.at[lanes[c], pl.ds(b * TB + n * P, P)],
                                         slab16(at("sk", b, n, c), H), in_sem.at[2, b])
                   for c in range(nc) for n in range(R)])

    def q_in(b):
        return cols_in(q_hbm, b, [at("q", b, c) for c in range(nc)], in_sem.at[3, b])

    out_copies = []

    def out_copy(b, c, src):
        return pltpu.make_async_copy(slab16(at("o", b, c), TB // 2) if src is ordered else obuf.at[c, 0:TB, :],
                                     o_hbm.at[pl.ds(b * TB, TB), lanes[c]], out_sem.at[b])

    def w1_in(lo, hi, n):
        return [pltpu.make_async_copy(w1_hbm.at[lo:hi, lanes[c]], slab16(at("w1", c) + lo // 2, (hi - lo) // 2),
                                      w_sem.at[n]) for c in range(nc)]

    small_in = [pltpu.make_async_copy(src, dst, w_sem.at[3]) for src, dst in (
        (shift_hbm, shift_ref), (sd_hbm, sd_ref), (b1_hbm, b1_ref), (b2_hbm, b2_ref))]
    tables_in = [pltpu.make_async_copy(fwd_hbm, fwd_ref, w_sem.at[4]),
                 pltpu.make_async_copy(inv_hbm, inv_ref, w_sem.at[5])]
    w2_in = [pltpu.make_async_copy(w2_hbm.at[:, lanes[c]], slab16(at("w2", c), F // 2), w_sem.at[1])
             for c in range(nc)]

    def start(cs):
        for c in cs:
            c.start()

    def wait(cs):
        for c in cs:
            c.wait()

    def delayed(x, n):
        for _ in range(n):
            x = jnp.tanh(x)
        return x

    tiles = {}

    def t_load(b, c, n):
        w = pltpu.bitcast(ordered[rows(at("sk", b, n, c), H), :], bf16)
        tiles[b, c, n] = pltpu.bitcast(w.T, u32)

    def t_store(b, c, n):
        st(at("kt", b, c) + n * H, tiles.pop((b, c, n)))

    def prep_unit(b, j, c, s0):
        base = at("k", b, c) + 8 + j + 2 * s0
        t = ordered[rows(at("k", b, c), 8), :]
        t = delayed(pltpu.bitcast(t, f32), PT)

        wa = ordered[pl.ds(base - 2, PR, stride=2), :]
        wb = ordered[pl.ds(base - 1, PR, stride=2), :]
        wc = ordered[pl.ds(base, PR, stride=2), :]
        ks = [_hi(wa), _lo(wb), _hi(wb), _lo(wc), _hi(wc)]
        vw = ordered[pl.ds(at("v", b, c) + j + 2 * s0, PR, stride=2), :]
        vs = [_lo(vw), _hi(vw)]
        tw = ordered[pl.ds(at("kt", b, c) + j + 2 * s0, PR, stride=2), :]
        ts = [_lo(tw), _hi(tw)]
        for e in range(2):
            acc = ks[3 + e] * prm[0:1, lanes[c]]
            for i in range(1, 4):
                acc = acc + ks[3 + e - i] * prm[i:i + 1, lanes[c]]
            st(at("xu", b, 2 * j + e, c) + s0 // 2, _packed(acc * vs[e]))
            st(at("xk", b, 2 * j + e, c) + s0 // 2, _packed(ts[e]))
        st(at("tick", 0), t)

    def m_unit(b, g0, c):
        def cld(name, slot, m):
            row = at(name, slot, m, c) + g0
            return ld(row, RG), ld(row + IM, RG)

        def cst(name, m, vr, vi):
            row = at(name, b, m, c) + g0
            st(row, vr)
            st(row + IM, vi)

        def bfly(which):
            offs = [(which * R + r) * SR + g0 for r in range(R)]
            er = [e_ord[b][rows(o, RG), lanes[c]] for o in offs]
            ei = [e_ord[b][rows(o + IM, RG), lanes[c]] for o in offs]
            ar, ai = er[0] + er[2], ei[0] + ei[2]
            br, bi = er[0] - er[2], ei[0] - ei[2]
            cr, ci = er[1] + er[3], ei[1] + ei[3]
            dr, di = er[1] - er[3], ei[1] - ei[3]
            return ([ar + cr, br + di, ar - cr, br - di],
                    [ai + ci, bi - dr, ai - ci, bi + dr])

        tick = pltpu.roll(e_ord[b][rows(g0, RG), lanes[c]], 1, 1)
        ur, ui = bfly(0)
        kr, ki = bfly(1)
        if b == 0:
            kr = [x + prm[4:5, lanes[c]] for x in kr]
        keep = []
        for m in range(R):
            if b == 0:
                keep.append((kr[m], ki[m]))
            else:
                pr, pi = cld("kp", b - 1, m)
                keep.append((kr[m] - pi, ki[m] + pr) if g0 < P // 2 else (kr[m] + pi, ki[m] - pr))
        if b < nb - 1:
            for m in range(R):
                cst("kp", m, kr[m], ki[m])
                cst("u", m, ur[m], ui[m])
                cst("kf", m, *keep[m])
        else:
            st(at("tick", 0), keep[R - 1][1])
        yr, yi = [], []
        for m in range(R):
            accr = acci = None
            for jj in range(b + 1):
                a_r, a_i = (ur[m], ui[m]) if jj == b else cld("u", jj, m)
                b_r, b_i = keep[m] if jj == 0 else cld("kf", b - jj, m)
                pr_ = a_r * b_r - a_i * b_i
                pi_ = a_r * b_i + a_i * b_r
                accr = pr_ if accr is None else accr + pr_
                acci = pi_ if acci is None else acci + pi_
            yr.append(accr)
            yi.append(acci)
            if b >= 2 and m == 1:
                st(at("tick", 0), acci)
        ar, ai = yr[0] + yr[2], yi[0] + yi[2]
        br, bi = yr[0] - yr[2], yi[0] - yi[2]
        cr, ci = yr[1] + yr[3], yi[1] + yi[3]
        dr, di = yr[1] - yr[3], yi[1] - yi[3]
        zr = [ar + cr, br - di, ar - cr, br + di]
        zi = [ai + ci, bi + dr, ai - ci, bi - dr]
        for r in range(R):
            st(at("z", b, r, c) + g0, _pair(zr[r], zi[r]))
        ebuf[b][E_ROWS:E_ROWS + RG, 0:LANES] = tick
        st(at("tick", 0), tick)

    def q_words(src, b, j, c):
        return src[pl.ds(at("q", b, c) + j, P, stride=2), :]

    def ln_rows(src, b, r, s0):
        return jnp.concatenate([(_lo, _hi)[r % 2](src[pl.ds(at("q", b, c) + r // 2 + 2 * s0, LR, stride=2), :])
                                for c in range(nc)], axis=1)

    mean, rstd = {}, {}

    def ln_mean(src, key):
        mean[key] = jnp.mean(ln_rows(src, *key), axis=-1, keepdims=True)

    def ln_rstd(src, key):
        xc = ln_rows(src, *key) - mean[key]
        rstd[key] = jax.lax.rsqrt(jnp.mean(xc * xc, axis=-1, keepdims=True) + 1e-5)

    def ln_store(src, key):
        b, r, s0 = key
        xn = _packed((ln_rows(src, *key) - mean.pop(key)) * rstd.pop(key))
        for c in range(nc):
            st(at("xn", b, r, c) + s0 // 2, xn[:, lanes[c]])

    def ln_unit(src, keys, n):
        for stage, fn in enumerate((ln_mean, ln_rstd, ln_store)):
            if 0 <= n - stage < len(keys):
                fn(src, keys[n - stage])

    def emit_out(src, fsrc, b, j, c, o, s0=0):
        n = o[0].shape[0]
        outs = []
        for e in range(2):
            r = 2 * j + e
            xn = pltpu.bitcast(src[rows(at("xn", b, r, c) + s0 // 2, n // 2), :], bf16).astype(f32)
            outs.append(o[e] + xn * fsrc[(R + r) * P + s0:(R + r) * P + s0 + n, lanes[c]])
        if src is ordered:
            arena[pl.ds(at("o", b, c) + j + 2 * s0, n, stride=2), :] = _pair(*outs)
        else:
            obuf.at[c].bitcast(u32)[pl.ds(j + 2 * s0, n, stride=2), :] = _pair(*outs)
        if j == 1 and s0 + n == P:
            out_copies.append(out_copy(b, c, src))
            out_copies[-1].start()

    def fin_gate(b):
        fbuf[b][F_ROWS:F_ROWS + 8, 0:LANES] = ld(at("k", 0, 0), 8)

    def fin_unit(b, j, c, s0):
        o = [f_ord[b][(2 * j + e) * P + s0:(2 * j + e) * P + s0 + FR, lanes[c]] for e in range(2)]
        tick = delayed(f_ord[b][0:8, lanes[c]], 7)
        emit_out(ordered, f_ord[b], b, j, c, o, s0)
        fbuf[b][F_ROWS:F_ROWS + 8, 0:LANES] = tick
        st(at("tick", 0), tick)

    queue = []
    credit = [0]

    def fill(cycles):
        credit[0] += cycles
        while queue and credit[0] >= queue[0][2]:
            _, fn, cost = queue.pop(0)
            credit[0] -= cost
            fn()
        if not queue:
            credit[0] = min(credit[0], 128)

    def need(tag):
        while any(t == tag for t, _, _ in queue):
            queue.pop(0)[1]()

    marks = {}
    pieces = []
    cursor = [0]

    def weights(row, n):
        i = cursor[0]
        assert pieces[i][0] == row
        cursor[0] += 1
        for p in range(len(marks), min(i + 1 + LAG, len(pieces))):
            need(pieces[p][1])
            marks[p] = ordered[rows(pieces[p][0], 8), :]
            fill(pieces[p][2])
        return pltpu.bitcast(jnp.concatenate([marks[i], arena[rows(row + 8, n - 8), :]], axis=0), bf16)

    def mm1_op(b, j, s0, s1):
        need(("ln", b, j))
        w = jnp.concatenate([weights(at("w1", c) + s0 // 2, (s1 - s0) // 2) for c in range(nc)], axis=1)
        x = pltpu.bitcast(jnp.concatenate([wide("xn", b, 2 * j), wide("xn", b, 2 * j + 1)], axis=0), bf16)
        h = jax.lax.dot_general(x, w, (((1,), (1,)), ((), ())), preferred_element_type=f32) + b1s[0:1, s0:s1]
        u = h * (h * h * (_GC * 0.044715) + _GC)
        hh = 0.5 * h
        hbuf[b][j][:, s0:s1] = _packed(hh * jnp.tanh(u) + hh)

    def mm2_op(b, j, c, fused):
        w = jnp.concatenate([weights(at("w2", c) + s0 // 2, (min(s0 + FC, F) - s0) // 2)
                             for s0 in range(0, F, FC)], axis=0)
        mlp = jnp.dot(pltpu.bitcast(hbuf[b][j][...], bf16), w, preferred_element_type=f32)
        mlp = [mlp[0:P], mlp[P:2 * P]]
        qw = q_words(arena, b, j, c)
        o = [mlp[0] + prm[5:6, lanes[c]] + _lo(qw), mlp[1] + prm[5:6, lanes[c]] + _hi(qw)]
        if fused:
            emit_out(arena, fbuf[b], b, j, c, o)
        else:
            for e in range(2):
                fbuf[b][(2 * j + e) * P:(2 * j + e + 1) * P, lanes[c]] = o[e]

    def fwd_op(b, r, src, dst):
        x = jnp.concatenate([weights(at(src, b, r, c), H) for c in range(nc)], axis=1)
        e = jnp.dot(pltpu.bitcast(fwd_ref[r], bf16), x, preferred_element_type=f32)
        row = (dst * R + r) * SR
        ebuf[b][row:row + P, :] = e[0:P]
        ebuf[b][row + IM:row + IM + P, :] = e[P:2 * P]

    def inv_op(b, r):
        z = jnp.concatenate([weights(at("z", b, r, c), P) for c in range(nc)], axis=1)
        fbuf[b][(R + r) * P:(R + r + 1) * P, :] = jnp.dot(pltpu.bitcast(inv_ref[r], bf16), z,
                                                         preferred_element_type=f32)

    part = functools.partial

    prog = []

    def push(units):
        prog.append(part(queue.extend, units))

    def ln(src, blocks):
        keys = [(b, r, s0) for b in blocks for r in range(R) for s0 in range(0, P, LR)]
        tag = lambda n: ("ln", keys[n][0], keys[n][1] // 2)
        return [(tag(max(n - 2, 0)), part(ln_unit, src, keys, n), C_LN) for n in range(len(keys) + 2)]

    def prep(blocks):
        ts = [(b, c, n) for b in blocks for c in range(nc) for n in range(R)]
        lead, out = [], []
        for i in range(-TL - 1, len(ts)):
            tag, dst = ("prep", ts[max(i, 0)][0]), lead if i < 0 else out
            if i + TL + 1 < len(ts):
                dst.append((tag, part(t_load, *ts[i + TL + 1]), 0))
            for j in range(2):
                if j == 1 and -1 <= i < len(ts) - 1:
                    dst.append((tag, part(t_store, *ts[i + 1]), 0))
                if i >= 0:
                    b, c, n = ts[i]
                    dst += [(tag, part(prep_unit, b, j, c, s0), C_PREP)
                            for s0 in range(n * P // R, (n + 1) * P // R, PR)]

        def enqueue():
            n = 2 * TL + 2
            tail = queue[-n:]
            tail += [(lead[0][0], lambda: None, C_LN)] * (n - len(tail))
            queue[-n:] = mix(tail, lead) + out

        prog.append(enqueue)

    def spectral(b):
        return [(("m", b), part(m_unit, b, g0, c), C_M[b]) for g0 in range(0, P, RG) for c in range(nc)]

    def fin(b, n=nc):
        return [(("fin", b), part(fin_gate, b), 0)] + [
            (("fin", b), part(fin_unit, b, j, c, s0), C_FIN)
            for c in range(n) for j in range(2) for s0 in range(0, P, FR)]

    def mix(main, extra):
        out = []
        for i, u in enumerate(main):
            out += extra[i * len(extra) // len(main):(i + 1) * len(extra) // len(main)] + [u]
        return out

    def mm1(b, lo=0, hi=None):
        for s0, j in [(s0, j) for s0 in range(0, F, FC) for j in range(2)][lo:hi]:
            s1 = min(s0 + FC, F)
            pieces.extend((at("w1", c) + s0 // 2, None, 64 * pl.cdiv(s1 - s0, LANES)) for c in range(nc))
            prog.append(part(mm1_op, b, j, s0, s1))

    def mm2(b, lo=0, hi=None, fused=False):
        for c, j in [(c, j) for c in range(nc) for j in range(2)][lo:hi]:
            pieces.extend((at("w2", c) + s0 // 2, None, 128) for s0 in range(0, F, FC))
            prog.append(part(mm2_op, b, j, c, fused))

    def fwd(b):
        for r in range(R):
            for dst, src in enumerate(("xu", "xk")):
                pieces.extend((at(src, b, r, c), ("prep", b), 64) for c in range(nc))
                prog.append(part(fwd_op, b, r, src, dst))

    def inv(b):
        for r in range(R):
            pieces.extend((at("z", b, r, c), ("m", b), 64) for c in range(nc))
            prog.append(part(inv_op, b, r))

    def run(then_wait=(), then_start=()):
        for step in prog:
            step()
        prog.clear(), pieces.clear(), marks.clear()
        cursor[0] = 0
        credit[0] = -256
        start(then_start)
        wait(then_wait)

    feed = [q_in(0), w1_in(0, 2 * FC, 0) + small_in, w1_in(2 * FC, 5 * FC, 2), w1_in(5 * FC, F, 6) + q_in(1),
            q_in(2) + conv_in(0) + tables_in[:1], w2_in + conv_in(1) + q_in(3) + tables_in[1:],
            conv_in(2) + conv_in(3)]
    cuts = [pltpu.make_async_copy(q_hbm.at[0:16, 0:LANES], cut_buf.at[i], cut_sem.at[i]) for i in range(NCUT)]

    def params():
        prm[0:4, :] = shift_ref[...].astype(f32)
        prm[4:5, :] = sd_ref[...].astype(f32).reshape(1, D)
        prm[5:6, :] = b2_ref[...].astype(f32).reshape(1, D)
        b1s[...] = b1_ref[...].astype(f32).reshape(1, F)

    start(feed[0] + feed[1])
    for c in range(nc):
        st(at("k", 0, c), jnp.zeros((8, LANES), u32))
    wait(feed[0])
    start(feed[2])
    push(ln(arena, [0]))
    prog.append(part(need, ("ln", 0, 1)))
    run(feed[1])
    params()
    mm1(0, 0, 4)
    run(feed[2], feed[3])
    mm1(0, 4, 10)
    run(feed[3], feed[4] + cuts)
    push([(t, f, 125) for t, f, _ in ln(ordered, [1])])
    mm1(0, 10)
    mm1(1, 0, 8)
    run(feed[4], feed[5])
    prep([0])
    mm1(1, 8)
    push(ln(ordered, [2]))
    fwd(0)
    push(spectral(0))
    mm1(2)
    run(feed[5], feed[6])
    prep([1])
    mm2(0, 0, 6)
    push(ln(ordered, [3]))
    fwd(1)
    push(spectral(1))
    mm2(0, 6)
    inv(0)
    mm2(1, 0, 4)
    run(feed[6])
    prep([2, 3])
    mm1(3)
    fwd(2)
    run(cuts[0:1])
    push(spectral(2))
    mm2(1, 4, 6)
    fwd(3)
    mm2(1, 6)
    mm2(2, 0, 2)
    inv(1)
    run(cuts[1:2])
    push(spectral(3))
    mm2(2, 2)
    inv(2)
    mm2(3, 0, 2)
    inv(3)
    push(fin(0) + fin(1) + fin(2) + fin(3, 1))
    mm2(3, 2, fused=True)
    prog.append(part(need, ("fin", 3)))
    run()
    wait(out_copies)


@jax.jit
def pallas_parallel_sum__ssm_conv_h3__dense_activation_gelu__prompt_kernel(
    A_q: jax.Array,
    A_k: jax.Array,
    A_v: jax.Array,
    A_shift_k: jax.Array,
    A_ssm_k: jax.Array,
    A_ssm_D: jax.Array,
    B_x: jax.Array,
    B_w1: jax.Array,
    B_b1: jax.Array,
    B_w2: jax.Array,
    B_b2: jax.Array,
):
    B, S, D = A_q.shape
    F = B_w1.shape[1]
    nc, nb = D // LANES, S // TB
    assert (B, nb, D % LANES, F // FC, A_shift_k.shape[1]) == (1, 4, 0, 6, 4)
    q, k, v = (a.reshape(S, D) for a in (A_q, A_k, A_v))
    hbm = pl.BlockSpec(memory_space=pltpu.HBM)
    out = pl.pallas_call(
        functools.partial(_kernel, nc=nc, nb=nb, D=D, F=F),
        in_specs=[pl.BlockSpec(memory_space=pltpu.SMEM)] + [hbm] * 12,
        out_specs=hbm,
        out_shape=jax.ShapeDtypeStruct((S, D), A_q.dtype),
        scratch_shapes=[
            pltpu.VMEM((4, D), bf16), pltpu.VMEM((D,), bf16), pltpu.VMEM((F,), bf16), pltpu.VMEM((D,), bf16),
            pltpu.VMEM(_FWD.shape, u32), pltpu.VMEM(_INV.shape, u32),
            pltpu.VMEM((2 * _layout(nb, nc, F)[1], LANES), bf16),
            [pltpu.VMEM((2 * R * SR + 8, D), f32) for _ in range(nb)],
            [pltpu.VMEM((2 * R * P + 8, D), f32) for _ in range(nb)],
            pltpu.VMEM((nc, TB + 16, LANES), bf16),
            pltpu.VMEM((8, D), f32),
            pltpu.VMEM((1, F), f32),
            [[pltpu.VMEM((P, F), u32) for _ in range(2)] for _ in range(nb)],
            pltpu.SemaphoreType.DMA((4, nb)),
            pltpu.SemaphoreType.DMA((7,)),
            pltpu.SemaphoreType.DMA((nb,)),
            pltpu.VMEM((NCUT, 16, LANES), bf16),
            pltpu.SemaphoreType.DMA((NCUT,)),
        ],
        compiler_params=pltpu.CompilerParams(vmem_limit_bytes=120 * 1024 * 1024),
    )(jnp.asarray(np.zeros((1,), np.int32)), q, k, v, A_ssm_k, B_w1.T, B_w2, A_shift_k.T, A_ssm_D, B_b1, B_b2,
      jnp.asarray(_FWD), jnp.asarray(_INV))
    return out.reshape(B, S, D)
```

```python
import functools

import numpy as np
import jax
import jax.numpy as jnp
import jax.experimental.pallas as pl
import jax.experimental.pallas.tpu as pltpu

R = 4
P = 128
H = P // 2
TB = R * P
NFFT = 2 * TB
LANES = 128
IM, SR = P + 8, 2 * P + 24
RG = 8
PR, LR, FR = 16, 16, 64
C_LN, C_PREP, C_FIN, C_M = 135, 70, 105, (120, 118, 118, 124)
LAG, TL, PT, NCUT = 2, 2, 5, 2
NP = 3
WR, C_WS = 32, 85
MT = (0, 0, 0, 0)
FC = 256


def _pack_rows(m):
    u = np.ascontiguousarray(m, np.float32).view(np.uint32).astype(np.uint64)
    h = ((u + 0x7FFF + ((u >> 16) & 1)) >> 16).astype(np.uint32)
    return h[..., 0::2, :] | (h[..., 1::2, :] << np.uint32(16))


def _dft_tables():
    g = np.concatenate([np.arange(0, P, 2), np.arange(1, P, 2)]).astype(np.float64)
    s = np.arange(P, dtype=np.float64)
    fwd, inv = [], []
    for r in range(R):
        th = 2.0 * np.pi * (g[:, None] + 0.5) * (R * s[None, :] + r) / NFFT
        fwd.append(np.concatenate([np.cos(th), -np.sin(th)], 0))
        inv.append(np.stack([np.cos(th).T, -np.sin(th).T], 2).reshape(P, 2 * P) * (2.0 / NFFT))
    return _pack_rows(np.stack(fwd)), _pack_rows(np.stack(inv))


_FWD, _INV = _dft_tables()
_GC = float(np.sqrt(2.0 / np.pi))
f32, bf16, u32 = jnp.float32, jnp.bfloat16, jnp.uint32


def _layout(nb, nc, F):
    spec = dict(q=(nb * nc, TB // 2 + 8), k=(nb * nc, 8 + TB // 2 + 8),
                v=(nb * nc, TB // 2 + 8), kt=(nb * nc, TB // 2 + 8),
                sk=(nb * R * nc, H),
                o=(nb * nc, TB // 2 + 8), w1=(nc, F // 2), w2=(nc, F // 2),
                xn=(nb * R * nc, H), xu=(nb * R * nc, H), xk=(nb * R * nc, H),
                u=((nb - 1) * R * nc, SR), kf=((nb - 1) * R * nc, SR),
                z=(nb * R * nc, P + 8), tick=(1, 8),
                ws=(10, NP * FC // 2))
    off, out = 0, {}
    for name, (n, rows) in spec.items():
        out[name] = (off, rows)
        off += n * rows
    return out, off


def _lo(w):
    return pltpu.bitcast(w << 16, f32)


def _hi(w):
    return pltpu.bitcast(w & np.uint32(0xFFFF0000), f32)


def _packed(x):
    return pltpu.bitcast(x.astype(bf16), u32)


def _pair(a, b):
    return pltpu.bitcast(pltpu.pack_elementwise([a, b], packed_dtype=bf16), u32)


def _gelu(h):
    hh = 0.5 * h
    return hh * jnp.tanh(h * (h * h * (_GC * 0.044715) + _GC)) + hh


def _kernel(zero_ref, q_hbm, k_hbm, v_hbm, sk_hbm, w1_hbm, w2_hbm,
            shift_hbm, sd_hbm, b1_hbm, b2_hbm, fwd_hbm, inv_hbm,
            o_hbm,
            shift_ref, sd_ref, b1_ref, b2_ref, fwd_ref, inv_ref,
            arena16, ebuf, fbuf, obuf, prm, b1s, b1t, hbuf, hsum, cacc, in_sem, w_sem, out_sem, cut_buf, cut_sem, *, nc, nb, D, F):
    lanes = [slice(c * LANES, (c + 1) * LANES) for c in range(nc)]
    lay, _ = _layout(nb, nc, F)
    FA = F // LANES * LANES
    arena = arena16.bitcast(u32)
    zero = pl.multiple_of(zero_ref[0], 8)

    i0 = jnp.zeros((), jnp.int32)

    def rows(start, n):
        return pl.ds(pl.multiple_of(i0 + start, 8), n)

    def late(ref):
        return ref.at[pl.ds(zero, ref.shape[0]), :]

    ordered = late(arena)
    e_ord, f_ord = [late(r) for r in ebuf], [late(r) for r in fbuf]
    E_ROWS, F_ROWS = 2 * R * SR, 2 * R * P

    def at(name, *idx):
        n = 0
        for i in idx[:-1]:
            n = n * R + i
        return lay[name][0] + (n * nc + idx[-1]) * lay[name][1]

    def ws_at(i, ci):
        return lay["ws"][0] + (i * 2 + ci) * lay["ws"][1]

    def ld(row, n):
        return pltpu.bitcast(ordered[rows(row, n), :], f32)

    def st(row, val):
        arena[rows(row, val.shape[0]), :] = pltpu.bitcast(val, u32)

    def slab16(row, n):
        return arena16.at[2 * row:2 * (row + n), :]

    def wide(name, *idx):
        return jnp.concatenate([arena[rows(at(name, *idx, c), lay[name][1]), :] for c in range(nc)], axis=1)

    def cols_in(src, b, offs, sem, history=0):
        return [pltpu.make_async_copy(src.at[pl.ds(b * TB - 2 * history, TB + 2 * history), lanes[c]],
                                      slab16(offs[c] - history, TB // 2 + history), sem) for c in range(nc)]

    def conv_in(b):
        return (cols_in(k_hbm, b, [at("k", b, c) + 8 for c in range(nc)], in_sem.at[0, b], 8 if b else 0)
                + cols_in(v_hbm, b, [at("v", b, c) for c in range(nc)], in_sem.at[1, b])
                + [pltpu.make_async_copy(sk_hbm.at[lanes[c], pl.ds(b * TB + n * P, P)],
                                         slab16(at("sk", b, n, c), H), in_sem.at[2, b])
                   for c in range(nc) for n in range(R)])

    def q_in(b):
        return cols_in(q_hbm, b, [at("q", b, c) for c in range(nc)], in_sem.at[3, b])

    out_copies, written = [], {}

    def out_copy(b, c, src):
        return pltpu.make_async_copy(slab16(at("o", b, c), TB // 2) if src is ordered else obuf.at[b * nc + c, 0:TB, :],
                                     o_hbm.at[pl.ds(b * TB, TB), lanes[c]], out_sem.at[b])

    def w1_in(lo, hi, n):
        return [pltpu.make_async_copy(w1_hbm.at[lo:hi, lanes[c]], slab16(at("w1", c) + lo // 2, (hi - lo) // 2),
                                      w_sem.at[n]) for c in range(nc)]

    small_in = [pltpu.make_async_copy(src, dst, w_sem.at[3]) for src, dst in (
        (shift_hbm, shift_ref), (sd_hbm, sd_ref), (b1_hbm, b1_ref), (b2_hbm, b2_ref))]
    tables_in = [pltpu.make_async_copy(fwd_hbm, fwd_ref, w_sem.at[4]),
                 pltpu.make_async_copy(inv_hbm, inv_ref, w_sem.at[5])]
    w2_in = [pltpu.make_async_copy(w2_hbm.at[:, lanes[c]], slab16(at("w2", c), F // 2), w_sem.at[1])
             for c in range(nc)]

    def start(cs):
        for c in cs:
            c.start()

    def wait(cs):
        for c in cs:
            c.wait()

    def delayed(x, n):
        for _ in range(n):
            x = jnp.tanh(x)
        return x

    tiles = {}

    def t_load(b, c, n):
        w = pltpu.bitcast(ordered[rows(at("sk", b, n, c), H), :], bf16)
        tiles[b, c, n] = pltpu.bitcast(w.T, u32)

    def t_store(b, c, n):
        st(at("kt", b, c) + n * H, tiles.pop((b, c, n)))

    def prep_unit(b, j, c, s0):
        base = at("k", b, c) + 8 + j + 2 * s0
        t = ordered[rows(at("k", b, c), 8), :]
        t = delayed(pltpu.bitcast(t, f32), PT)

        wa = ordered[pl.ds(base - 2, PR, stride=2), :]
        wb = ordered[pl.ds(base - 1, PR, stride=2), :]
        wc = ordered[pl.ds(base, PR, stride=2), :]
        ks = [_hi(wa), _lo(wb), _hi(wb), _lo(wc), _hi(wc)]
        vw = ordered[pl.ds(at("v", b, c) + j + 2 * s0, PR, stride=2), :]
        vs = [_lo(vw), _hi(vw)]
        tw = ordered[pl.ds(at("kt", b, c) + j + 2 * s0, PR, stride=2), :]
        ts = [_lo(tw), _hi(tw)]
        for e in range(2):
            acc = ks[3 + e] * prm[0:1, lanes[c]]
            for i in range(1, 4):
                acc = acc + ks[3 + e - i] * prm[i:i + 1, lanes[c]]
            st(at("xu", b, 2 * j + e, c) + s0 // 2, _packed(acc * vs[e]))
            st(at("xk", b, 2 * j + e, c) + s0 // 2, _packed(ts[e]))
        st(at("tick", 0), t)

    def m_unit(b, g0, c):
        def cld(name, slot, m):
            row = at(name, slot, m, c) + g0
            return ld(row, RG), ld(row + IM, RG)

        def cst(name, m, vr, vi):
            row = at(name, b, m, c) + g0
            st(row, vr)
            st(row + IM, vi)

        def bfly(which):
            offs = [(which * R + r) * SR + g0 for r in range(R)]
            er = [e_ord[b % 2][rows(o, RG), lanes[c]] for o in offs]
            ei = [e_ord[b % 2][rows(o + IM, RG), lanes[c]] for o in offs]
            ar, ai = er[0] + er[2], ei[0] + ei[2]
            br, bi = er[0] - er[2], ei[0] - ei[2]
            cr, ci = er[1] + er[3], ei[1] + ei[3]
            dr, di = er[1] - er[3], ei[1] - ei[3]
            return ([ar + cr, br + di, ar - cr, br - di],
                    [ai + ci, bi - dr, ai - ci, bi + dr])

        tick = e_ord[b % 2][rows(g0, RG), lanes[c]]
        tick = delayed(tick, MT[b]) if MT[b] else pltpu.roll(tick, 1, 1)
        ur, ui = bfly(0)
        kr, ki = bfly(1)
        if b == 0:
            kr = [x + prm[4:5, lanes[c]] for x in kr]
        if b < nb - 1:
            for m in range(R):
                cst("u", m, ur[m], ui[m])
                cst("kf", m, kr[m], ki[m])
        else:
            st(at("tick", 0), ki[R - 1])
        yr, yi = [], []
        for m in range(R):
            us = [cld("u", n, m) for n in range(b)] + [(ur[m], ui[m])]
            ks = [cld("kf", n, m) for n in range(b)] + [(kr[m], ki[m])]
            accr = acci = None
            for n in range(b + 1):
                (a_r, a_i), (b_r, b_i) = us[b - n], ks[n]
                if n:
                    p_r, p_i = ks[n - 1]
                    b_r, b_i = (b_r - p_i, b_i + p_r) if g0 < P // 2 else (b_r + p_i, b_i - p_r)
                pr_ = a_r * b_r - a_i * b_i
                pi_ = a_r * b_i + a_i * b_r
                accr = pr_ if accr is None else accr + pr_
                acci = pi_ if acci is None else acci + pi_
            yr.append(accr)
            yi.append(acci)
            if b >= 2 and m == 1:
                st(at("tick", 0), acci)
        ar, ai = yr[0] + yr[2], yi[0] + yi[2]
        br, bi = yr[0] - yr[2], yi[0] - yi[2]
        cr, ci = yr[1] + yr[3], yi[1] + yi[3]
        dr, di = yr[1] - yr[3], yi[1] - yi[3]
        zr = [ar + cr, br - di, ar - cr, br + di]
        zi = [ai + ci, bi + dr, ai - ci, bi - dr]
        for r in range(R):
            st(at("z", b, r, c) + g0, _pair(zr[r], zi[r]))
        ebuf[b % 2][E_ROWS:E_ROWS + RG, 0:LANES] = tick
        st(at("tick", 0), tick)

    def q_words(src, b, j, c):
        return src[pl.ds(at("q", b, c) + j, P, stride=2), :]

    def ln_rows(src, b, e, s0):
        return jnp.concatenate([
            jnp.concatenate([(_lo, _hi)[e](src[pl.ds(at("q", b, c) + j + 2 * s0, LR, stride=2), :])
                             for c in range(nc)], axis=1) for j in range(2)], axis=0)

    mean, rstd = {}, {}

    def ln_mean(src, key):
        mean[key] = jnp.mean(ln_rows(src, *key), axis=-1, keepdims=True)

    def ln_rstd(src, key):
        xc = ln_rows(src, *key) - mean[key]
        rstd[key] = jax.lax.rsqrt(jnp.mean(xc * xc, axis=-1, keepdims=True) + 1e-5)

    def ln_store(src, key):
        b, e, s0 = key
        xn = (ln_rows(src, *key) - mean.pop(key)) * rstd.pop(key)
        for j in range(2):
            for c in range(nc):
                st(at("xn", b, 2 * j + e, c) + s0 // 2, _packed(xn[j * LR:(j + 1) * LR, lanes[c]]))

    def ln_unit(src, keys, n):
        for stage, fn in enumerate((ln_mean, ln_rstd, ln_store)):
            if 0 <= n - stage < len(keys):
                fn(src, keys[n - stage])

    def wsum_unit(ci, s0):
        words = [ordered[rows(at("w2", ci + 2 * n) + k * NP * FC // 2 + s0, WR), :] for k in range(2) for n in range(2)]
        tick = delayed(_lo(words[0][0:8]), PT)
        halves = []
        for half in (_lo, _hi):
            b11, b12, b21, b22 = map(half, words)
            halves.append((b11 + b22, b12 - b22, b21 - b11, b11 + b12, b21 + b22))
        for i in range(5):
            st(ws_at(i, ci) + s0, _pair(halves[0][i], halves[1][i]))
        st(at("tick", 0), tick)

    def emit_out(src, fsrc, b, j, c, o, s0=0):
        n = o[0].shape[0]
        outs = []
        for e in range(2):
            r = 2 * j + e
            xn = pltpu.bitcast(src[rows(at("xn", b, r, c) + s0 // 2, n // 2), :], bf16).astype(f32)
            outs.append(o[e] + xn * fsrc[(R + r) * P + s0:(R + r) * P + s0 + n, lanes[c]])
        if src is ordered:
            arena[pl.ds(at("o", b, c) + j + 2 * s0, n, stride=2), :] = _pair(*outs)
        else:
            obuf.at[b * nc + c].bitcast(u32)[pl.ds(j + 2 * s0, n, stride=2), :] = _pair(*outs)
        written[b, c] = written.get((b, c), 0) + n
        if written[b, c] == 2 * P:
            out_copies.append(out_copy(b, c, src))
            out_copies[-1].start()

    def fin_gate(b):
        fbuf[b][F_ROWS:F_ROWS + 8, 0:LANES] = ld(at("k", 0, 0), 8)

    def fin_unit(b, j, c, s0):
        o = [f_ord[b][(2 * j + e) * P + s0:(2 * j + e) * P + s0 + FR, lanes[c]] for e in range(2)]
        tick = delayed(f_ord[b][0:8, lanes[c]], 7)
        emit_out(ordered, f_ord[b], b, j, c, o, s0)
        fbuf[b][F_ROWS:F_ROWS + 8, 0:LANES] = tick
        st(at("tick", 0), tick)

    queue = []
    credit = [0]

    def fill(cycles):
        credit[0] += cycles
        while queue and credit[0] >= queue[0][2]:
            _, fn, cost = queue.pop(0)
            credit[0] -= cost
            fn()
        if not queue:
            credit[0] = min(credit[0], 128)

    def need(tag):
        while any(t == tag for t, _, _ in queue):
            queue.pop(0)[1]()

    marks = {}
    pieces = []
    cursor = [0]

    def weights(row, n):
        i = cursor[0]
        assert pieces[i][0] == row
        cursor[0] += 1
        for p in range(len(marks), min(i + 1 + LAG, len(pieces))):
            need(pieces[p][1])
            marks[p] = ordered[rows(pieces[p][0], 8), :]
            fill(pieces[p][2])
        return pltpu.bitcast(jnp.concatenate([marks[i], arena[rows(row + 8, n - 8), :]], axis=0), bf16)

    def nt_dot(x_rows, w_rows, n):
        w = jnp.concatenate([weights(row, n) for row in w_rows], axis=1)
        x = jnp.concatenate([jnp.concatenate([arena[rows(row, H), :] for row in xe], axis=1) for xe in x_rows], axis=0)
        return jax.lax.dot_general(pltpu.bitcast(x, bf16), w, (((1,), (1,)), ((), ())), preferred_element_type=f32)

    def hidden(b, p, quarter, h):
        j, k = divmod(quarter, 2)
        g = _gelu(h)
        h11, h21, h22 = cacc[p % 2]
        hbuf[b][j][:, (k * NP + p) * FC:(k * NP + p + 1) * FC] = _packed(g)
        if quarter == 2:
            h21[...], sums = g, {}
        elif quarter == 3:
            h22[...], sums = g, {1: h21[...] + g}
        elif quarter == 0:
            h11[...], sums = g, {0: g + h22[...], 3: h21[...] - g}
        else:
            sums = {2: h11[...] + g, 4: g - h22[...]}
        for i, v in sums.items():
            hsum[b][i][:, p * FC:(p + 1) * FC] = _packed(v)

    def bias1(p, quarter):
        s0 = (quarter % 2 * NP + p) * FC
        return b1s[0:1, s0:s0 + FC]

    def mm1_plain(b, p, quarter):
        j, k = divmod(quarter, 2)
        x = [[at("xn", b, 2 * j + e, c) for c in range(nc)] for e in range(2)]
        w = [at("w1", c) + (k * NP + p) * FC // 2 for c in range(nc)]
        return w, None, lambda: hidden(b, p, quarter, nt_dot(x, w, FC // 2) + bias1(p, quarter))

    def mm1_tail(b, j):
        x = [[at("xn", b, 2 * j + e, c) for c in range(nc)] for e in range(2)]
        w = [at("w1", c) + NP * FC for c in range(nc)]

        def op():
            h = nt_dot(x, w, (FA - 2 * NP * FC) // 2) + b1s[0:1, 2 * NP * FC:FA]
            hbuf[b][j][:, 2 * NP * FC:FA] = _packed(_gelu(h))

        return w, None, op

    def mm1_rest_op(b):
        x = jnp.concatenate([jnp.concatenate([weights(at("xn", b, r, c), H) for c in range(nc)], axis=1)
                             for r in range(R)], axis=0)
        w = jnp.concatenate([arena[rows(at("w1", c) + FA // 2, (F - FA) // 2), :] for c in range(nc)], axis=1)
        h = jax.lax.dot_general(pltpu.bitcast(w, bf16), x, (((1,), (1,)), ((), ())), preferred_element_type=f32)
        for r in range(R):
            g = _gelu(h[:, r * P:(r + 1) * P] + b1t[...])
            hbuf[b][r // 2][(r % 2) * H:(r % 2 + 1) * H, FA:F] = _packed(g.T)

    def nn_dot(h, w_pieces):
        w = jnp.concatenate([weights(row, n) for row, n in w_pieces], axis=0)
        return jnp.dot(pltpu.bitcast(h, bf16), w, preferred_element_type=f32)

    def mlp_update(b, j, c, m, sign, action, fused):
        window = [(slice((2 * j + e) * P, (2 * j + e + 1) * P), lanes[c]) for e in range(2)]
        if action in ("init", "all"):
            qw = q_words(arena, b, j, c)
            old = [prm[5:6, lanes[c]] + half(qw) for half in (_lo, _hi)]
        else:
            old = [fbuf[b][win] for win in window]
        new = [old[e] + m[e * P:(e + 1) * P] if sign > 0 else old[e] - m[e * P:(e + 1) * P] for e in range(2)]
        if fused and action in ("done", "all"):
            emit_out(arena, fbuf[b], b, j, c, new)
        else:
            for e in range(2):
                fbuf[b][window[e]] = new[e]

    def mm2_plain(b, j, c, fused):
        w = [(at("w2", c) + s0 // 2, (min(s0 + FC, F) - s0) // 2) for s0 in range(0, F, FC)]
        return w, None, lambda: mlp_update(b, j, c, nn_dot(hbuf[b][j][...], w), 1, "all", fused)

    STRASSEN = (
        ([("s", 1)], [0], [(2, 1, "init"), (3, -1, "init")]),
        ([("r", 1)], [("r", 0)], [(2, 1, "add")]),
        ([0], [("s", 1)], [(1, 1, "init"), (3, 1, "add")]),
        ([("r", 0)], [("r", 1)], [(1, 1, "add")]),
        ([("s", 0)], [("s", 0)], [(0, 1, "init"), (3, 1, "add")]),
        ([3], [("s", 2)], [(2, 1, "done"), (0, 1, "add")]),
        ([("s", 2)], [3], [(1, 1, "done"), (0, -1, "add")]),
        ([("s", 3), ("r", 1)], [("s", 3), ("r", 1)], [(3, 1, "done")]),
        ([("s", 4), ("r", 0)], [("s", 4), ("r", 0)], [(0, 1, "done")]),
    )

    def mm2_strassen(b, ci, n, fused):
        left, right, updates = STRASSEN[n]
        w = []
        for o in right:
            if not isinstance(o, int) and o[0] == "r":
                w.append((at("w2", ci + 2 * o[1]) + NP * FC, F // 2 - NP * FC))
            else:
                row = at("w2", ci + 2 * (o % 2)) + o // 2 * NP * FC // 2 if isinstance(o, int) else ws_at(o[1], ci)
                w += [(row + p * FC // 2, FC // 2) for p in range(NP)]

        def op():
            h = [hbuf[b][o // 2][:, o % 2 * NP * FC:(o % 2 + 1) * NP * FC] if isinstance(o, int)
                 else hsum[b][o[1]][...] if o[0] == "s" else hbuf[b][o[1]][:, 2 * NP * FC:F] for o in left]
            m = nn_dot(jnp.concatenate(h, axis=1), w)
            for quarter, sign, action in updates:
                mlp_update(b, quarter // 2, ci + 2 * (quarter % 2), m, sign, action, fused)

        return w, ("ws", ci), op

    def fwd_op(b, r, src, dst):
        x = jnp.concatenate([weights(at(src, b, r, c), H) for c in range(nc)], axis=1)
        e = jnp.dot(pltpu.bitcast(fwd_ref[r], bf16), x, preferred_element_type=f32)
        row = (dst * R + r) * SR
        ebuf[b % 2][row:row + P, :] = e[0:P]
        ebuf[b % 2][row + IM:row + IM + P, :] = e[P:2 * P]

    def inv_op(b, r):
        z = jnp.concatenate([weights(at("z", b, r, c), P) for c in range(nc)], axis=1)
        fbuf[b][(R + r) * P:(R + r + 1) * P, :] = jnp.dot(pltpu.bitcast(inv_ref[r], bf16), z,
                                                         preferred_element_type=f32)

    part = functools.partial

    prog = []

    def push(units):
        prog.append(part(queue.extend, units))

    def ln(src, blocks, cycles=C_LN):
        keys = [(b, e, s0) for b in blocks for e in range(2) for s0 in range(0, P, LR)]
        tag = lambda n: ("ln", keys[n][0])
        return [(tag(max(n - 2, 0)), part(ln_unit, src, keys, n), cycles) for n in range(len(keys) + 2)]

    def prep(blocks):
        ts = [(b, c, n) for b in blocks for c in range(nc) for n in range(R)]
        lead, out = [], []
        for i in range(-TL - 1, len(ts)):
            tag, dst = ("prep", ts[max(i, 0)][0]), lead if i < 0 else out
            if i + TL + 1 < len(ts):
                dst.append((tag, part(t_load, *ts[i + TL + 1]), 0))
            for j in range(2):
                if j == 1 and -1 <= i < len(ts) - 1:
                    dst.append((tag, part(t_store, *ts[i + 1]), 0))
                if i >= 0:
                    b, c, n = ts[i]
                    dst += [(tag, part(prep_unit, b, j, c, s0), C_PREP)
                            for s0 in range(n * P // R, (n + 1) * P // R, PR)]

        def enqueue():
            n = 2 * TL + 2
            tail = queue[-n:]
            tail += [(lead[0][0], lambda: None, C_LN)] * (n - len(tail))
            queue[-n:] = mix(tail, lead) + out

        prog.append(enqueue)

    def spectral(b):
        return [(("m", b), part(m_unit, b, g0, c), C_M[b]) for g0 in range(0, P, RG) for c in range(nc)]

    def fin(b, tiles=range(nc)):
        return [(("fin", b), part(fin_gate, b), 0)] + [
            (("fin", b), part(fin_unit, b, j, c, s0), C_FIN)
            for c in tiles for j in range(2) for s0 in range(0, P, FR)]

    def mix(main, extra):
        out = []
        for i, u in enumerate(main):
            out += extra[i * len(extra) // len(main):(i + 1) * len(extra) // len(main)] + [u]
        return out

    def mm1(b, p, lo=0, hi=None):
        ops = [mm1_tail(b, j) for j in range(2)] if p == NP else [mm1_plain(b, p, quarter) for quarter in (2, 3, 0, 1)]
        for w, tag, op in ops[lo:hi]:
            pieces.extend((row, tag, 64 if p == NP else 128) for row in w)
            prog.extend([part(need, ("ln", b)), op])
        if p == NP:
            pieces.extend((at("xn", b, r, c), ("ln", b), 16) for r in range(R) for c in range(nc))
            prog.append(part(mm1_rest_op, b))

    def mm2(b, ci, fused=False, lo=0, hi=None):
        ops = ([mm2_plain(b, j, nc - 1, fused) for j in range(2)] if ci == 2
               else [mm2_strassen(b, ci, n, fused) for n in range(len(STRASSEN))])
        for w, tag, op in ops[lo:hi]:
            pieces.extend((row, tag, 128) for row, _ in w)
            prog.append(op)

    def wsums():
        return [(("ws", ci), part(wsum_unit, ci, s0), C_WS) for ci in range(2) for s0 in range(0, NP * FC // 2, WR)]

    def fwd(b):
        for r in range(R):
            for dst, src in enumerate(("xu", "xk")):
                pieces.extend((at(src, b, r, c), ("prep", b), 64) for c in range(nc))
                prog.append(part(fwd_op, b, r, src, dst))

    def inv(b):
        for r in range(R):
            pieces.extend((at("z", b, r, c), ("m", b), 64) for c in range(nc))
            prog.append(part(inv_op, b, r))

    def run(then_wait=(), then_start=()):
        for step in prog:
            step()
        prog.clear(), pieces.clear(), marks.clear()
        cursor[0] = 0
        credit[0] = -256
        start(then_start)
        wait(then_wait)

    def w1_pair(p, n):
        return w1_in(p * FC, (p + 1) * FC, n) + w1_in((NP + p) * FC, (NP + p + 1) * FC, n)

    feed = [q_in(0), w1_pair(0, 0) + small_in, w1_pair(1, 2) + w1_in(2 * NP * FC, F, 2), w1_pair(2, 6) + q_in(1),
            q_in(2), q_in(3) + conv_in(0) + tables_in[:1], w2_in + conv_in(1) + conv_in(2) + tables_in[1:], conv_in(3)]
    cuts = [pltpu.make_async_copy(q_hbm.at[0:16, 0:LANES], cut_buf.at[i], cut_sem.at[i]) for i in range(NCUT)]

    def params():
        prm[0:4, :] = shift_ref[...].astype(f32)
        prm[4:5, :] = sd_ref[...].astype(f32).reshape(1, D)
        prm[5:6, :] = b2_ref[...].astype(f32).reshape(1, D)
        b1s[...] = jnp.zeros(b1s.shape, f32)
        b1s[:, 0:F] = b1_ref[...].astype(f32).reshape(1, F)
        b1t[...] = jnp.broadcast_to(b1s[:, FA:FA + LANES], (LANES, LANES)).T[0:F - FA]

    start(feed[0] + feed[1])
    for c in range(nc):
        st(at("k", 0, c), jnp.zeros((8, LANES), u32))
    wait(feed[0])
    start(feed[2])
    push(ln(arena, [0]))
    prog.append(part(need, ("ln", 0)))
    run(feed[1])
    params()
    mm1(0, 0)
    run(feed[2], feed[3])
    mm1(0, NP)
    mm1(0, 1)
    run(feed[3], feed[4] + feed[5] + cuts)
    push(ln(ordered, [1]))
    mm1(0, 2)
    mm1(1, 0, 0, 2)
    run(feed[4])
    push(ln(ordered, [2], 190))
    mm1(1, 0, 2)
    mm1(1, 1)
    run(feed[5], feed[6])
    prep([0])
    mm1(1, 2)
    mm1(1, NP)
    mm1(2, 0)
    push(ln(ordered, [3]))
    fwd(0)
    push(spectral(0))
    mm1(2, 1)
    mm1(2, 2)
    mm1(2, NP)
    mm1(3, 0)
    run(feed[6], feed[7])
    push(wsums())
    prep([1, 2])
    mm1(3, 1, 0, 2)
    inv(0)
    mm2(0, 2, True)
    mm2(0, 0, True)
    mm2(0, 1, True, 0, 4)
    fwd(1)
    push(spectral(1))
    mm2(0, 1, True, 4)
    mm1(3, 1, 2)
    fwd(2)
    run(feed[7])
    mm1(3, NP)
    mm1(3, 2)
    mm2(1, 0, True, 0, 5)
    prep([3])
    mm2(1, 1, True, 0, 5)
    inv(1)
    mm2(1, 0, True, 5)
    mm2(1, 1, True, 5)
    mm2(1, 2, True)
    push(spectral(2))
    fwd(3)
    run(cuts[0:1])
    mm2(2, 0, True, 0, 5)
    mm2(2, 1, True, 0, 5)
    mm2(3, 2)
    run(cuts[1:2])
    push(spectral(3))
    mm2(3, 0, False, 0, 5)
    mm2(3, 1, True, 0, 5)
    inv(2)
    mm2(2, 0, True, 5)
    mm2(2, 1, True, 5)
    mm2(2, 2, True)
    mm2(3, 0, False, 5)
    inv(3)
    push(fin(3, [4, 0, 2]))
    mm2(3, 1, True, 5)
    prog.append(part(need, ("fin", 3)))
    run()
    wait(out_copies)


@jax.jit
def pallas_parallel_sum__ssm_conv_h3__dense_activation_gelu__prompt_kernel(
    A_q: jax.Array,
    A_k: jax.Array,
    A_v: jax.Array,
    A_shift_k: jax.Array,
    A_ssm_k: jax.Array,
    A_ssm_D: jax.Array,
    B_x: jax.Array,
    B_w1: jax.Array,
    B_b1: jax.Array,
    B_w2: jax.Array,
    B_b2: jax.Array,
):
    B, S, D = A_q.shape
    F = B_w1.shape[1]
    nc, nb = D // LANES, S // TB
    assert (B, nb, D % LANES, F // FC, A_shift_k.shape[1]) == (1, 4, 0, 6, 4)
    q, k, v = (a.reshape(S, D) for a in (A_q, A_k, A_v))
    hbm = pl.BlockSpec(memory_space=pltpu.HBM)
    out = pl.pallas_call(
        functools.partial(_kernel, nc=nc, nb=nb, D=D, F=F),
        in_specs=[pl.BlockSpec(memory_space=pltpu.SMEM)] + [hbm] * 12,
        out_specs=hbm,
        out_shape=jax.ShapeDtypeStruct((S, D), A_q.dtype),
        scratch_shapes=[
            pltpu.VMEM((4, D), bf16), pltpu.VMEM((D,), bf16), pltpu.VMEM((F,), bf16), pltpu.VMEM((D,), bf16),
            pltpu.VMEM(_FWD.shape, u32), pltpu.VMEM(_INV.shape, u32),
            pltpu.VMEM((2 * _layout(nb, nc, F)[1], LANES), bf16),
            [pltpu.VMEM((2 * R * SR + 8, D), f32) for _ in range(2)],
            [pltpu.VMEM((2 * R * P + 8, D), f32) for _ in range(nb)],
            pltpu.VMEM((nb * nc, TB + 16, LANES), bf16),
            pltpu.VMEM((8, D), f32),
            pltpu.VMEM((1, pl.cdiv(F, LANES) * LANES), f32),
            pltpu.VMEM((F % LANES, LANES), f32),
            [[pltpu.VMEM((P, F), u32) for _ in range(2)] for _ in range(nb)],
            [[pltpu.VMEM((P, NP * FC), u32) for _ in range(5)] for _ in range(nb)],
            [[pltpu.VMEM((2 * P, FC), f32) for _ in range(3)] for _ in range(2)],
            pltpu.SemaphoreType.DMA((4, nb)),
            pltpu.SemaphoreType.DMA((7,)),
            pltpu.SemaphoreType.DMA((nb,)),
            pltpu.VMEM((NCUT, 16, LANES), bf16),
            pltpu.SemaphoreType.DMA((NCUT,)),
        ],
        compiler_params=pltpu.CompilerParams(vmem_limit_bytes=124 * 1024 * 1024),
    )(jnp.asarray(np.zeros((1,), np.int32)), q, k, v, A_ssm_k, B_w1.T, B_w2, A_shift_k.T, A_ssm_D, B_b1, B_b2,
      jnp.asarray(_FWD), jnp.asarray(_INV))
    return out.reshape(B, S, D)
```

```python
import functools

import numpy as np
import jax
import jax.numpy as jnp
import jax.experimental.pallas as pl
import jax.experimental.pallas.tpu as pltpu

R = 4
P = 128
H = P // 2
TB = R * P
NFFT = 2 * TB
LANES = 128
IM, SR = P + 8, 2 * P + 24
RG = 8
PR, LR, FR, WR = 16, 16, 64, 32
C_LN, C_PREP, C_FIN, C_WS, C_M = 135, 70, 105, 85, (120, 118, 116, 121)
LAG, TL, PT, NCUT = 2, 2, 5, 2
NP = 3
FC = 256


def _pack_rows(m):
    u = np.ascontiguousarray(m, np.float32).view(np.uint32).astype(np.uint64)
    h = ((u + 0x7FFF + ((u >> 16) & 1)) >> 16).astype(np.uint32)
    return h[..., 0::2, :] | (h[..., 1::2, :] << np.uint32(16))


def _dft_tables():
    g = np.concatenate([np.arange(0, P, 2), np.arange(1, P, 2)]).astype(np.float64)
    s = np.arange(P, dtype=np.float64)
    fwd, inv = [], []
    for r in range(R):
        th = 2.0 * np.pi * (g[:, None] + 0.5) * (R * s[None, :] + r) / NFFT
        fwd.append(np.concatenate([np.cos(th), -np.sin(th)], 0))
        inv.append(np.stack([np.cos(th).T, -np.sin(th).T], 2).reshape(P, 2 * P) * (2.0 / NFFT))
    return _pack_rows(np.stack(fwd)), _pack_rows(np.stack(inv))


_FWD, _INV = _dft_tables()
_GC = float(np.sqrt(2.0 / np.pi))
f32, bf16, u32 = jnp.float32, jnp.bfloat16, jnp.uint32


def _layout(nb, nc, F):
    spec = dict(q=(nb * nc, TB // 2 + 8), k=(nb * nc, 8 + TB // 2 + 8),
                v=(nb * nc, TB // 2 + 8), kt=(nb * nc, TB // 2 + 8),
                sk=(nb * R * nc, H),
                o=(nb * nc, TB // 2 + 8), w1=(nc, F // 2), w2=(nc, F // 2),
                xn=(nb * R * nc, H), xu=(nb * R * nc, H), xk=(nb * R * nc, H),
                u=((nb - 1) * R * nc, SR), kf=((nb - 1) * R * nc, SR),
                z=(nb * R * nc, P + 8), tick=(1, 8),
                ws=(10, NP * FC // 2))
    off, out = 0, {}
    for name, (n, rows) in spec.items():
        out[name] = (off, rows)
        off += n * rows
    return out, off


def _lo(w):
    return pltpu.bitcast(w << 16, f32)


def _hi(w):
    return pltpu.bitcast(w & np.uint32(0xFFFF0000), f32)


def _packed(x):
    return pltpu.bitcast(x.astype(bf16), u32)


def _pair(a, b):
    return pltpu.bitcast(pltpu.pack_elementwise([a, b], packed_dtype=bf16), u32)


def _gelu(h):
    hh = 0.5 * h
    return hh * jnp.tanh(h * (h * h * (_GC * 0.044715) + _GC)) + hh


def _kernel(zero_ref, q_hbm, k_hbm, v_hbm, sk_hbm, w1_hbm, w2_hbm,
            shift_hbm, sd_hbm, b1_hbm, b2_hbm, fwd_hbm, inv_hbm,
            o_hbm,
            shift_ref, sd_ref, b1_ref, b2_ref, fwd_ref, inv_ref,
            arena16, ebuf, fbuf, obuf, prm, b1s, b1t, hbuf, hsum, cacc, in_sem, w_sem, out_sem, cut_buf, cut_sem, *, nc, nb, D, F):
    lanes = [slice(c * LANES, (c + 1) * LANES) for c in range(nc)]
    lay, _ = _layout(nb, nc, F)
    FA = F // LANES * LANES
    arena = arena16.bitcast(u32)
    zero = pl.multiple_of(zero_ref[0], 8)

    i0 = jnp.zeros((), jnp.int32)

    def rows(start, n):
        return pl.ds(pl.multiple_of(i0 + start, 8), n)

    def late(ref):
        return ref.at[pl.ds(zero, ref.shape[0]), :]

    ordered = late(arena)
    e_ord, f_ord = [late(r) for r in ebuf], [late(r) for r in fbuf]
    E_ROWS, F_ROWS = 2 * R * SR, 2 * R * IM

    def at(name, *idx):
        n = 0
        for i in idx[:-1]:
            n = n * R + i
        return lay[name][0] + (n * nc + idx[-1]) * lay[name][1]

    def ws_at(i, ci):
        return lay["ws"][0] + (i * 2 + ci) * lay["ws"][1]

    def ld(row, n):
        return pltpu.bitcast(ordered[rows(row, n), :], f32)

    def st(row, val):
        arena[rows(row, val.shape[0]), :] = pltpu.bitcast(val, u32)

    def slab16(row, n):
        return arena16.at[2 * row:2 * (row + n), :]

    def cols_in(src, b, offs, sem, history=0):
        return [pltpu.make_async_copy(src.at[pl.ds(b * TB - 2 * history, TB + 2 * history), lanes[c]],
                                      slab16(offs[c] - history, TB // 2 + history), sem) for c in range(nc)]

    def conv_in(b):
        return (cols_in(k_hbm, b, [at("k", b, c) + 8 for c in range(nc)], in_sem.at[0, b], 8 if b else 0)
                + cols_in(v_hbm, b, [at("v", b, c) for c in range(nc)], in_sem.at[1, b])
                + [pltpu.make_async_copy(sk_hbm.at[lanes[c], pl.ds(b * TB + n * P, P)],
                                         slab16(at("sk", b, n, c), H), in_sem.at[2, b])
                   for c in range(nc) for n in range(R)])

    def q_in(b):
        return cols_in(q_hbm, b, [at("q", b, c) for c in range(nc)], in_sem.at[3, b])

    out_copies, written = [], {}

    def out_copy(b, c, src):
        return pltpu.make_async_copy(slab16(at("o", b, c), TB // 2) if src is ordered else obuf.at[b * nc + c, 0:TB, :],
                                     o_hbm.at[pl.ds(b * TB, TB), lanes[c]], out_sem.at[b])

    def w1_in(lo, hi, n):
        return [pltpu.make_async_copy(w1_hbm.at[lo:hi, lanes[c]], slab16(at("w1", c) + lo // 2, (hi - lo) // 2),
                                      w_sem.at[n]) for c in range(nc)]

    small_in = [pltpu.make_async_copy(src, dst, w_sem.at[3]) for src, dst in (
        (shift_hbm, shift_ref), (sd_hbm, sd_ref), (b1_hbm, b1_ref), (b2_hbm, b2_ref))]
    tables_in = [pltpu.make_async_copy(fwd_hbm, fwd_ref, w_sem.at[4]),
                 pltpu.make_async_copy(inv_hbm, inv_ref, w_sem.at[5])]
    w2_in = [pltpu.make_async_copy(w2_hbm.at[:, lanes[c]], slab16(at("w2", c), F // 2), w_sem.at[1])
             for c in range(nc)]

    def start(cs):
        for c in cs:
            c.start()

    def wait(cs):
        for c in cs:
            c.wait()

    def delayed(x, n):
        for _ in range(n):
            x = jnp.tanh(x)
        return x

    tiles = {}

    def t_load(b, c, n):
        w = pltpu.bitcast(ordered[rows(at("sk", b, n, c), H), :], bf16)
        tiles[b, c, n] = pltpu.bitcast(w.T, u32)

    def t_store(b, c, n):
        st(at("kt", b, c) + n * H, tiles.pop((b, c, n)))

    def prep_unit(b, j, c, s0):
        base = at("k", b, c) + 8 + j + 2 * s0
        t = ordered[rows(at("k", b, c), 8), :]
        t = delayed(pltpu.bitcast(t, f32), PT)

        wa = ordered[pl.ds(base - 2, PR, stride=2), :]
        wb = ordered[pl.ds(base - 1, PR, stride=2), :]
        wc = ordered[pl.ds(base, PR, stride=2), :]
        ks = [_hi(wa), _lo(wb), _hi(wb), _lo(wc), _hi(wc)]
        vw = ordered[pl.ds(at("v", b, c) + j + 2 * s0, PR, stride=2), :]
        vs = [_lo(vw), _hi(vw)]
        tw = ordered[pl.ds(at("kt", b, c) + j + 2 * s0, PR, stride=2), :]
        ts = [_lo(tw), _hi(tw)]
        for e in range(2):
            acc = ks[3 + e] * prm[0:1, lanes[c]]
            for i in range(1, 4):
                acc = acc + ks[3 + e - i] * prm[i:i + 1, lanes[c]]
            st(at("xu", b, 2 * j + e, c) + s0 // 2, _packed(acc * vs[e]))
            st(at("xk", b, 2 * j + e, c) + s0 // 2, _packed(ts[e]))
        st(at("tick", 0), t)

    def m_unit(b, g0, c):
        def cld(name, slot, m):
            row = at(name, slot, m, c) + g0
            return ld(row, RG), ld(row + IM, RG)

        def cst(name, m, vr, vi):
            row = at(name, b, m, c) + g0
            st(row, vr)
            st(row + IM, vi)

        def bfly(which):
            offs = [(which * R + r) * SR + g0 for r in range(R)]
            er = [e_ord[b % 2][rows(o, RG), lanes[c]] for o in offs]
            ei = [e_ord[b % 2][rows(o + IM, RG), lanes[c]] for o in offs]
            ar, ai = er[0] + er[2], ei[0] + ei[2]
            br, bi = er[0] - er[2], ei[0] - ei[2]
            cr, ci = er[1] + er[3], ei[1] + ei[3]
            dr, di = er[1] - er[3], ei[1] - ei[3]
            return ([ar + cr, br + di, ar - cr, br - di],
                    [ai + ci, bi - dr, ai - ci, bi + dr])

        tick = pltpu.roll(e_ord[b % 2][rows(g0, RG), lanes[c]], 1, 1)
        ur, ui = bfly(0)
        kr, ki = bfly(1)
        if b == 0:
            kr = [x + prm[4:5, lanes[c]] for x in kr]
        if b < nb - 1:
            for m in range(R):
                cst("u", m, ur[m], ui[m])
                cst("kf", m, kr[m], ki[m])
        else:
            st(at("tick", 0), ki[R - 1])
        yr, yi = [], []
        for m in range(R):
            us = [cld("u", n, m) for n in range(b)] + [(ur[m], ui[m])]
            ks = [cld("kf", n, m) for n in range(b)] + [(kr[m], ki[m])]
            accr = acci = None
            for n in range(b + 1):
                (a_r, a_i), (b_r, b_i) = us[b - n], ks[n]
                if n:
                    p_r, p_i = ks[n - 1]
                    b_r, b_i = (b_r - p_i, b_i + p_r) if g0 < P // 2 else (b_r + p_i, b_i - p_r)
                pr_ = a_r * b_r - a_i * b_i
                pi_ = a_r * b_i + a_i * b_r
                accr = pr_ if accr is None else accr + pr_
                acci = pi_ if acci is None else acci + pi_
            yr.append(accr)
            yi.append(acci)
            if b >= 2 and m == 1:
                st(at("tick", 0), acci)
        ar, ai = yr[0] + yr[2], yi[0] + yi[2]
        br, bi = yr[0] - yr[2], yi[0] - yi[2]
        cr, ci = yr[1] + yr[3], yi[1] + yi[3]
        dr, di = yr[1] - yr[3], yi[1] - yi[3]
        zr = [ar + cr, br - di, ar - cr, br + di]
        zi = [ai + ci, bi + dr, ai - ci, bi - dr]
        for r in range(R):
            st(at("z", b, r, c) + g0, _pair(zr[r], zi[r]))
        ebuf[b % 2][E_ROWS:E_ROWS + RG, 0:LANES] = tick
        st(at("tick", 0), tick)

    def q_words(src, b, j, c):
        return src[pl.ds(at("q", b, c) + j, P, stride=2), :]

    def ln_rows(src, b, e, s0):
        return jnp.concatenate([
            jnp.concatenate([(_lo, _hi)[e](src[pl.ds(at("q", b, c) + j + 2 * s0, LR, stride=2), :])
                             for c in range(nc)], axis=1) for j in range(2)], axis=0)

    mean, rstd = {}, {}

    def ln_mean(src, key):
        mean[key] = jnp.mean(ln_rows(src, *key), axis=-1, keepdims=True)

    def ln_rstd(src, key):
        xc = ln_rows(src, *key) - mean[key]
        rstd[key] = jax.lax.rsqrt(jnp.mean(xc * xc, axis=-1, keepdims=True) + 1e-5)

    def ln_store(src, key):
        b, e, s0 = key
        xn = (ln_rows(src, *key) - mean.pop(key)) * rstd.pop(key)
        for j in range(2):
            for c in range(nc):
                st(at("xn", b, 2 * j + e, c) + s0 // 2, _packed(xn[j * LR:(j + 1) * LR, lanes[c]]))

    def ln_unit(src, keys, n):
        for stage, fn in enumerate((ln_mean, ln_rstd, ln_store)):
            if 0 <= n - stage < len(keys):
                fn(src, keys[n - stage])

    def wsum_unit(ci, s0):
        words = [ordered[rows(at("w2", ci + 2 * n) + k * NP * FC // 2 + s0, WR), :] for k in range(2) for n in range(2)]
        tick = delayed(_lo(words[0][0:8]), PT)
        halves = []
        for half in (_lo, _hi):
            b11, b12, b21, b22 = map(half, words)
            halves.append((b11 + b22, b12 - b22, b21 - b11, b11 + b12, b21 + b22))
        for i in range(5):
            st(ws_at(i, ci) + s0, _pair(halves[0][i], halves[1][i]))
        st(at("tick", 0), tick)

    def emit_out(src, fsrc, b, j, c, o, s0=0):
        n = o[0].shape[0]
        outs = []
        for e in range(2):
            r = 2 * j + e
            xn = pltpu.bitcast(src[rows(at("xn", b, r, c) + s0 // 2, n // 2), :], bf16).astype(f32)
            outs.append(o[e] + xn * fsrc[(R + r) * IM + s0:(R + r) * IM + s0 + n, lanes[c]])
        if src is ordered:
            arena[pl.ds(at("o", b, c) + j + 2 * s0, n, stride=2), :] = _pair(*outs)
        else:
            obuf.at[b * nc + c].bitcast(u32)[pl.ds(j + 2 * s0, n, stride=2), :] = _pair(*outs)
        written[b, c] = written.get((b, c), 0) + n
        if written[b, c] == 2 * P:
            out_copies.append(out_copy(b, c, src))
            out_copies[-1].start()

    def fin_gate(b):
        fbuf[b][F_ROWS:F_ROWS + 8, 0:LANES] = ld(at("k", 0, 0), 8)

    def fin_unit(b, j, c, s0):
        o = [f_ord[b][(2 * j + e) * IM + s0:(2 * j + e) * IM + s0 + FR, lanes[c]] for e in range(2)]
        tick = delayed(f_ord[b][0:8, lanes[c]], 7)
        emit_out(ordered, f_ord[b], b, j, c, o, s0)
        fbuf[b][F_ROWS:F_ROWS + 8, 0:LANES] = tick
        st(at("tick", 0), tick)

    queue = []
    credit = [0]

    def fill(cycles):
        credit[0] += cycles
        while queue and credit[0] >= queue[0][2]:
            _, fn, cost = queue.pop(0)
            credit[0] -= cost
            fn()
        if not queue:
            credit[0] = min(credit[0], 128)

    def need(tag):
        while any(t == tag for t, _, _ in queue):
            queue.pop(0)[1]()

    marks = {}
    pieces = []
    cursor = [0]

    def weights(row, n):
        i = cursor[0]
        assert pieces[i][0] == row
        cursor[0] += 1
        for p in range(len(marks), min(i + 1 + LAG, len(pieces))):
            need(pieces[p][1])
            marks[p] = ordered[rows(pieces[p][0], 8), :]
            fill(pieces[p][2])
        return pltpu.bitcast(jnp.concatenate([marks[i], arena[rows(row + 8, n - 8), :]], axis=0), bf16)

    def nt_dot(x_rows, w_rows, n):
        w = jnp.concatenate([weights(row, n) for row in w_rows], axis=1)
        x = jnp.concatenate([jnp.concatenate([arena[rows(row, H), :] for row in xe], axis=1) for xe in x_rows], axis=0)
        return jax.lax.dot_general(pltpu.bitcast(x, bf16), w, (((1,), (1,)), ((), ())), preferred_element_type=f32)

    def hidden(b, p, quarter, h):
        j, k = divmod(quarter, 2)
        g = _gelu(h)
        h11, h21, h22 = cacc[p % 2]
        hbuf[b][j][:, (k * NP + p) * FC:(k * NP + p + 1) * FC] = _packed(g)
        if quarter == 2:
            h21[...], sums = g, {}
        elif quarter == 3:
            h22[...], sums = g, {1: h21[...] + g}
        elif quarter == 0:
            h11[...], sums = g, {0: g + h22[...], 3: h21[...] - g}
        else:
            sums = {2: h11[...] + g, 4: g - h22[...]}
        for i, v in sums.items():
            hsum[b][i][:, p * FC:(p + 1) * FC] = _packed(v)

    def bias1(p, quarter):
        s0 = (quarter % 2 * NP + p) * FC
        return b1s[0:1, s0:s0 + FC]

    def mm1_plain(b, p, quarter):
        j, k = divmod(quarter, 2)
        x = [[at("xn", b, 2 * j + e, c) for c in range(nc)] for e in range(2)]
        w = [at("w1", c) + (k * NP + p) * FC // 2 for c in range(nc)]
        return w, None, lambda: hidden(b, p, quarter, nt_dot(x, w, FC // 2) + bias1(p, quarter))

    def mm1_tail(b, j):
        x = [[at("xn", b, 2 * j + e, c) for c in range(nc)] for e in range(2)]
        w = [at("w1", c) + NP * FC for c in range(nc)]

        def op():
            h = nt_dot(x, w, (FA - 2 * NP * FC) // 2) + b1s[0:1, 2 * NP * FC:FA]
            hbuf[b][j][:, 2 * NP * FC:FA] = _packed(_gelu(h))

        return w, None, op

    def mm1_rest_op(b):
        x = jnp.concatenate([jnp.concatenate([weights(at("xn", b, r, c), H) for c in range(nc)], axis=1)
                             for r in range(R)], axis=0)
        w = jnp.concatenate([arena[rows(at("w1", c) + FA // 2, (F - FA) // 2), :] for c in range(nc)], axis=1)
        h = jax.lax.dot_general(pltpu.bitcast(w, bf16), x, (((1,), (1,)), ((), ())), preferred_element_type=f32)
        for r in range(R):
            g = _gelu(h[:, r * P:(r + 1) * P] + b1t[...])
            hbuf[b][r // 2][(r % 2) * H:(r % 2 + 1) * H, FA:F] = _packed(g.T)

    def nn_dot(h, w_pieces):
        w = jnp.concatenate([weights(row, n) for row, n in w_pieces], axis=0)
        return jnp.dot(pltpu.bitcast(h, bf16), w, preferred_element_type=f32)

    def mlp_update(b, j, c, m, sign, action, fused):
        window = [(slice((2 * j + e) * IM, (2 * j + e) * IM + P), lanes[c]) for e in range(2)]
        if action in ("init", "all"):
            qw = q_words(arena, b, j, c)
            old = [prm[5:6, lanes[c]] + half(qw) for half in (_lo, _hi)]
        else:
            old = [fbuf[b][win] for win in window]
        new = [old[e] + m[e * P:(e + 1) * P] if sign > 0 else old[e] - m[e * P:(e + 1) * P] for e in range(2)]
        if fused and action in ("done", "all"):
            emit_out(arena, fbuf[b], b, j, c, new)
        else:
            for e in range(2):
                fbuf[b][window[e]] = new[e]

    def mm2_plain(b, j, c, fused):
        w = [(at("w2", c) + s0 // 2, (min(s0 + FC, F) - s0) // 2) for s0 in range(0, F, FC)]
        return w, None, lambda: mlp_update(b, j, c, nn_dot(hbuf[b][j][...], w), 1, "all", fused)

    STRASSEN = (
        ([("s", 1)], [0], [(2, 1, "init"), (3, -1, "init")]),
        ([("r", 1)], [("r", 0)], [(2, 1, "add")]),
        ([0], [("s", 1)], [(1, 1, "init"), (3, 1, "add")]),
        ([("r", 0)], [("r", 1)], [(1, 1, "add")]),
        ([("s", 0)], [("s", 0)], [(0, 1, "init"), (3, 1, "add")]),
        ([3], [("s", 2)], [(2, 1, "done"), (0, 1, "add")]),
        ([("s", 2)], [3], [(1, 1, "done"), (0, -1, "add")]),
        ([("s", 3), ("r", 1)], [("s", 3), ("r", 1)], [(3, 1, "done")]),
        ([("s", 4), ("r", 0)], [("s", 4), ("r", 0)], [(0, 1, "done")]),
    )

    def mm2_strassen(b, ci, n, fused):
        left, right, updates = STRASSEN[n]
        w = []
        for o in right:
            if not isinstance(o, int) and o[0] == "r":
                w.append((at("w2", ci + 2 * o[1]) + NP * FC, F // 2 - NP * FC))
            else:
                row = at("w2", ci + 2 * (o % 2)) + o // 2 * NP * FC // 2 if isinstance(o, int) else ws_at(o[1], ci)
                w += [(row + p * FC // 2, FC // 2) for p in range(NP)]

        def op():
            h = [hbuf[b][o // 2][:, o % 2 * NP * FC:(o % 2 + 1) * NP * FC] if isinstance(o, int)
                 else hsum[b][o[1]][...] if o[0] == "s" else hbuf[b][o[1]][:, 2 * NP * FC:F] for o in left]
            m = nn_dot(jnp.concatenate(h, axis=1), w)
            for quarter, sign, action in updates:
                mlp_update(b, quarter // 2, ci + 2 * (quarter % 2), m, sign, action, fused)

        return w, ("ws", ci), op

    def fwd_op(b, r, src, dst):
        x = jnp.concatenate([weights(at(src, b, r, c), H) for c in range(nc)], axis=1)
        e = jnp.dot(pltpu.bitcast(fwd_ref[r], bf16), x, preferred_element_type=f32)
        row = (dst * R + r) * SR
        ebuf[b % 2][row:row + P, :] = e[0:P]
        ebuf[b % 2][row + IM:row + IM + P, :] = e[P:2 * P]

    def inv_op(b, r):
        z = jnp.concatenate([weights(at("z", b, r, c), P) for c in range(nc)], axis=1)
        fbuf[b][(R + r) * IM:(R + r) * IM + P, :] = jnp.dot(pltpu.bitcast(inv_ref[r], bf16), z,
                                                         preferred_element_type=f32)

    part = functools.partial

    prog = []

    def push(units):
        prog.append(part(queue.extend, units))

    def ln(src, blocks, cycles=C_LN):
        keys = [(b, e, s0) for b in blocks for e in range(2) for s0 in range(0, P, LR)]
        tag = lambda n: ("ln", keys[n][0])
        return [(tag(max(n - 2, 0)), part(ln_unit, src, keys, n), cycles) for n in range(len(keys) + 2)]

    def prep(blocks):
        ts = [(b, c, n) for b in blocks for c in range(nc) for n in range(R)]
        lead, out = [], []
        for i in range(-TL - 1, len(ts)):
            tag, dst = ("prep", ts[max(i, 0)][0]), lead if i < 0 else out
            if i + TL + 1 < len(ts):
                dst.append((tag, part(t_load, *ts[i + TL + 1]), 0))
            for j in range(2):
                if j == 1 and -1 <= i < len(ts) - 1:
                    dst.append((tag, part(t_store, *ts[i + 1]), 0))
                if i >= 0:
                    b, c, n = ts[i]
                    dst += [(tag, part(prep_unit, b, j, c, s0), C_PREP)
                            for s0 in range(n * P // R, (n + 1) * P // R, PR)]

        def enqueue():
            n = 2 * TL + 2
            tail = queue[-n:]
            tail += [(lead[0][0], lambda: None, C_LN)] * (n - len(tail))
            queue[-n:] = mix(tail, lead) + out

        prog.append(enqueue)

    def spectral(b):
        return [(("m", b), part(m_unit, b, g0, c), C_M[b]) for g0 in range(0, P, RG) for c in range(nc)]

    def fin(b, tiles=range(nc)):
        return [(("fin", b), part(fin_gate, b), 0)] + [
            (("fin", b), part(fin_unit, b, j, c, s0), C_FIN)
            for c in tiles for j in range(2) for s0 in range(0, P, FR)]

    def mix(main, extra):
        out = []
        for i, u in enumerate(main):
            out += extra[i * len(extra) // len(main):(i + 1) * len(extra) // len(main)] + [u]
        return out

    def mm1(b, p, lo=0, hi=None):
        ops = [mm1_tail(b, j) for j in range(2)] if p == NP else [mm1_plain(b, p, quarter) for quarter in (2, 3, 0, 1)]
        for w, tag, op in ops[lo:hi]:
            pieces.extend((row, tag, 64 if p == NP else 128) for row in w)
            prog.extend([part(need, ("ln", b)), op])
        if p == NP:
            pieces.extend((at("xn", b, r, c), ("ln", b), 16) for r in range(R) for c in range(nc))
            prog.append(part(mm1_rest_op, b))

    def mm2(b, ci, fused=False, lo=0, hi=None):
        ops = ([mm2_plain(b, j, nc - 1, fused) for j in range(2)] if ci == 2
               else [mm2_strassen(b, ci, n, fused) for n in range(len(STRASSEN))])
        for w, tag, op in ops[lo:hi]:
            pieces.extend((row, tag, 128) for row, _ in w)
            prog.append(op)

    def wsums():
        return [(("ws", ci), part(wsum_unit, ci, s0), C_WS) for ci in range(2) for s0 in range(0, NP * FC // 2, WR)]

    def fwd(b):
        for r in range(R):
            for dst, src in enumerate(("xu", "xk")):
                pieces.extend((at(src, b, r, c), ("prep", b), 64) for c in range(nc))
                prog.append(part(fwd_op, b, r, src, dst))

    def inv(b):
        for r in range(R):
            pieces.extend((at("z", b, r, c), ("m", b), 64) for c in range(nc))
            prog.append(part(inv_op, b, r))

    def run(then_wait=(), then_start=()):
        for step in prog:
            step()
        prog.clear(), pieces.clear(), marks.clear()
        cursor[0] = 0
        credit[0] = -256
        start(then_start)
        wait(then_wait)

    def w1_pair(p, n):
        return w1_in(p * FC, (p + 1) * FC, n) + w1_in((NP + p) * FC, (NP + p + 1) * FC, n)

    feed = [q_in(0), w1_pair(0, 0) + small_in, w1_pair(1, 2) + w1_in(2 * NP * FC, F, 2), w1_pair(2, 6) + q_in(1),
            q_in(2), q_in(3) + conv_in(0) + tables_in[:1], w2_in + conv_in(1) + conv_in(2) + tables_in[1:], conv_in(3)]
    cuts = [pltpu.make_async_copy(q_hbm.at[0:16, 0:LANES], cut_buf.at[i], cut_sem.at[i]) for i in range(NCUT)]

    def params():
        prm[0:4, :] = shift_ref[...].astype(f32)
        prm[4:5, :] = sd_ref[...].astype(f32).reshape(1, D)
        prm[5:6, :] = b2_ref[...].astype(f32).reshape(1, D)
        b1s[...] = jnp.zeros(b1s.shape, f32)
        b1s[:, 0:F] = b1_ref[...].astype(f32).reshape(1, F)
        b1t[...] = jnp.broadcast_to(b1s[:, FA:FA + LANES], (LANES, LANES)).T[0:F - FA]

    start(feed[0] + feed[1])
    for c in range(nc):
        st(at("k", 0, c), jnp.zeros((8, LANES), u32))
    wait(feed[0])
    start(feed[2])
    push(ln(arena, [0]))
    prog.append(part(need, ("ln", 0)))
    run(feed[1])
    params()
    mm1(0, 0)
    run(feed[2], feed[3])
    mm1(0, NP)
    mm1(0, 1)
    run(feed[3], feed[4] + feed[5] + cuts)
    push(ln(ordered, [1]))
    mm1(0, 2)
    mm1(1, 0, 0, 2)
    run(feed[4])
    push(ln(ordered, [2], 190))
    mm1(1, 0, 2)
    mm1(1, 1)
    run(feed[5], feed[6])
    prep([0])
    mm1(1, 2)
    mm1(1, NP)
    mm1(2, 0)
    push(ln(ordered, [3]))
    fwd(0)
    push(spectral(0))
    mm1(2, 1)
    mm1(2, 2)
    mm1(2, NP)
    mm1(3, 0)
    run(feed[6], feed[7])
    push(wsums())
    prep([1, 2])
    mm1(3, 1, 0, 2)
    inv(0)
    mm2(0, 2, True)
    mm2(0, 0, True)
    mm2(0, 1, True, 0, 4)
    fwd(1)
    push(spectral(1))
    mm2(0, 1, True, 4)
    mm1(3, 1, 2)
    fwd(2)
    run(feed[7])
    mm1(3, NP)
    mm1(3, 2)
    mm2(1, 0, True, 0, 5)
    prep([3])
    mm2(1, 1, True, 0, 5)
    inv(1)
    mm2(1, 0, True, 5)
    mm2(1, 1, True, 5)
    mm2(1, 2, True)
    push(spectral(2))
    fwd(3)
    run(cuts[0:1])
    mm2(2, 0, True, 0, 5)
    mm2(2, 1, True, 0, 5)
    mm2(3, 2)
    run(cuts[1:2])
    push(spectral(3))
    mm2(3, 0, False, 0, 5)
    mm2(3, 1, True, 0, 5)
    inv(2)
    mm2(2, 0, True, 5)
    mm2(2, 1, True, 5)
    mm2(2, 2, True)
    mm2(3, 0, False, 5)
    inv(3)
    push(fin(3, [4, 0, 2]))
    mm2(3, 1, True, 5)
    prog.append(part(need, ("fin", 3)))
    run()
    wait(out_copies)


@jax.jit
def pallas_parallel_sum__ssm_conv_h3__dense_activation_gelu__prompt_kernel(
    A_q: jax.Array,
    A_k: jax.Array,
    A_v: jax.Array,
    A_shift_k: jax.Array,
    A_ssm_k: jax.Array,
    A_ssm_D: jax.Array,
    B_x: jax.Array,
    B_w1: jax.Array,
    B_b1: jax.Array,
    B_w2: jax.Array,
    B_b2: jax.Array,
):
    B, S, D = A_q.shape
    F = B_w1.shape[1]
    nc, nb = D // LANES, S // TB
    assert (B, nb, D, F, A_shift_k.shape[1]) == (1, 4, 640, 1728, 4)
    q, k, v = (a.reshape(S, D) for a in (A_q, A_k, A_v))
    hbm = pl.BlockSpec(memory_space=pltpu.HBM)
    out = pl.pallas_call(
        functools.partial(_kernel, nc=nc, nb=nb, D=D, F=F),
        in_specs=[pl.BlockSpec(memory_space=pltpu.SMEM)] + [hbm] * 12,
        out_specs=hbm,
        out_shape=jax.ShapeDtypeStruct((S, D), A_q.dtype),
        scratch_shapes=[
            pltpu.VMEM((4, D), bf16), pltpu.VMEM((D,), bf16), pltpu.VMEM((F,), bf16), pltpu.VMEM((D,), bf16),
            pltpu.VMEM(_FWD.shape, u32), pltpu.VMEM(_INV.shape, u32),
            pltpu.VMEM((2 * _layout(nb, nc, F)[1], LANES), bf16),
            [pltpu.VMEM((2 * R * SR + 8, D), f32) for _ in range(2)],
            [pltpu.VMEM((2 * R * IM + 8, D), f32) for _ in range(nb)],
            pltpu.VMEM((nb * nc, TB + 16, LANES), bf16),
            pltpu.VMEM((8, D), f32),
            pltpu.VMEM((1, pl.cdiv(F, LANES) * LANES), f32),
            pltpu.VMEM((F % LANES, LANES), f32),
            [[pltpu.VMEM((P, F), u32) for _ in range(2)] for _ in range(nb)],
            [[pltpu.VMEM((P, NP * FC), u32) for _ in range(5)] for _ in range(nb)],
            [[pltpu.VMEM((2 * P, FC), f32) for _ in range(3)] for _ in range(2)],
            pltpu.SemaphoreType.DMA((4, nb)),
            pltpu.SemaphoreType.DMA((7,)),
            pltpu.SemaphoreType.DMA((nb,)),
            pltpu.VMEM((NCUT, 16, LANES), bf16),
            pltpu.SemaphoreType.DMA((NCUT,)),
        ],
        compiler_params=pltpu.CompilerParams(vmem_limit_bytes=124 * 1024 * 1024),
    )(jnp.asarray(np.zeros((1,), np.int32)), q, k, v, A_ssm_k, B_w1.T, B_w2, A_shift_k.T, A_ssm_D, B_b1, B_b2,
      jnp.asarray(_FWD), jnp.asarray(_INV))
    return out.reshape(B, S, D)
```
